```python
import jax
import jax.numpy as jnp

def _softmax(x, axis=-1):
    return jax.nn.softmax(x, axis=axis)

def _gelu(x):
    return jax.nn.gelu(x, approximate=True)

def _silu(x):
    return jax.nn.silu(x)

def _sigmoid(x):
    return jax.nn.sigmoid(x)

def _layernorm(x, axis=-1, eps=1e-05):
    m = jnp.mean(x, axis=axis, keepdims=True)
    v = jnp.var(x, axis=axis, keepdims=True)
    return (x - m) / jnp.sqrt(v + eps)

def _scatter_add(tgt, idx, src, axis=0):
    return tgt.at[idx].add(src)

def _segment_sum(src, seg, n):
    return jax.ops.segment_sum(src, seg, n)

class _Rng:

    def __init__(self, key):
        self._k = key

    def _next(self):
        self._k, sub = jax.random.split(self._k)
        return sub

    def normal(self, shape):
        return jax.random.normal(self._next(), shape, dtype=jnp.bfloat16)

    def randint(self, lo, hi, shape):
        return jax.random.randint(self._next(), shape, lo, hi, dtype=jnp.int32)

    def uniform(self, shape, lo=0.0, hi=1.0):
        return jax.random.uniform(self._next(), shape, jnp.bfloat16, lo, hi)

    def permutation(self, n):
        return jax.random.permutation(self._next(), n)
kernel_name = 'sequential_preLN__memory_aug_recurrent_mem_tr__moe_arch_mod__prompt'

def setup_inputs():
    _rng = _Rng(jax.random.key(int.from_bytes(__import__("os").urandom(4), "little")))
    _w = lambda a: (lambda t: t.astype(jnp.bfloat16) if jnp.issubdtype(t.dtype, jnp.floating) else t)(jnp.asarray(a))

    def _A_setup():
        B, S, Dm = (1, 2048, 512)
        H, Dh = (32, 128)
        M, seg = (8, 32)
        seg = min(seg, S)
        S = S // seg * seg
        return {'x': _w((lambda *s: _rng.normal(s) * 0.05)(B, S, Dm)), 'mem0': _w((lambda *s: _rng.normal(s) * 0.05)(B, M, Dm)), 'Wq': _w((lambda *s: _rng.normal(s) * 0.05)(Dm, H, Dh) * Dm ** (-0.5)), 'Wk': _w((lambda *s: _rng.normal(s) * 0.05)(Dm, H, Dh) * Dm ** (-0.5)), 'Wv': _w((lambda *s: _rng.normal(s) * 0.05)(Dm, H, Dh) * Dm ** (-0.5)), 'Wo': _w((lambda *s: _rng.normal(s) * 0.05)(H, Dh, Dm) * (H * Dh) ** (-0.5)), 'seg_len': seg}
    _A_in = _A_setup()

    def _B_setup():
        B, S, D, F, C = (1, 2048, 512, 1792, 2)
        return {'x': _w((lambda *s: _rng.normal(s) * 0.05)(B, S, D)), 'w_r': _w((lambda *s: _rng.normal(s) * 0.05)(D)), 'w_gate': _w((lambda *s: _rng.normal(s) * 0.05)(D, F)), 'w_up': _w((lambda *s: _rng.normal(s) * 0.05)(D, F)), 'w_down': _w((lambda *s: _rng.normal(s) * 0.05)(F, D))}
    _B_in = _B_setup()
    return {'A_x': _A_in['x'], 'A_mem0': _A_in['mem0'], 'A_Wq': _A_in['Wq'], 'A_Wk': _A_in['Wk'], 'A_Wv': _A_in['Wv'], 'A_Wo': _A_in['Wo'], 'A_seg_len': _A_in['seg_len'], 'B_x': _B_in['x'], 'B_w_r': _B_in['w_r'], 'B_w_gate': _B_in['w_gate'], 'B_w_up': _B_in['w_up'], 'B_w_down': _B_in['w_down']}

def reference(A_x, A_mem0, A_Wq, A_Wk, A_Wv, A_Wo, A_seg_len, B_x, B_w_r, B_w_gate, B_w_up, B_w_down):

    def _A_ref(x, mem0, Wq, Wk, Wv, Wo, seg_len):
        B, S, Dm = x.shape
        H, Dh = (Wq.shape[1], Wq.shape[2])
        M = mem0.shape[1]
        scale = Dh ** (-0.5)
        n_seg = S // seg_len
        L = M + seg_len
        idx = jnp.arange(L)
        mask = (idx[:, None] < M) | (idx[:, None] >= idx[None, :])
        mem = mem0
        outs = []
        for s in range(n_seg):
            xs = x[:, s * seg_len:(s + 1) * seg_len, :].copy()
            h = jnp.concatenate([mem, xs], axis=1)
            q = jnp.einsum('btd,dhe->bhte', h, Wq)
            k = jnp.einsum('btd,dhe->bhte', h, Wk)
            v = jnp.einsum('btd,dhe->bhte', h, Wv)
            scores = jnp.einsum('bhqe,bhke->bhqk', q, k) * scale
            scores = jnp.where(mask[None, None], scores, -1000000000.0)
            p = _softmax(scores, axis=-1)
            o = jnp.einsum('bhqk,bhke->bhqe', p, v)
            o = jnp.einsum('bhte,hed->btd', o, Wo)
            mem = o[:, :M, :].copy()
            outs.append(o[:, M:, :])
        return jnp.concatenate(outs, axis=1)

    def _B_ref(x, w_r, w_gate, w_up, w_down):
        B, S, D = x.shape
        C = 2
        r = x @ w_r
        idx = jnp.argsort(-r, axis=-1)[:, :C]
        idx_e = jnp.repeat(idx.reshape(B, C, 1), D, axis=2)
        x_sel = jnp.take_along_axis(x, idx_e, axis=1)
        g = _silu(x_sel @ w_gate)
        u = x_sel @ w_up
        y = g * u @ w_down
        r_sel = _sigmoid(jnp.take_along_axis(r, idx, axis=1))
        y = y * r_sel.reshape(B, C, 1)
        b_off = (jnp.arange(B) * S).reshape(B, 1)
        flat_idx = (idx + b_off).reshape(B * C)
        zero = (x * 0.0).reshape(B * S, D)
        upd = _scatter_add(zero, flat_idx, y.reshape(B * C, D), axis=0)
        return x + upd.reshape(B, S, D)
    x = A_x
    h = x + _A_ref(_layernorm(x, axis=-1), A_mem0, A_Wq, A_Wk, A_Wv, A_Wo, A_seg_len)
    h2 = h + _B_ref(_layernorm(h, axis=-1), B_w_r, B_w_gate, B_w_up, B_w_down)
    return h2
```

```python
import functools
import math

import jax
import jax.numpy as jnp
from jax import lax
import jax.experimental.pallas as pl
import jax.experimental.pallas.tpu as pltpu

BF = jnp.bfloat16
F32 = jnp.float32
U32 = jnp.uint32
I32 = jnp.int32

H, DH, DM, MEM, SEG, NSEG, DFF = 32, 128, 512, 8, 32, 64, 1792
L = MEM + SEG
XR = 8
XS = SEG - XR
GH = 8
NCH = 3 * H // GH
UNROLL = 8
D1, D2, D3, OTAIL = 3, 4, 1, 3
EPS = 1e-5
SCALE = 0.08837890625
C2 = SCALE * math.log2(math.e)
NEG = -1e9 / SCALE


def _dot(a, b):
    return lax.dot_general(a, b, (((1,), (0,)), ((), ())), preferred_element_type=F32)


def _dot_t(a, b):
    return lax.dot_general(a, b, (((1,), (1,)), ((), ())), preferred_element_type=F32)


def _rb(x):
    return x.astype(BF).astype(F32)


def _layernorm(x):
    n = x.shape[-1]
    mean = jnp.sum(x, axis=-1, keepdims=True) * (1.0 / n)
    xc = x - mean
    var = jnp.sum(xc * xc, axis=-1, keepdims=True) * (1.0 / n)
    den = _rb(jnp.sqrt(_rb(_rb(var) + EPS)))
    return _rb(_rb(x - _rb(mean)) * (1.0 / den))


def _kernel(x_hbm, m0_hbm, wq_hbm, wk_hbm, wv_hbm, wo_hbm, wr_hbm, wg_hbm, wu_hbm, wd_hbm,
            out_hbm,
            xs, m0s, wrs, stage, wos, wg, wu, wd,
            wqkv, wop, ex, xe, xn, mem, ybuf, hbuf, hnbuf, obuf, b1, i1, b2, i2,
            sem_w, sem_o, sem_x, sem_out):
    w_hbm = (wq_hbm, wk_hbm, wv_hbm)

    def w_copy(c):
        return pltpu.make_async_copy(
            w_hbm[c // 4].at[:, pl.ds((c % 4) * GH, GH), :], stage.at[c], sem_w.at[c])

    def wo_copy(j):
        return pltpu.make_async_copy(
            wo_hbm.at[pl.ds(j * 1024, 1024), :], wos.at[pl.ds(j * 1024, 1024), :], sem_o.at[j])

    xe_copy = pltpu.make_async_copy(x_hbm.at[:, pl.ds(XS, XR), :], xs.at[:, pl.ds(XS, XR), :], sem_x.at[0])
    xr_copy = pltpu.make_async_copy(x_hbm.at[:, pl.ds(0, XS), :], xs.at[:, pl.ds(0, XS), :], sem_x.at[1])
    m0_copy = pltpu.make_async_copy(m0_hbm, m0s, sem_x.at[2])
    wr_copy = pltpu.make_async_copy(wr_hbm, wrs, sem_x.at[3])
    wg_copy = pltpu.make_async_copy(wg_hbm, wg, sem_x.at[4])
    wu_copy = pltpu.make_async_copy(wu_hbm, wu, sem_x.at[5])
    wd_copy = pltpu.make_async_copy(wd_hbm, wd, sem_x.at[6])

    def repack_w(c):
        blk = 32
        for d0 in range(0, DM, blk):
            w = pltpu.bitcast(stage[c, d0:d0 + blk], U32).reshape(blk // 2, 2, GH // 2, DH)
            a = jnp.swapaxes(w[:, 0], 0, 1)
            b = jnp.swapaxes(w[:, 1], 0, 1)
            lo = (a & jnp.uint32(0xFFFF)) | (b << 16)
            hi = (a >> 16) | (b & jnp.uint32(0xFFFF0000))
            for hp in range(GH // 2):
                r0 = (c * GH + 2 * hp) * (DM // 2) + d0 // 2
                wqkv[r0:r0 + blk // 2, :] = lo[hp]
                wqkv[r0 + DM // 2:r0 + DM // 2 + blk // 2, :] = hi[hp]

    def repack_wo(j):
        for r in range(j * 1024, (j + 1) * 1024, 128):
            wop[r // 2:r // 2 + 64, :] = pltpu.bitcast(wos[r:r + 128, :], U32)

    def w_tile(j):
        return pltpu.bitcast(wqkv[j * (DM // 2):(j + 1) * (DM // 2), :], BF)

    def project_extra(c):
        for j in range(c * GH, (c + 1) * GH):
            y = _dot(xe[...], w_tile(j))
            ex[:, :, j * DH:(j + 1) * DH] = y.reshape(NSEG, XR, DH)

    def ln1_step_rows(g):
        for s in range(g * 8, (g + 1) * 8):
            xn[s] = _layernorm(xs[s, 0:XS, :].astype(F32))

    xe_copy.start()
    w_copy(0).start()
    m0_copy.start()
    wr_copy.start()
    queue = [w_copy(1), w_copy(2), xr_copy] + [w_copy(c) for c in range(3, NCH)]
    queue += [wo_copy(j) for j in range(4)] + [wg_copy, wu_copy, wd_copy]

    xe_copy.wait()
    for g in range(NSEG // 8):
        v = xs[g * 8:(g + 1) * 8, XS:SEG, :].astype(F32).reshape(8 * XR, DM)
        xe[g * 8 * XR:(g + 1) * 8 * XR, :] = _layernorm(v).astype(BF)
    w_copy(0).wait()
    for _ in range(3):
        queue.pop(0).start()
    repack_w(0)
    for c in range(NCH):
        if c + 1 < NCH:
            w_copy(c + 1).wait()
        if c == 1:
            xr_copy.wait()
        if c >= NCH - 4:
            wo_copy(c - (NCH - 4)).wait()
        for _ in range(2):
            if queue:
                queue.pop(0).start()
        project_extra(c)
        if c + 1 < NCH:
            repack_w(c + 1)
        if 1 <= c < 1 + NSEG // 8:
            ln1_step_rows(c - 1)
        if c >= NCH - 4:
            repack_wo(c - (NCH - 4))
    assert not queue

    m0_copy.wait()
    wr_copy.wait()
    mem[...] = m0s[...].astype(F32)
    ybuf[...] = jnp.zeros((SEG, DM), F32)
    rows = lax.broadcasted_iota(I32, (SEG, 1), 0)
    b1[...] = jnp.full((SEG, 1), -jnp.inf, F32)
    b2[...] = jnp.full((SEG, 1), -jnp.inf, F32)
    i1[...] = rows
    i2[...] = rows + SEG

    def finish_segment(s, live):
        h = _rb(xs[s].astype(F32) + _rb(ybuf[...]))
        hn = _layernorm(h)
        hbuf[s] = h
        hnbuf[s] = hn
        obuf[s] = (h + hn).astype(BF)
        r = _rb(jnp.sum(hn * wrs[...].astype(F32), axis=-1, keepdims=True))
        if live is not None:
            r = jnp.where(live, r, -jnp.inf)
        idx = lax.broadcasted_iota(I32, (SEG, 1), 0) + s * SEG
        pb1, pb2, pi1, pi2 = b1[...], b2[...], i1[...], i2[...]
        gt1 = r > pb1
        gt2 = r > pb2
        b2[...] = jnp.where(gt1, pb1, jnp.where(gt2, r, pb2))
        i2[...] = jnp.where(gt1, pi1, jnp.where(gt2, idx, pi2))
        b1[...] = jnp.where(gt1, r, pb1)
        i1[...] = jnp.where(gt1, idx, pi1)

    def step(s):
        row = lax.broadcasted_iota(I32, (L, L), 0)
        col = lax.broadcasted_iota(I32, (L, L), 1)
        mask = (row < MEM) | (row >= col)
        finish_segment(jnp.maximum(s - 1, 0), s > 0)
        hs = jnp.concatenate([mem[...], xn[s]], axis=0).astype(BF)

        def qkv(t):
            return [jnp.concatenate([_dot(hs, w_tile(m * H + t)),
                                     ex[s, :, (m * H + t) * DH:(m * H + t + 1) * DH]], axis=0)
                    for m in range(3)]

        def probs(q, k):
            sc = jnp.where(mask, _dot_t(q, k), NEG)
            p = jnp.exp2((sc - jnp.max(sc, axis=-1, keepdims=True)) * C2)
            return p, jnp.sum(p, axis=-1, keepdims=True)

        def mix(p, l, v):
            r = pl.reciprocal(l, approx=True)
            r = r * (2.0 - l * r)
            return _dot(p, v) * r

        def project_out(o, t, acc):
            y = _dot(o, pltpu.bitcast(wop[t * (DH // 2):(t + 1) * (DH // 2), :], BF))
            return y if acc is None else acc + y

        proj, pr, mixed = {}, {}, {}
        acc, nxt = None, 0
        for t in range(H + D1 + D2):
            if t < H:
                proj[t] = qkv(t)
            if 0 <= t - D1 < H:
                pr[t - D1] = probs(proj[t - D1][0], proj[t - D1][1])
            u = t - D1 - D2
            if 0 <= u < H:
                mixed[u] = mix(pr[u][0], pr[u][1], proj[u][2])
            if t >= H:
                for _ in range(OTAIL):
                    if nxt <= u - D3:
                        acc = project_out(mixed[nxt], nxt, acc)
                        nxt += 1
        while nxt < H:
            acc = project_out(mixed[nxt], nxt, acc)
            nxt += 1
        mem[...] = acc[0:MEM]
        ybuf[...] = acc[MEM:]

    def out_copy(first, count, j):
        return pltpu.make_async_copy(obuf.at[pl.ds(first, count)], out_hbm.at[pl.ds(first, count)],
                                     sem_out.at[j])

    def block(it, carry):
        for k in range(UNROLL):
            step(it * UNROLL + k)

        @pl.when(it == 0)
        def _():
            out_copy(0, UNROLL - 1, 0).start()

        @pl.when(it > 0)
        def _():
            out_copy(it * UNROLL - 1, UNROLL, it).start()

        return carry

    nblk = NSEG // UNROLL
    lax.fori_loop(0, nblk, block, 0)

    finish_segment(NSEG - 1, None)
    out_copy(NSEG - 1, 1, nblk).start()

    big = jnp.int32(2 ** 30)
    c1, j1, c2, j2 = b1[...], i1[...], b2[...], i2[...]
    r1 = jnp.max(c1, axis=0, keepdims=True)
    k1 = jnp.min(jnp.where(c1 == r1, j1, big), axis=0, keepdims=True)
    won = j1 == k1
    c3 = jnp.where(won, c2, c1)
    j3 = jnp.where(won, j2, j1)
    r2 = jnp.max(c3, axis=0, keepdims=True)
    k2 = jnp.min(jnp.where(c3 == r2, j3, big), axis=0, keepdims=True)
    n1 = jnp.clip(k1[0, 0], 0, NSEG * SEG - 1)
    n2 = jnp.clip(k2[0, 0], 0, NSEG * SEG - 1)
    s1, s2 = n1 // SEG, n2 // SEG
    sub = lax.broadcasted_iota(I32, (8, 1), 0)
    xsel = jnp.where(sub == 0, hnbuf[s1, pl.ds(n1 % SEG, 1), :],
                     jnp.where(sub == 1, hnbuf[s2, pl.ds(n2 % SEG, 1), :], 0.0))
    wg_copy.wait()
    wu_copy.wait()
    wd_copy.wait()
    g = _rb(_dot(xsel, wg[...]))
    g = _rb(g * jax.nn.sigmoid(g))
    u = _rb(_dot(xsel, wu[...]))
    y = _rb(_dot(_rb(g * u), wd[...]))
    gate = _rb(jax.nn.sigmoid(jnp.where(sub == 0, r1, r2)))
    y = _rb(y * gate)

    out_copy(0, UNROLL - 1, 0).wait()
    for j in range(1, nblk):
        out_copy(j * UNROLL - 1, UNROLL, j).wait()
    out_copy(NSEG - 1, 1, nblk).wait()

    def patch(s):
        idx = lax.broadcasted_iota(I32, (SEG, 1), 0) + s * SEG
        upd = jnp.where(idx == n1, y[0:1], jnp.where(idx == n2, y[1:2], 0.0))
        obuf[s] = (hbuf[s] + _rb(hnbuf[s] + upd)).astype(BF)

    patch(s1)
    patch(s2)
    out_copy(s1, 1, 0).start()

    @pl.when(s2 != s1)
    def _():
        out_copy(s2, 1, 1).start()
        out_copy(s2, 1, 1).wait()

    out_copy(s1, 1, 0).wait()


@functools.partial(jax.jit, static_argnames=("A_seg_len",))
def pallas_sequential_preLN__memory_aug_recurrent_mem_tr__moe_arch_mod__prompt_kernel(
    A_x, A_mem0, A_Wq, A_Wk, A_Wv, A_Wo, A_seg_len, B_x, B_w_r, B_w_gate, B_w_up, B_w_down,
):
    del B_x
    assert A_seg_len == SEG and A_x.shape == (1, NSEG * SEG, DM) and A_mem0.shape == (1, MEM, DM)
    assert A_Wq.shape == (DM, H, DH) and A_Wo.shape == (H, DH, DM) and B_w_gate.shape == (DM, DFF)
    vmem = pltpu.VMEM
    out = pl.pallas_call(
        _kernel,
        out_shape=jax.ShapeDtypeStruct((NSEG, SEG, DM), BF),
        in_specs=[pl.BlockSpec(memory_space=pl.ANY)] * 10,
        out_specs=pl.BlockSpec(memory_space=pl.ANY),
        scratch_shapes=[
            vmem((NSEG, SEG, DM), BF),
            vmem((MEM, DM), BF),
            vmem((1, DM), BF),
            vmem((NCH, DM, GH, DH), BF),
            vmem((H * DH, DM), BF),
            vmem((DM, DFF), BF),
            vmem((DM, DFF), BF),
            vmem((DFF, DM), BF),
            vmem((3 * H * DM // 2, DH), U32),
            vmem((H * DH // 2, DM), U32),
            vmem((NSEG, XR, 3 * H * DH), F32),
            vmem((NSEG * XR, DM), BF),
            vmem((NSEG, XS, DM), F32),
            vmem((MEM, DM), F32),
            vmem((SEG, DM), F32),
            vmem((NSEG, SEG, DM), F32),
            vmem((NSEG, SEG, DM), F32),
            vmem((NSEG, SEG, DM), BF),
            vmem((SEG, 1), F32),
            vmem((SEG, 1), I32),
            vmem((SEG, 1), F32),
            vmem((SEG, 1), I32),
            pltpu.SemaphoreType.DMA((NCH,)),
            pltpu.SemaphoreType.DMA((4,)),
            pltpu.SemaphoreType.DMA((7,)),
            pltpu.SemaphoreType.DMA((NSEG // UNROLL + 1,)),
        ],
        compiler_params=pltpu.CompilerParams(vmem_limit_bytes=110 * 1024 * 1024),
    )(
        A_x.reshape(NSEG, SEG, DM), A_mem0.reshape(MEM, DM), A_Wq, A_Wk, A_Wv,
        A_Wo.reshape(H * DH, DM), B_w_r.reshape(1, DM), B_w_gate, B_w_up, B_w_down,
    )
    return out.reshape(1, NSEG * SEG, DM)
```

```python
import functools
import math

import jax
import jax.numpy as jnp
from jax import lax
import jax.experimental.pallas as pl
import jax.experimental.pallas.tpu as pltpu

BF = jnp.bfloat16
F32 = jnp.float32
U32 = jnp.uint32
I32 = jnp.int32

H, DH, DM, MEM, SEG, NSEG, DFF = 32, 128, 512, 8, 32, 64, 1792
L = MEM + SEG
XR = 8
XS = SEG - XR
GH = 8
NCH = 3 * H // GH
NCB = DM // DH
UNROLL = 8
FILL = 1
D1, D2, D3, OTAIL = 3, 4, 1, 3
TOK = 1
NEARLY = 7
NA = 4
QM = 0
OUTLOOP = 1
QBF = 1
PBF = 0
S0, S1, S2, SDUE = 0, 1, 2, 2
NV = 1
DV = 3
PD = 2
ORDER = 0
SIDE = 7
SCOPES = 0
EPS = 1e-5
SCALE = 0.08837890625
C2 = SCALE * math.log2(math.e)
NEG = -1e9 / SCALE


def _dot(a, b):
    return lax.dot_general(a, b, (((1,), (0,)), ((), ())), preferred_element_type=F32)


def _dot_t(a, b):
    return lax.dot_general(a, b, (((1,), (1,)), ((), ())), preferred_element_type=F32)


def _rb(x):
    return x.astype(BF).astype(F32)


def _layernorm(x):
    n = x.shape[-1]
    mean = jnp.sum(x, axis=-1, keepdims=True) * (1.0 / n)
    xc = x - mean
    var = jnp.sum(xc * xc, axis=-1, keepdims=True) * (1.0 / n)
    den = _rb(jnp.sqrt(_rb(_rb(var) + EPS)))
    return _rb(_rb(x - _rb(mean)) * (1.0 / den))


def _recip(l):
    r = pl.reciprocal(l, approx=True)
    return r * (2.0 - l * r)


def _tree(f, xs):
    while len(xs) > 1:
        xs = [f(xs[a], xs[a + 1]) if a + 1 < len(xs) else xs[a] for a in range(0, len(xs), 2)]
    return xs[0]


class _NoScope:
    def __enter__(self):
        return self

    def __exit__(self, *a):
        return False


def _scope(name):
    return jax.named_scope(name) if SCOPES else _NoScope()


def _kernel(x_hbm, m0_hbm, wq_hbm, wk_hbm, wv_hbm, wo_hbm, wr_hbm, wg_hbm, wu_hbm, wd_hbm,
            out_hbm,
            xs, m0s, wrs, stage, wo, wg, wu, wd,
            wp, ex, xe, xn, mem, ybuf, hh, obuf, top, st,
            sem_w, sem_x, sem_out):
    w_hbm = tuple(w.bitcast(U32) for w in (wq_hbm, wk_hbm, wv_hbm))
    nfill = 8 * XR if FILL else 0
    npro = NSEG * XR - nfill

    def w_start(c):
        for hp in range(GH // 2):
            for t in range(2):
                pltpu.make_async_copy(w_hbm[c // 4].at[:, t, (c % 4) * (GH // 2) + hp, :],
                                      stage.at[c, hp, t], sem_w.at[c]).start()

    def w_wait(c):
        pltpu.make_async_copy(stage.at[c], stage.at[c], sem_w.at[c]).wait()

    def wo_copy(j):
        rows = pl.ds(j * (H * DH // 4), H * DH // 4)
        return pltpu.make_async_copy(wo_hbm.bitcast(U32).at[rows], wo.at[rows], sem_x.at[10 + j])


    half = NSEG // 2

    def x_copy(j):
        return pltpu.make_async_copy(x_hbm.at[pl.ds(j * half, half), pl.ds(XS, XR), :],
                                     xs.at[pl.ds(j * half, half), pl.ds(XS, XR), :], sem_x.at[8 + j])

    def xr_copy(j):
        return pltpu.make_async_copy(x_hbm.at[pl.ds(j * half, half), pl.ds(0, XS), :],
                                     xs.at[pl.ds(j * half, half), pl.ds(0, XS), :], sem_x.at[12 + j])

    m0_copy = pltpu.make_async_copy(m0_hbm, m0s, sem_x.at[2])
    wr_copy = pltpu.make_async_copy(wr_hbm, wrs, sem_x.at[3])
    wg_copy = pltpu.make_async_copy(wg_hbm, wg, sem_x.at[4])
    wu_copy = pltpu.make_async_copy(wu_hbm, wu, sem_x.at[5])
    wd_copy = pltpu.make_async_copy(wd_hbm, wd, sem_x.at[6])

    def repack(c, hp):
        a = stage[c, hp, 0]
        b = stage[c, hp, 1]
        wp[c, 2 * hp] = (a & jnp.uint32(0xFFFF)) | (b << 16)
        wp[c, 2 * hp + 1] = (a >> 16) | (b & jnp.uint32(0xFFFF0000))

    def w_tile(c, k):
        return pltpu.bitcast(wp[c, k], BF)

    def project_extra(c, k, r0, n):
        lhs = pltpu.bitcast(xe[r0 // 2:(r0 + n) // 2, :], BF)
        ex[c, k, r0:r0 + n, :] = _dot(lhs, w_tile(c, k))

    def ln_extra(g0, g1):
        for g in range(g0, g1):
            v = xs[g * 4:(g + 1) * 4, XS:SEG, :].astype(F32).reshape(4 * XR, DM)
            xe[g * 2 * XR:(g + 1) * 2 * XR, :] = pltpu.bitcast(_layernorm(v).astype(BF), U32)

    def start_late(j, carry):
        xr_copy(j).start()
        wo_copy(j).start()
        return carry

    def start_x(j, carry):
        x_copy(j).start()
        return carry

    lax.fori_loop(0, 2, start_x, 0)
    w_start(0)
    with _scope("wait_xa"):
        x_copy(0).wait()
    w_start(1)
    with _scope("ln_xa"):
        ln_extra(0, NSEG // 8)
    with _scope("wait_xb"):
        x_copy(1).wait()
    for c in range(2, NEARLY):
        w_start(c)
    with _scope("ln_xb"):
        ln_extra(NSEG // 8, NSEG // 4)

    def pro_part(c, carry):
        with _scope("pw"):
            w_wait(c)
        with _scope("part"):
            repack(c, 0)
            for k in range(GH):
                project_extra(c, k, 0, npro)
                if k % 2 == 0 and k + 2 < GH:
                    repack(c, k // 2 + 1)
        return carry

    with _scope("pro"):
        lax.fori_loop(0, NA, pro_part, 0)
        for c in range(NEARLY, NCH):
            w_start(c)
        m0_copy.start()
        wr_copy.start()
        lax.fori_loop(0, 2, start_late, 0)
        lax.fori_loop(NA, NCH, pro_part, 0)
    for cp in (wg_copy, wu_copy, wd_copy):
        cp.start()

    for j in range(2):
        xr_copy(j).wait()
        wo_copy(j).wait()
    m0_copy.wait()
    wr_copy.wait()
    mem[...] = m0s[...].astype(F32)
    xn[...] = _layernorm(xs[0, 0:XS, :].astype(F32))
    ybuf[...] = jnp.zeros((SEG, DM), F32)
    rows = lax.broadcasted_iota(I32, (SEG, 1), 0).astype(F32)
    top[0] = jnp.full((SEG, 1), -jnp.inf, F32)
    top[1] = rows
    top[2] = jnp.full((SEG, 1), -jnp.inf, F32)
    top[3] = rows + SEG

    def finish_rows(s, y, r0, n, live):
        h = _rb(xs[s, r0:r0 + n, :].astype(F32) + _rb(y))
        hn = _layernorm(h)
        hh[s, r0:r0 + n, :] = h
        hh[s, SEG + r0:SEG + r0 + n, :] = hn
        obuf[s, r0:r0 + n, :] = (h + hn).astype(BF)
        r = _rb(jnp.sum(hn * wrs[...].astype(F32), axis=-1, keepdims=True))
        if live is not None:
            r = jnp.where(live, r, -jnp.inf)
        idx = (lax.broadcasted_iota(I32, (n, 1), 0) + (s * SEG + r0)).astype(F32)
        b1, i1, b2, i2 = (top[j, r0:r0 + n, :] for j in range(4))
        gt1 = r > b1
        gt2 = r > b2
        top[0, r0:r0 + n, :] = jnp.where(gt1, r, b1)
        top[1, r0:r0 + n, :] = jnp.where(gt1, idx, i1)
        top[2, r0:r0 + n, :] = jnp.where(gt1, b1, jnp.where(gt2, r, b2))
        top[3, r0:r0 + n, :] = jnp.where(gt1, i1, jnp.where(gt2, idx, i2))

    def step(it, k):
        s = it * UNROLL + k
        row = lax.broadcasted_iota(I32, (L, L), 0)
        col = lax.broadcasted_iota(I32, (L, L), 1)
        mask = (row < MEM) | (row >= col)
        hs = jnp.concatenate([mem[...], xn[...]], axis=0).astype(BF)
        prev = jnp.maximum(s - 1, 0)
        yprev = ybuf[...]
        never = s < 0
        zero = jnp.minimum(s, 0)
        e0 = pl.multiple_of(it * (UNROLL * XR), UNROLL * XR) + k * XR

        def side_work(j):
            if j < 2:
                finish_rows(prev, yprev[16 * j:16 * j + 16], 16 * j, 16, s > 0)
                if not TOK:
                    return None
                z8 = pl.multiple_of(zero, 8)
                z16 = pl.multiple_of(zero, 16)
                t = hh[prev, pl.ds(z8, 8), 0:DH] + top[0, pl.ds(z8, 8), :]
                return t + obuf[prev, pl.ds(z16, 16), 0:DH].astype(F32)[0:8]
            xn[...] = _layernorm(xs[jnp.minimum(s + 1, NSEG - 1), 0:XS, :].astype(F32))
            if not TOK:
                return None
            return xn[pl.ds(pl.multiple_of(zero, 8), 8), 0:DH]

        side_at = {S0: 0, S1: 1, S2: 2}
        due = {}

        sub = lax.broadcasted_iota(I32, (8, 1), 0)
        groups = [0] + list(range(1 + NV, L // 8))

        def full(t, m):
            return QM and m == 0 and t % QM == QM - 1

        if QM:
            xl = pltpu.bitcast(xe[pl.ds(pl.multiple_of((s // 2) * 8, 8), 8), :], BF).astype(F32)
            xl = jnp.where(s % 2 == 0, xl[0:8], xl[8:16])
            h40 = jnp.concatenate([mem[...], xn[...], xl], axis=0)

        def project(t, m):
            c, kk = divmod(m * H + t, GH)
            if full(t, m):
                st[t, m] = _dot(h40, w_tile(c, kk))
            else:
                st[t, m, 0:MEM + XS] = _dot(hs, w_tile(c, kk))

        def rows(t, m, gs):
            c, kk = divmod(m * H + t, GH)
            return [ex[c, kk, pl.ds(e0, XR), :] if g == L // 8 - 1 and not full(t, m)
                    else st[t, m, 8 * g:8 * g + 8, :] for g in gs]

        def probs(t):
            q = rows(t, 0, groups)
            if due.get(t) is not None:
                q[-1] = jnp.where(never, due[t], q[-1])
            kk = jnp.concatenate(rows(t, 1, range(L // 8)), axis=0)
            mk = jnp.concatenate([mask[8 * g:8 * g + 8] for g in groups], axis=0)
            qq = jnp.concatenate(q, axis=0)
            sc = jnp.where(mk, _dot_t(qq.astype(BF) if QBF else qq, kk), NEG)
            p = jnp.exp2((sc - jnp.max(sc, axis=-1, keepdims=True)) * C2)
            return p, jnp.sum(p, axis=-1, keepdims=True)

        def first_rows(t):
            q = rows(t, 0, [1])[0] * C2
            sc = []
            for j in range(MEM + 8):
                sj = jnp.sum(q * st[t, 1, pl.ds(j, 8, stride=0), :], axis=-1, keepdims=True)
                sc.append(jnp.where(sub >= j - MEM, sj, NEG * C2) if j > MEM else sj)
            mx = _tree(jnp.maximum, sc)
            p = [jnp.exp2(sj - mx) for sj in sc]
            o = _tree(jnp.add, [p[j] * st[t, 2, pl.ds(j, 8, stride=0), :] for j in range(MEM + 8)])
            return o * _recip(_tree(jnp.add, p))

        def mix(t):
            p, l = pr[t]
            v = rows(t, 2, range(L // 8))
            if NV and t - PD >= 0:
                v[0] = jnp.where(never, first[t - PD], v[0])
            o = _dot(p.astype(BF) if PBF else p, jnp.concatenate(v, axis=0)) * _recip(l)
            return jnp.concatenate([o[0:MEM], first[t], o[MEM:]], axis=0) if NV else o

        def project_out(o, t, acc):
            y = _dot(o, pltpu.bitcast(wo[t * (DH // 2):(t + 1) * (DH // 2), :], BF))
            return y if acc is None else acc + y

        pr, first, mixed = {}, {}, {}
        acc, nxt = None, 0
        for t in range(H + D1 + D2):
            u = t - D1 - D2
            for ch in ("kvqspx", "qkvsxp", "kqsvpx")[ORDER]:
                if ch in "qkv":
                    if t < H:
                        project(t, "qkv".index(ch))
                elif ch == "s":
                    if t in side_at and (SIDE >> side_at[t]) & 1:
                        due[t + SDUE] = side_work(side_at[t])
                    if 0 <= t - D1 < H:
                        pr[t - D1] = probs(t - D1)
                elif ch == "x":
                    if NV and 0 <= t - DV < H:
                        first[t - DV] = first_rows(t - DV)
                elif 0 <= u < H:
                    if NV and u not in first:
                        first[u] = first_rows(u)
                    mixed[u] = mix(u)
            if t >= H:
                for _ in range(OTAIL):
                    if nxt <= u - D3:
                        acc = project_out(mixed[nxt], nxt, acc)
                        nxt += 1
        while nxt < H:
            acc = project_out(mixed[nxt], nxt, acc)
            nxt += 1
        mem[...] = acc[0:MEM]
        ybuf[...] = acc[MEM:]

    def fill(it, k):
        s = it * UNROLL + k
        slot = jnp.minimum(s // GH, NCH // 2 - 1)
        for par in range(2):
            project_extra(2 * slot + par, k if UNROLL == GH else s % GH, npro, nfill)

    def out_copy(first, count, j):
        return pltpu.make_async_copy(obuf.at[pl.ds(first, count)], out_hbm.at[pl.ds(first, count)],
                                     sem_out.at[j])

    def block(it, carry):
        with _scope("blk"):
            for k in range(UNROLL):
                if FILL:
                    fill(it, k)
                step(it, k)

        if OUTLOOP:
            @pl.when(it == 0)
            def _():
                out_copy(0, UNROLL - 1, 0).start()

            @pl.when(it > 0)
            def _():
                out_copy(it * UNROLL - 1, UNROLL, it).start()

        return carry

    nblk = NSEG // UNROLL
    lax.fori_loop(0, nblk, block, 0)

    if not OUTLOOP:
        out_copy(0, NSEG - 1, 0).start()
    finish_rows(NSEG - 1, ybuf[...], 0, SEG, None)
    out_copy(NSEG - 1, 1, nblk).start()

    big = float(2 ** 24)
    c1, j1, c2, j2 = top[0], top[1], top[2], top[3]
    r1 = jnp.max(c1, axis=0, keepdims=True)
    k1 = jnp.min(jnp.where(c1 == r1, j1, big), axis=0, keepdims=True)
    won = j1 == k1
    c3 = jnp.where(won, c2, c1)
    j3 = jnp.where(won, j2, j1)
    r2 = jnp.max(c3, axis=0, keepdims=True)
    k2 = jnp.min(jnp.where(c3 == r2, j3, big), axis=0, keepdims=True)
    n1 = jnp.clip(k1.astype(I32)[0, 0], 0, NSEG * SEG - 1)
    n2 = jnp.clip(k2.astype(I32)[0, 0], 0, NSEG * SEG - 1)
    s1, s2 = n1 // SEG, n2 // SEG
    sub = lax.broadcasted_iota(I32, (8, 1), 0)
    xsel = jnp.where(sub == 0, hh[s1, pl.ds(SEG + n1 % SEG, 1), :],
                     jnp.where(sub == 1, hh[s2, pl.ds(SEG + n2 % SEG, 1), :], 0.0))
    wg_copy.wait()
    wu_copy.wait()
    wd_copy.wait()
    g = _rb(_dot(xsel, wg[...]))
    g = _rb(g * jax.nn.sigmoid(g))
    u = _rb(_dot(xsel, wu[...]))
    y = _rb(_dot(_rb(g * u), wd[...]))
    gate = _rb(jax.nn.sigmoid(jnp.where(sub == 0, r1, r2)))
    y = _rb(y * gate)

    if OUTLOOP:
        out_copy(0, UNROLL - 1, 0).wait()
        for j in range(1, nblk):
            out_copy(j * UNROLL - 1, UNROLL, j).wait()
    else:
        out_copy(0, NSEG - 1, 0).wait()
    out_copy(NSEG - 1, 1, nblk).wait()

    def patch(s):
        idx = lax.broadcasted_iota(I32, (SEG, 1), 0) + s * SEG
        upd = jnp.where(idx == n1, y[0:1], jnp.where(idx == n2, y[1:2], 0.0))
        obuf[s] = (hh[s, 0:SEG, :] + _rb(hh[s, SEG:2 * SEG, :] + upd)).astype(BF)

    patch(s1)
    patch(s2)
    out_copy(s1, 1, 0).start()

    @pl.when(s2 != s1)
    def _():
        out_copy(s2, 1, 1).start()
        out_copy(s2, 1, 1).wait()

    out_copy(s1, 1, 0).wait()


@functools.partial(jax.jit, static_argnames=("A_seg_len",))
def pallas_sequential_preLN__memory_aug_recurrent_mem_tr__moe_arch_mod__prompt_kernel(
    A_x, A_mem0, A_Wq, A_Wk, A_Wv, A_Wo, A_seg_len, B_x, B_w_r, B_w_gate, B_w_up, B_w_down,
):
    del B_x
    assert A_seg_len == SEG and A_x.shape == (1, NSEG * SEG, DM) and A_mem0.shape == (1, MEM, DM)
    assert A_Wq.shape == (DM, H, DH) and A_Wo.shape == (H, DH, DM) and B_w_gate.shape == (DM, DFF)
    vmem = pltpu.VMEM
    out = pl.pallas_call(
        _kernel,
        out_shape=jax.ShapeDtypeStruct((NSEG, SEG, DM), BF),
        in_specs=[pl.BlockSpec(memory_space=pl.ANY)] * 10,
        out_specs=pl.BlockSpec(memory_space=pl.ANY),
        scratch_shapes=[
            vmem((NSEG, SEG, DM), BF),
            vmem((MEM, DM), BF),
            vmem((DM,), BF),
            vmem((NCH, GH // 2, 2, DM // 2, DH), U32),
            vmem((H * DH // 2, DM), U32),
            vmem((DM, DFF), BF),
            vmem((DM, DFF), BF),
            vmem((DFF, DM), BF),
            vmem((NCH, GH, DM // 2, DH), U32),
            vmem((NCH, GH, NSEG * XR, DH), F32),
            vmem((NSEG * XR // 2, DM), U32),
            vmem((XS, DM), F32),
            vmem((MEM, DM), F32),
            vmem((SEG, DM), F32),
            vmem((NSEG, 2 * SEG, DM), F32),
            vmem((NSEG, SEG, DM), BF),
            vmem((4, SEG, 1), F32),
            vmem((H, 3, L, DH), F32),
            pltpu.SemaphoreType.DMA((NCH,)),
            pltpu.SemaphoreType.DMA((14,)),
            pltpu.SemaphoreType.DMA((NSEG // UNROLL + 1,)),
        ],
        compiler_params=pltpu.CompilerParams(vmem_limit_bytes=110 * 1024 * 1024),
    )(
        A_x.reshape(NSEG, SEG, DM), A_mem0.reshape(MEM, DM),
        *(w.reshape(DM // 2, 2, H, DH) for w in (A_Wq, A_Wk, A_Wv)),
        A_Wo.reshape(H * DH, DM), B_w_r, B_w_gate, B_w_up, B_w_down,
    )
    return out.reshape(1, NSEG * SEG, DM)
```

```python
import functools
import math

import jax
import jax.numpy as jnp
from jax import lax
import jax.experimental.pallas as pl
import jax.experimental.pallas.tpu as pltpu

BF = jnp.bfloat16
F32 = jnp.float32
U32 = jnp.uint32
I32 = jnp.int32

H, DH, DM, MEM, SEG, NSEG, DFF = 32, 128, 512, 8, 32, 64, 1792
L = MEM + SEG
XR = 8
XS = SEG - XR
GH = 8
NCH = 3 * H // GH
NCB = DM // DH
UNROLL = 8
FILL = 1
D1, D2, D3, OTAIL = 3, 4, 1, 3
TOK = 1
NEARLY = 7
NA = 4
QM = 0
STR = 32
OUTLOOP = 1
QBF = 1
PBF = 0
S0, S1, S2, SDUE = 0, 1, 2, 2
NV = 1
DV = 3
PD = 2
ORDER = 0
SIDE = 7
SCOPES = 0
EPS = 1e-5
SCALE = 0.08837890625
C2 = SCALE * math.log2(math.e)
NEG = -1e9 / SCALE


def _dot(a, b):
    return lax.dot_general(a, b, (((1,), (0,)), ((), ())), preferred_element_type=F32)


def _dot_t(a, b):
    return lax.dot_general(a, b, (((1,), (1,)), ((), ())), preferred_element_type=F32)


def _rb(x):
    return x.astype(BF).astype(F32)


def _layernorm(x):
    n = x.shape[-1]
    mean = jnp.sum(x, axis=-1, keepdims=True) * (1.0 / n)
    xc = x - mean
    var = jnp.sum(xc * xc, axis=-1, keepdims=True) * (1.0 / n)
    den = _rb(jnp.sqrt(_rb(_rb(var) + EPS)))
    return _rb(_rb(x - _rb(mean)) * (1.0 / den))


def _recip(l):
    r = pl.reciprocal(l, approx=True)
    return r * (2.0 - l * r)


def _tree(f, xs):
    while len(xs) > 1:
        xs = [f(xs[a], xs[a + 1]) if a + 1 < len(xs) else xs[a] for a in range(0, len(xs), 2)]
    return xs[0]


class _NoScope:
    def __enter__(self):
        return self

    def __exit__(self, *a):
        return False


def _scope(name):
    return jax.named_scope(name) if SCOPES else _NoScope()


def _kernel(x_hbm, m0_hbm, wq_hbm, wk_hbm, wv_hbm, wo_hbm, wr_hbm, wg_hbm, wu_hbm, wd_hbm,
            out_hbm,
            wp, wo, ex, st, stage, hh, xs, obuf, wg, wu, wd, xe, ybuf, top, xn, mem, m0s, wrs,
            sem_w, sem_x, sem_out):
    w_hbm = tuple(w.bitcast(U32) for w in (wq_hbm, wk_hbm, wv_hbm))
    nfill = 8 * XR if FILL else 0
    npro = NSEG * XR - nfill

    def w_start(c):
        for hp in range(GH // 2):
            for t in range(2):
                pltpu.make_async_copy(w_hbm[c // 4].at[:, t, (c % 4) * (GH // 2) + hp, :],
                                      stage.at[c, hp, t], sem_w.at[c]).start()

    def w_wait(c):
        pltpu.make_async_copy(stage.at[c], stage.at[c], sem_w.at[c]).wait()

    def wo_copy(j):
        rows = pl.ds(j * (H * DH // 4), H * DH // 4)
        return pltpu.make_async_copy(wo_hbm.bitcast(U32).at[rows], wo.at[rows], sem_x.at[10 + j])


    half = NSEG // 2

    def x_copy(j):
        return pltpu.make_async_copy(x_hbm.at[pl.ds(j * half, half), pl.ds(XS, XR), :],
                                     xs.at[pl.ds(j * half, half), pl.ds(XS, XR), :], sem_x.at[8 + j])

    def xr_copy(j):
        return pltpu.make_async_copy(x_hbm.at[pl.ds(j * half, half), pl.ds(0, XS), :],
                                     xs.at[pl.ds(j * half, half), pl.ds(0, XS), :], sem_x.at[12 + j])

    m0_copy = pltpu.make_async_copy(m0_hbm, m0s, sem_x.at[2])
    wr_copy = pltpu.make_async_copy(wr_hbm, wrs, sem_x.at[3])
    wg_copy = pltpu.make_async_copy(wg_hbm, wg, sem_x.at[4])
    wu_copy = pltpu.make_async_copy(wu_hbm, wu, sem_x.at[5])
    wd_copy = pltpu.make_async_copy(wd_hbm, wd, sem_x.at[6])

    def repack(c, hp):
        a = stage[c, hp, 0]
        b = stage[c, hp, 1]
        wp[c, 2 * hp] = (a & jnp.uint32(0xFFFF)) | (b << 16)
        wp[c, 2 * hp + 1] = (a >> 16) | (b & jnp.uint32(0xFFFF0000))

    def w_tile(c, k):
        return pltpu.bitcast(wp[c, k], BF)

    def project_extra(c, k, r0, n):
        lhs = pltpu.bitcast(xe[r0 // 2:(r0 + n) // 2, :], BF)
        ex[r0 // XR:(r0 + n) // XR, c * GH + k] = _dot(lhs, w_tile(c, k)).reshape(n // XR, XR, DH)

    def ln_extra(g0, g1):
        for g in range(g0, g1):
            v = xs[g * 4:(g + 1) * 4, XS:SEG, :].astype(F32).reshape(4 * XR, DM)
            xe[g * 2 * XR:(g + 1) * 2 * XR, :] = pltpu.bitcast(_layernorm(v).astype(BF), U32)

    def start_late(j, carry):
        xr_copy(j).start()
        wo_copy(j).start()
        return carry

    def start_x(j, carry):
        x_copy(j).start()
        return carry

    lax.fori_loop(0, 2, start_x, 0)
    w_start(0)
    with _scope("wait_xa"):
        x_copy(0).wait()
    w_start(1)
    with _scope("ln_xa"):
        ln_extra(0, NSEG // 8)
    with _scope("wait_xb"):
        x_copy(1).wait()
    for c in range(2, NEARLY):
        w_start(c)
    with _scope("ln_xb"):
        ln_extra(NSEG // 8, NSEG // 4)

    def pro_part(c, carry):
        with _scope("pw"):
            w_wait(c)
        with _scope("part"):
            repack(c, 0)
            for k in range(GH):
                project_extra(c, k, 0, npro)
                if k % 2 == 0 and k + 2 < GH:
                    repack(c, k // 2 + 1)
        return carry

    with _scope("pro"):
        lax.fori_loop(0, NA, pro_part, 0)
        for c in range(NEARLY, NCH):
            w_start(c)
        m0_copy.start()
        wr_copy.start()
        lax.fori_loop(0, 2, start_late, 0)
        lax.fori_loop(NA, NCH, pro_part, 0)
    for cp in (wg_copy, wu_copy, wd_copy):
        cp.start()

    for j in range(2):
        xr_copy(j).wait()
        wo_copy(j).wait()
    m0_copy.wait()
    wr_copy.wait()
    mem[...] = m0s[...].astype(F32)
    xn[...] = _layernorm(xs[0, 0:XS, :].astype(F32))
    ybuf[...] = jnp.zeros((SEG, DM), F32)
    rows = lax.broadcasted_iota(I32, (SEG, 1), 0).astype(F32)
    top[0] = jnp.full((SEG, 1), -jnp.inf, F32)
    top[1] = rows
    top[2] = jnp.full((SEG, 1), -jnp.inf, F32)
    top[3] = rows + SEG

    def finish_rows(s, y, r0, n, live):
        h = _rb(xs[s, r0:r0 + n, :].astype(F32) + _rb(y))
        hn = _layernorm(h)
        hh[s, r0:r0 + n, :] = h
        hh[s, SEG + r0:SEG + r0 + n, :] = hn
        obuf[s, r0:r0 + n, :] = (h + hn).astype(BF)
        r = _rb(jnp.sum(hn * wrs[...].astype(F32), axis=-1, keepdims=True))
        if live is not None:
            r = jnp.where(live, r, -jnp.inf)
        idx = (lax.broadcasted_iota(I32, (n, 1), 0) + (s * SEG + r0)).astype(F32)
        b1, i1, b2, i2 = (top[j, r0:r0 + n, :] for j in range(4))
        gt1 = r > b1
        gt2 = r > b2
        top[0, r0:r0 + n, :] = jnp.where(gt1, r, b1)
        top[1, r0:r0 + n, :] = jnp.where(gt1, idx, i1)
        top[2, r0:r0 + n, :] = jnp.where(gt1, b1, jnp.where(gt2, r, b2))
        top[3, r0:r0 + n, :] = jnp.where(gt1, i1, jnp.where(gt2, idx, i2))

    def step(it, k):
        s = it * UNROLL + k
        row = lax.broadcasted_iota(I32, (L, L), 0)
        col = lax.broadcasted_iota(I32, (L, L), 1)
        mask = (row < MEM) | (row >= col)
        hs = jnp.concatenate([mem[...], xn[...]], axis=0).astype(BF)
        s0 = pl.multiple_of(it * UNROLL, UNROLL)
        prev = s0 + (k - 1) if k else jnp.maximum(s - 1, 0)
        succ = s0 + (k + 1) if k + 1 < UNROLL else jnp.minimum(s + 1, NSEG - 1)
        yprev = ybuf[...]
        never = s < 0
        zero = jnp.minimum(s, 0)
        e0 = pl.multiple_of(it * (UNROLL * XR), UNROLL * XR) + k * XR

        def side_work(j):
            if j < 2:
                finish_rows(prev, yprev[16 * j:16 * j + 16], 16 * j, 16, None if k else s > 0)
                if not TOK:
                    return None
                z8 = pl.multiple_of(zero, 8)
                z16 = pl.multiple_of(zero, 16)
                t = hh[prev, pl.ds(z8, 8), 0:DH] + top[0, pl.ds(z8, 8), :]
                return t + obuf[prev, pl.ds(z16, 16), 0:DH].astype(F32)[0:8]
            xn[...] = _layernorm(xs[succ, 0:XS, :].astype(F32))
            if not TOK:
                return None
            return xn[pl.ds(pl.multiple_of(zero, 8), 8), 0:DH]

        side_at = {S0: 0, S1: 1, S2: 2}
        due = {}

        sub = lax.broadcasted_iota(I32, (8, 1), 0)
        groups = [0] + list(range(1 + NV, L // 8))

        def full(t, m):
            return QM and m == 0 and t % QM == QM - 1

        if QM:
            xl = pltpu.bitcast(xe[pl.ds(pl.multiple_of((s // 2) * 8, 8), 8), :], BF).astype(F32)
            xl = jnp.where(s % 2 == 0, xl[0:8], xl[8:16])
            h40 = jnp.concatenate([mem[...], xn[...], xl], axis=0)

        def project(t, m):
            c, kk = divmod(m * H + t, GH)
            if full(t, m):
                st[t, m] = _dot(h40, w_tile(c, kk))
            else:
                st[t, m, 0:MEM + XS] = _dot(hs, w_tile(c, kk))

        def rows(t, m, gs):
            c, kk = divmod(m * H + t, GH)
            return [ex[s, m * H + t] if g == L // 8 - 1 and not full(t, m)
                    else st[t, m, 8 * g:8 * g + 8, :] for g in gs]

        def probs(t):
            q = rows(t, 0, groups)
            if due.get(t) is not None:
                q[-1] = jnp.where(never, due[t], q[-1])
            kk = jnp.concatenate(rows(t, 1, range(L // 8)), axis=0)
            mk = jnp.concatenate([mask[8 * g:8 * g + 8] for g in groups], axis=0)
            qq = jnp.concatenate(q, axis=0)
            sc = jnp.where(mk, _dot_t(qq.astype(BF) if QBF else qq, kk), NEG)
            p = jnp.exp2((sc - jnp.max(sc, axis=-1, keepdims=True)) * C2)
            return p, jnp.sum(p, axis=-1, keepdims=True)

        def first_rows(t):
            q = rows(t, 0, [1])[0] * C2
            sc = []
            for j in range(MEM + 8):
                sj = jnp.sum(q * st[t, 1, pl.ds(j, 8, stride=0), :], axis=-1, keepdims=True)
                sc.append(jnp.where(sub >= j - MEM, sj, NEG * C2) if j > MEM else sj)
            mx = _tree(jnp.maximum, sc)
            p = [jnp.exp2(sj - mx) for sj in sc]
            o = _tree(jnp.add, [p[j] * st[t, 2, pl.ds(j, 8, stride=0), :] for j in range(MEM + 8)])
            return o * _recip(_tree(jnp.add, p))

        def mix(t):
            p, l = pr[t]
            v = rows(t, 2, range(L // 8))
            if NV and t - PD >= 0:
                v[0] = jnp.where(never, first[t - PD], v[0])
            o = _dot(p.astype(BF) if PBF else p, jnp.concatenate(v, axis=0)) * _recip(l)
            return jnp.concatenate([o[0:MEM], first[t], o[MEM:]], axis=0) if NV else o

        def project_out(o, t, acc):
            y = _dot(o, pltpu.bitcast(wo[t * (DH // 2):(t + 1) * (DH // 2), :], BF))
            return y if acc is None else acc + y

        pr, first, mixed = {}, {}, {}
        acc, nxt = None, 0
        for t in range(H + D1 + D2):
            u = t - D1 - D2
            for ch in ("kvqspx", "qkvsxp", "kqsvpx")[ORDER]:
                if ch in "qkv":
                    if t < H:
                        project(t, "qkv".index(ch))
                elif ch == "s":
                    if t in side_at and (SIDE >> side_at[t]) & 1:
                        due[t + SDUE] = side_work(side_at[t])
                    if 0 <= t - D1 < H:
                        pr[t - D1] = probs(t - D1)
                elif ch == "x":
                    if NV and 0 <= t - DV < H:
                        first[t - DV] = first_rows(t - DV)
                elif 0 <= u < H:
                    if NV and u not in first:
                        first[u] = first_rows(u)
                    mixed[u] = mix(u)
            if t >= H:
                for _ in range(OTAIL):
                    if nxt <= u - D3:
                        acc = project_out(mixed[nxt], nxt, acc)
                        nxt += 1
        while nxt < H:
            acc = project_out(mixed[nxt], nxt, acc)
            nxt += 1
        mem[...] = acc[0:MEM]
        ybuf[...] = acc[MEM:]

    def fill(it, k):
        s = it * UNROLL + k
        slot = jnp.minimum(s // GH, NCH // 2 - 1)
        for par in range(2):
            project_extra(2 * slot + par, k if UNROLL == GH else s % GH, npro, nfill)

    def out_copy(first, count, j):
        return pltpu.make_async_copy(obuf.at[pl.ds(first, count)], out_hbm.at[pl.ds(first, count)],
                                     sem_out.at[j])

    def block(it, carry):
        with _scope("blk"):
            for k in range(UNROLL):
                if FILL:
                    fill(it, k)
                step(it, k)

        if OUTLOOP:
            @pl.when(it == 0)
            def _():
                out_copy(0, UNROLL - 1, 0).start()

            @pl.when(it > 0)
            def _():
                out_copy(it * UNROLL - 1, UNROLL, it).start()

        return carry

    nblk = NSEG // UNROLL
    lax.fori_loop(0, nblk, block, 0)

    if not OUTLOOP:
        out_copy(0, NSEG - 1, 0).start()
    finish_rows(NSEG - 1, ybuf[...], 0, SEG, None)
    out_copy(NSEG - 1, 1, nblk).start()

    big = float(2 ** 24)
    c1, j1, c2, j2 = top[0], top[1], top[2], top[3]
    r1 = jnp.max(c1, axis=0, keepdims=True)
    k1 = jnp.min(jnp.where(c1 == r1, j1, big), axis=0, keepdims=True)
    won = j1 == k1
    c3 = jnp.where(won, c2, c1)
    j3 = jnp.where(won, j2, j1)
    r2 = jnp.max(c3, axis=0, keepdims=True)
    k2 = jnp.min(jnp.where(c3 == r2, j3, big), axis=0, keepdims=True)
    n1 = jnp.clip(k1.astype(I32)[0, 0], 0, NSEG * SEG - 1)
    n2 = jnp.clip(k2.astype(I32)[0, 0], 0, NSEG * SEG - 1)
    s1, s2 = n1 // SEG, n2 // SEG
    sub = lax.broadcasted_iota(I32, (8, 1), 0)
    xsel = jnp.where(sub == 0, hh[s1, pl.ds(SEG + n1 % SEG, 1), :],
                     jnp.where(sub == 1, hh[s2, pl.ds(SEG + n2 % SEG, 1), :], 0.0))
    wg_copy.wait()
    wu_copy.wait()
    wd_copy.wait()
    g = _rb(_dot(xsel, wg[...]))
    g = _rb(g * jax.nn.sigmoid(g))
    u = _rb(_dot(xsel, wu[...]))
    y = _rb(_dot(_rb(g * u), wd[...]))
    gate = _rb(jax.nn.sigmoid(jnp.where(sub == 0, r1, r2)))
    y = _rb(y * gate)

    if OUTLOOP:
        out_copy(0, UNROLL - 1, 0).wait()
        for j in range(1, nblk):
            out_copy(j * UNROLL - 1, UNROLL, j).wait()
    else:
        out_copy(0, NSEG - 1, 0).wait()
    out_copy(NSEG - 1, 1, nblk).wait()

    def patch(s):
        idx = lax.broadcasted_iota(I32, (SEG, 1), 0) + s * SEG
        upd = jnp.where(idx == n1, y[0:1], jnp.where(idx == n2, y[1:2], 0.0))
        obuf[s] = (hh[s, 0:SEG, :] + _rb(hh[s, SEG:2 * SEG, :] + upd)).astype(BF)

    patch(s1)
    patch(s2)
    out_copy(s1, 1, 0).start()

    @pl.when(s2 != s1)
    def _():
        out_copy(s2, 1, 1).start()
        out_copy(s2, 1, 1).wait()

    out_copy(s1, 1, 0).wait()


@functools.partial(jax.jit, static_argnames=("A_seg_len",))
def pallas_sequential_preLN__memory_aug_recurrent_mem_tr__moe_arch_mod__prompt_kernel(
    A_x, A_mem0, A_Wq, A_Wk, A_Wv, A_Wo, A_seg_len, B_x, B_w_r, B_w_gate, B_w_up, B_w_down,
):
    del B_x
    assert A_seg_len == SEG and A_x.shape == (1, NSEG * SEG, DM) and A_mem0.shape == (1, MEM, DM)
    assert A_Wq.shape == (DM, H, DH) and A_Wo.shape == (H, DH, DM) and B_w_gate.shape == (DM, DFF)
    vmem = pltpu.VMEM
    out = pl.pallas_call(
        _kernel,
        out_shape=jax.ShapeDtypeStruct((NSEG, SEG, DM), BF),
        in_specs=[pl.BlockSpec(memory_space=pl.ANY)] * 10,
        out_specs=pl.BlockSpec(memory_space=pl.ANY),
        scratch_shapes=[
            vmem((NCH, GH, DM // 2, DH), U32),
            vmem((H * DH // 2, DM), U32),
            vmem((NSEG, 3 * H, XR, DH), F32),
            vmem((H, 3, STR, DH), F32),
            vmem((NCH, GH // 2, 2, DM // 2, DH), U32),
            vmem((NSEG, 2 * SEG, DM), F32),
            vmem((NSEG, SEG, DM), BF),
            vmem((NSEG, SEG, DM), BF),
            vmem((DM, DFF), BF),
            vmem((DM, DFF), BF),
            vmem((DFF, DM), BF),
            vmem((NSEG * XR // 2, DM), U32),
            vmem((SEG, DM), F32),
            vmem((4, SEG, 1), F32),
            vmem((XS, DM), F32),
            vmem((MEM, DM), F32),
            vmem((MEM, DM), BF),
            vmem((DM,), BF),
            pltpu.SemaphoreType.DMA((NCH,)),
            pltpu.SemaphoreType.DMA((14,)),
            pltpu.SemaphoreType.DMA((NSEG // UNROLL + 1,)),
        ],
        compiler_params=pltpu.CompilerParams(vmem_limit_bytes=110 * 1024 * 1024),
    )(
        A_x.reshape(NSEG, SEG, DM), A_mem0.reshape(MEM, DM),
        *(w.reshape(DM // 2, 2, H, DH) for w in (A_Wq, A_Wk, A_Wv)),
        A_Wo.reshape(H * DH, DM), B_w_r, B_w_gate, B_w_up, B_w_down,
    )
    return out.reshape(1, NSEG * SEG, DM)
```

```python
import functools
import math

import jax
import jax.numpy as jnp
from jax import lax
import jax.experimental.pallas as pl
import jax.experimental.pallas.tpu as pltpu

BF = jnp.bfloat16
F32 = jnp.float32
U32 = jnp.uint32
I32 = jnp.int32

H, DH, DM, MEM, SEG, NSEG, DFF = 32, 128, 512, 8, 32, 64, 1792
L = MEM + SEG
XR = 8
XS = SEG - XR
GH = 8
NCH = 3 * H // GH
NCB = DM // DH
UNROLL = 8
FILL = 1
D1, D2, D3, OTAIL = 4, 4, 1, 3
TOK = 1
NEARLY = 7
NFILL = 64
INITFIRST = 0
PAIRB = 1
NA = 4
QM = 0
STR = 32
OUTLOOP = 1
QBF = 0
PBF = 1
S0, S1, S2, SDUE = 0, 1, 2, 2
NV = 1
DV = 2
PD = 4
ORDER = 10
KBF = 0
VBF = 0
NPIN = 0
OSTART = 0
ORDERS = ("kvqspx", "qkvsxp", "kqsvpx", "qkvspx", "kvsqpx", "kpvsqx", "skvpqx", "xkvqsp", "kxvsqp", "vkqpsx", "pkvqsx", "kvxqps")
SIDE = 7
SCOPES = 0
EPS = 1e-5
SCALE = 0.08837890625
C2 = SCALE * math.log2(math.e)
NEG = -1e9 / SCALE


def _dot(a, b):
    return lax.dot_general(a, b, (((1,), (0,)), ((), ())), preferred_element_type=F32)


def _dot_t(a, b):
    return lax.dot_general(a, b, (((1,), (1,)), ((), ())), preferred_element_type=F32)


def _rb(x):
    return x.astype(BF).astype(F32)


def _layernorm(x):
    n = x.shape[-1]
    mean = jnp.sum(x, axis=-1, keepdims=True) * (1.0 / n)
    xc = x - mean
    var = jnp.sum(xc * xc, axis=-1, keepdims=True) * (1.0 / n)
    den = _rb(jnp.sqrt(_rb(_rb(var) + EPS)))
    return _rb(_rb(x - _rb(mean)) * (1.0 / den))


def _layernorm_f32(x):
    n = x.shape[-1]
    xc = x - jnp.sum(x, axis=-1, keepdims=True) * (1.0 / n)
    var = jnp.sum(xc * xc, axis=-1, keepdims=True) * (1.0 / n)
    return xc * lax.rsqrt(var + EPS)


def _recip(l):
    r = pl.reciprocal(l, approx=True)
    return r * (2.0 - l * r)


def _tree(f, xs):
    while len(xs) > 1:
        xs = [f(xs[a], xs[a + 1]) if a + 1 < len(xs) else xs[a] for a in range(0, len(xs), 2)]
    return xs[0]


class _NoScope:
    def __enter__(self):
        return self

    def __exit__(self, *a):
        return False


def _scope(name):
    return jax.named_scope(name) if SCOPES else _NoScope()


def _kernel(x_hbm, m0_hbm, wq_hbm, wk_hbm, wv_hbm, wo_hbm, wr_hbm, wg_hbm, wu_hbm, wd_hbm,
            out_hbm,
            wp, wo, ex, st, stage, hh, xs, obuf, wg, wu, wd, xe, ybuf, top, xn, mem, x0s, m0s, wrs,
            sem_w, sem_x, sem_out):
    w_hbm = tuple(w.bitcast(U32) for w in (wq_hbm, wk_hbm, wv_hbm))
    nfill = NFILL if FILL else 0
    npro = NSEG * XR - nfill

    def w_start(c, hps=range(GH // 2), sem=None):
        for hp in hps:
            for t in range(2):
                pltpu.make_async_copy(w_hbm[c // 4].at[:, t, (c % 4) * (GH // 2) + hp, :],
                                      stage.at[c, hp, t], sem_w.at[c] if sem is None else sem).start()

    def w_wait(c, hp0=0, n=GH // 2, sem=None):
        part = stage.at[c, pl.ds(hp0, n)]
        pltpu.make_async_copy(part, part, sem_w.at[c] if sem is None else sem).wait()

    def wo_copy(j):
        rows = pl.ds(j * (H * DH // 4), H * DH // 4)
        return pltpu.make_async_copy(wo_hbm.bitcast(U32).at[rows], wo.at[rows], sem_x.at[10 + j])


    half = NSEG // 2

    hx = npro // XR // 2

    def x_copy(j):
        return pltpu.make_async_copy(x_hbm.at[pl.ds(j * hx, hx), pl.ds(XS, XR), :],
                                     xs.at[pl.ds(j * hx, hx), pl.ds(XS, XR), :], sem_x.at[8 + j])

    if nfill:
        xc_copy = pltpu.make_async_copy(x_hbm.at[pl.ds(2 * hx, NSEG - 2 * hx), pl.ds(XS, XR), :],
                                        xs.at[pl.ds(2 * hx, NSEG - 2 * hx), pl.ds(XS, XR), :], sem_x.at[7])

    def xr_copy(j):
        return pltpu.make_async_copy(x_hbm.at[pl.ds(j * half, half), pl.ds(0, XS), :],
                                     xs.at[pl.ds(j * half, half), pl.ds(0, XS), :], sem_x.at[12 + j])

    x0_copy = pltpu.make_async_copy(x_hbm.at[0, pl.ds(0, XS), :], x0s, sem_x.at[1])
    m0_copy = pltpu.make_async_copy(m0_hbm, m0s, sem_x.at[2])
    wr_copy = pltpu.make_async_copy(wr_hbm, wrs, sem_x.at[3])
    wg_copy = pltpu.make_async_copy(wg_hbm.bitcast(U32), wg, sem_x.at[4])
    wu_copy = pltpu.make_async_copy(wu_hbm.bitcast(U32), wu, sem_x.at[5])
    wd_copy = pltpu.make_async_copy(wd_hbm.bitcast(U32), wd, sem_x.at[6])

    def repack(c, hp):
        a = stage[c, hp, 0]
        b = stage[c, hp, 1]
        wp[c, 2 * hp] = (a & jnp.uint32(0xFFFF)) | (b << 16)
        wp[c, 2 * hp + 1] = (a >> 16) | (b & jnp.uint32(0xFFFF0000))

    def w_tile(c, k):
        return pltpu.bitcast(wp[c, k], BF)

    def project_extra(c, k, r0, n):
        lhs = xe[r0:r0 + n, :]
        ex[r0 // XR:(r0 + n) // XR, c * GH + k] = _dot(lhs, w_tile(c, k)).reshape(n // XR, XR, DH)

    def ln_extra(s0, n):
        for g in range(s0, s0 + n):
            v = xs[g, XS:SEG, :].astype(F32)
            xe[g * XR:(g + 1) * XR, :] = _layernorm_f32(v)

    def start_late(j, carry):
        xr_copy(j).start()
        wo_copy(j).start()
        return carry

    def start_x(j, carry):
        x_copy(j).start()
        return carry

    lax.fori_loop(0, 2, start_x, 0)
    w_start(0, [0], sem_x.at[0])
    with _scope("wait_xa"):
        x_copy(0).wait()
    w_start(0, [1, 2], sem_x.at[14])
    with _scope("ln_xa"):
        ln_extra(0, hx)
    with _scope("wait_xb"):
        x_copy(1).wait()
    w_start(0, [3])
    for cp in (x0_copy, m0_copy, wr_copy) + ((xc_copy,) if nfill else ()):
        cp.start()
    with _scope("ln_xb"):
        ln_extra(hx, hx)

    def project_pairs(pairs):
        repack(*pairs[0])
        for i, (c, hp) in enumerate(pairs):
            project_extra(c, 2 * hp, 0, npro)
            if i + 1 < len(pairs):
                repack(*pairs[i + 1])
            project_extra(c, 2 * hp + 1, 0, npro)

    def pro_one(c, carry):
        with _scope("pw"):
            w_wait(c)
        with _scope("part"):
            project_pairs([(c, hp) for hp in range(GH // 2)])
        return carry

    def pro_two(i, carry):
        with _scope("pw"):
            w_wait(2 * i)
            w_wait(2 * i + 1)
        with _scope("part"):
            project_pairs([(2 * i + e, hp) for e in range(2) for hp in range(GH // 2)])
        return carry

    def init_state():
        mem[...] = m0s[...].astype(F32)
        xn[...] = _layernorm_f32(x0s[...].astype(F32))
        if nfill:
            ln_extra(2 * hx, NSEG - 2 * hx)
        ybuf[...] = jnp.zeros((SEG, DM), F32)
        rows = lax.broadcasted_iota(I32, (SEG, 1), 0).astype(F32)
        top[0] = jnp.full((SEG, 1), -jnp.inf, F32)
        top[1] = rows
        top[2] = jnp.full((SEG, 1), -jnp.inf, F32)
        top[3] = rows + SEG

    with _scope("pro"):
        with _scope("pw"):
            w_wait(0, 0, 1, sem_x.at[0])
        for c in range(1, NEARLY):
            w_start(c)
        with _scope("p0a"):
            project_pairs([(0, 0)])
        with _scope("pw"):
            w_wait(0, 1, 2, sem_x.at[14])
        with _scope("p0b"):
            project_pairs([(0, 1), (0, 2)])
        with _scope("pw"):
            w_wait(0, 3, 1)
            for cp in (x0_copy, m0_copy, wr_copy) + ((xc_copy,) if nfill else ()):
                cp.wait()
        with _scope("p0c"):
            if INITFIRST:
                init_state()
            project_pairs([(0, 3)])
            if not INITFIRST:
                init_state()
        lax.fori_loop(1, NA, pro_one, 0)
        for c in range(NEARLY, NCH):
            w_start(c)
        lax.fori_loop(0, 2, start_late, 0)
        if PAIRB:
            lax.fori_loop(NA // 2, NCH // 2, pro_two, 0)
        else:
            lax.fori_loop(NA, NCH, pro_one, 0)
    for cp in (wg_copy, wu_copy, wd_copy):
        cp.start()
    for j in range(2):
        xr_copy(j).wait()
        wo_copy(j).wait()

    def finish_rows(s, y, r0, n, live):
        h = _rb(xs[s, r0:r0 + n, :].astype(F32) + _rb(y))
        hn = _layernorm(h)
        hh[s, r0:r0 + n, :] = h
        hh[s, SEG + r0:SEG + r0 + n, :] = hn
        obuf[s, r0:r0 + n, :] = (h + hn).astype(BF)
        r = _rb(jnp.sum(hn * wrs[...].astype(F32), axis=-1, keepdims=True))
        if live is not None:
            r = jnp.where(live, r, -jnp.inf)
        idx = (lax.broadcasted_iota(I32, (n, 1), 0) + (s * SEG + r0)).astype(F32)
        b1, i1, b2, i2 = (top[j, r0:r0 + n, :] for j in range(4))
        gt1 = r > b1
        gt2 = r > b2
        new = (jnp.where(gt1, r, b1), jnp.where(gt1, idx, i1),
               jnp.where(gt1, b1, jnp.where(gt2, r, b2)), jnp.where(gt1, i1, jnp.where(gt2, idx, i2)))
        for j in range(4):
            top[j, r0:r0 + n, :] = new[j]
        return new

    def step(it, k):
        s = it * UNROLL + k
        row = lax.broadcasted_iota(I32, (L, L), 0)
        col = lax.broadcasted_iota(I32, (L, L), 1)
        mask = (row < MEM) | (row >= col)
        hs = jnp.concatenate([mem[...], xn[...]], axis=0).astype(BF)
        s0 = pl.multiple_of(it * UNROLL, UNROLL)
        prev = s0 + (k - 1) if k else jnp.maximum(s - 1, 0)
        succ = s0 + (k + 1) if k + 1 < UNROLL else jnp.minimum(s + 1, NSEG - 1)
        yprev = ybuf[...]
        never = s < 0
        zero = jnp.minimum(s, 0)
        e0 = pl.multiple_of(it * (UNROLL * XR), UNROLL * XR) + k * XR

        def side_work(j):
            if j < 2:
                finish_rows(prev, yprev[16 * j:16 * j + 16], 16 * j, 16, None if k else s > 0)
                if not TOK:
                    return None
                z8 = pl.multiple_of(zero, 8)
                z16 = pl.multiple_of(zero, 16)
                t = hh[prev, pl.ds(z8, 8), 0:DH] + top[0, pl.ds(z8, 8), :]
                return t + obuf[prev, pl.ds(z16, 16), 0:DH].astype(F32)[0:8]
            xn[...] = _layernorm_f32(xs[succ, 0:XS, :].astype(F32))
            if not TOK:
                return None
            return xn[pl.ds(pl.multiple_of(zero, 8), 8), 0:DH]

        side_at = {S0: 0, S1: 1, S2: 2}
        due = {}

        sub = lax.broadcasted_iota(I32, (8, 1), 0)
        groups = [0] + list(range(1 + NV, L // 8))

        def full(t, m):
            return QM and m == 0 and t % QM == QM - 1

        if QM:
            xl = pltpu.bitcast(xe[pl.ds(pl.multiple_of((s // 2) * 8, 8), 8), :], BF).astype(F32)
            xl = jnp.where(s % 2 == 0, xl[0:8], xl[8:16])
            h40 = jnp.concatenate([mem[...], xn[...], xl], axis=0)

        def project(t, m):
            c, kk = divmod(m * H + t, GH)
            if full(t, m):
                st[t, m] = _dot(h40, w_tile(c, kk))
            else:
                st[t, m, 0:MEM + XS] = _dot(hs, w_tile(c, kk))

        def rows(t, m, gs):
            c, kk = divmod(m * H + t, GH)
            return [ex[s, m * H + t] if g == L // 8 - 1 and not full(t, m)
                    else st[t, m, 8 * g:8 * g + 8, :] for g in gs]

        def probs(t):
            q = rows(t, 0, groups)
            if due.get(t) is not None:
                q[-1] = jnp.where(never, due[t], q[-1])
            kk = jnp.concatenate(rows(t, 1, range(L // 8)), axis=0)
            if KBF:
                kk = kk.astype(BF)
            mk = jnp.concatenate([mask[8 * g:8 * g + 8] for g in groups], axis=0)
            qq = jnp.concatenate(q, axis=0)
            sc = jnp.where(mk, _dot_t(qq.astype(BF) if QBF else qq, kk), NEG)
            p = jnp.exp2((sc - jnp.max(sc, axis=-1, keepdims=True)) * C2)
            return p, jnp.sum(p, axis=-1, keepdims=True)

        def first_rows(t):
            q = rows(t, 0, [1])[0] * C2
            kk = rows(t, 1, [0, 1])
            vv = rows(t, 2, [0, 1])

            def row(a, j):
                return jnp.broadcast_to(a[j // 8][j % 8:j % 8 + 1], (8, DH))

            sc = []
            for j in range(MEM + 8):
                sj = jnp.sum(q * row(kk, j), axis=-1, keepdims=True)
                sc.append(jnp.where(sub >= j - MEM, sj, NEG * C2) if j > MEM else sj)
            mx = _tree(jnp.maximum, sc)
            p = [jnp.exp2(sj - mx) for sj in sc]
            o = _tree(jnp.add, [p[j] * row(vv, j) for j in range(MEM + 8)])
            return o * _recip(_tree(jnp.add, p))

        def mix(t):
            p, l = pr[t]
            v = rows(t, 2, range(L // 8))
            if NV and t - PD >= 0:
                v[0] = jnp.where(never, first[t - PD], v[0])
            if NPIN and t - NPIN >= 0:
                v[2] = jnp.where(never, _tree(jnp.add, [mixed[t - NPIN][8 * g:8 * g + 8] for g in groups]), v[2])
            vv = jnp.concatenate(v, axis=0)
            o = _dot(p.astype(BF) if PBF else p, vv.astype(BF) if VBF else vv) * _recip(l)
            return jnp.concatenate([o[0:MEM], first[t], o[MEM:]], axis=0) if NV else o

        def project_out(o, t, acc):
            y = _dot(o, pltpu.bitcast(wo[t * (DH // 2):(t + 1) * (DH // 2), :], BF))
            return y if acc is None else acc + y

        pr, first, mixed = {}, {}, {}
        acc, nxt = None, 0
        for t in range(H + D1 + D2):
            u = t - D1 - D2
            for ch in ORDERS[ORDER]:
                if ch in "qkv":
                    if t < H:
                        project(t, "qkv".index(ch))
                elif ch == "s":
                    if t in side_at and (SIDE >> side_at[t]) & 1:
                        due[t + SDUE] = side_work(side_at[t])
                    if 0 <= t - D1 < H:
                        pr[t - D1] = probs(t - D1)
                elif ch == "x":
                    if NV and 0 <= t - DV < H:
                        first[t - DV] = first_rows(t - DV)
                elif 0 <= u < H:
                    if NV and u not in first:
                        first[u] = first_rows(u)
                    mixed[u] = mix(u)
            if t >= H or nxt < OSTART:
                for _ in range(OTAIL if t >= H else 1):
                    if nxt <= u - D3:
                        acc = project_out(mixed[nxt], nxt, acc)
                        nxt += 1
        while nxt < H:
            acc = project_out(mixed[nxt], nxt, acc)
            nxt += 1
        mem[...] = acc[0:MEM]
        ybuf[...] = acc[MEM:]

    def fill(it, k):
        s = it * UNROLL + k
        slot = jnp.minimum(s // GH, NCH // 2 - 1)
        for par in range(2):
            project_extra(2 * slot + par, k if UNROLL == GH else s % GH, npro, nfill)

    def out_copy(first, count, j):
        return pltpu.make_async_copy(obuf.at[pl.ds(first, count)], out_hbm.at[pl.ds(first, count)],
                                     sem_out.at[j])

    def block(it, carry):
        with _scope("blk"):
            for k in range(UNROLL):
                if FILL:
                    fill(it, k)
                step(it, k)

        if OUTLOOP:
            @pl.when(it == 0)
            def _():
                out_copy(0, UNROLL - 1, 0).start()

            @pl.when(it > 0)
            def _():
                out_copy(it * UNROLL - 1, UNROLL, it).start()

        return carry

    nblk = NSEG // UNROLL
    lax.fori_loop(0, nblk, block, 0)

    if not OUTLOOP:
        out_copy(0, NSEG - 1, 0).start()
    c1, j1, c2, j2 = finish_rows(NSEG - 1, ybuf[...], 0, SEG, None)

    big = float(2 ** 24)
    r1 = jnp.max(c1, axis=0, keepdims=True)
    k1 = jnp.min(jnp.where(c1 == r1, j1, big), axis=0, keepdims=True)
    won = j1 == k1
    c3 = jnp.where(won, c2, c1)
    j3 = jnp.where(won, j2, j1)
    r2 = jnp.max(c3, axis=0, keepdims=True)
    k2 = jnp.min(jnp.where(c3 == r2, j3, big), axis=0, keepdims=True)
    n1 = jnp.clip(k1.astype(I32)[0, 0], 0, NSEG * SEG - 1)
    n2 = jnp.clip(k2.astype(I32)[0, 0], 0, NSEG * SEG - 1)
    s1, s2 = n1 // SEG, n2 // SEG
    sub = lax.broadcasted_iota(I32, (8, 1), 0)
    xsel = jnp.where(sub == 0, hh[s1, pl.ds(SEG + n1 % SEG, 1), :],
                     jnp.where(sub == 1, hh[s2, pl.ds(SEG + n2 % SEG, 1), :], 0.0))
    out_copy(NSEG - 1, 1, nblk).start()
    wg_copy.wait()
    wu_copy.wait()
    wd_copy.wait()
    g = _rb(_dot(xsel, pltpu.bitcast(wg[...], BF)))
    g = _rb(g * jax.nn.sigmoid(g))
    u = _rb(_dot(xsel, pltpu.bitcast(wu[...], BF)))
    y = _rb(_dot(_rb(g * u), pltpu.bitcast(wd[...], BF)))
    gate = _rb(jax.nn.sigmoid(jnp.where(sub == 0, r1, r2)))
    y = _rb(y * gate)

    if OUTLOOP:
        out_copy(0, UNROLL - 1, 0).wait()
        for j in range(1, nblk):
            out_copy(j * UNROLL - 1, UNROLL, j).wait()
    else:
        out_copy(0, NSEG - 1, 0).wait()
    out_copy(NSEG - 1, 1, nblk).wait()

    def patch(s):
        idx = lax.broadcasted_iota(I32, (SEG, 1), 0) + s * SEG
        upd = jnp.where(idx == n1, y[0:1], jnp.where(idx == n2, y[1:2], 0.0))
        obuf[s] = (hh[s, 0:SEG, :] + _rb(hh[s, SEG:2 * SEG, :] + upd)).astype(BF)

    patch(s1)
    patch(s2)
    out_copy(s1, 1, 0).start()

    @pl.when(s2 != s1)
    def _():
        out_copy(s2, 1, 1).start()
        out_copy(s2, 1, 1).wait()

    out_copy(s1, 1, 0).wait()


@functools.partial(jax.jit, static_argnames=("A_seg_len",))
def pallas_sequential_preLN__memory_aug_recurrent_mem_tr__moe_arch_mod__prompt_kernel(
    A_x, A_mem0, A_Wq, A_Wk, A_Wv, A_Wo, A_seg_len, B_x, B_w_r, B_w_gate, B_w_up, B_w_down,
):
    del B_x
    assert A_seg_len == SEG and A_x.shape == (1, NSEG * SEG, DM) and A_mem0.shape == (1, MEM, DM)
    assert A_Wq.shape == (DM, H, DH) and A_Wo.shape == (H, DH, DM) and B_w_gate.shape == (DM, DFF)
    vmem = pltpu.VMEM
    out = pl.pallas_call(
        _kernel,
        out_shape=jax.ShapeDtypeStruct((NSEG, SEG, DM), BF),
        in_specs=[pl.BlockSpec(memory_space=pl.ANY)] * 10,
        out_specs=pl.BlockSpec(memory_space=pl.ANY),
        scratch_shapes=[
            vmem((NCH, GH, DM // 2, DH), U32),
            vmem((H * DH // 2, DM), U32),
            vmem((NSEG, 3 * H, XR, DH), F32),
            vmem((H, 3, STR, DH), F32),
            vmem((NCH, GH // 2, 2, DM // 2, DH), U32),
            vmem((NSEG, 2 * SEG, DM), F32),
            vmem((NSEG, SEG, DM), BF),
            vmem((NSEG, SEG, DM), BF),
            vmem((DM // 2, DFF), U32),
            vmem((DM // 2, DFF), U32),
            vmem((DFF // 2, DM), U32),
            vmem((NSEG * XR, DM), F32),
            vmem((SEG, DM), F32),
            vmem((4, SEG, 1), F32),
            vmem((XS, DM), F32),
            vmem((MEM, DM), F32),
            vmem((XS, DM), BF),
            vmem((MEM, DM), BF),
            vmem((DM,), BF),
            pltpu.SemaphoreType.DMA((NCH,)),
            pltpu.SemaphoreType.DMA((15,)),
            pltpu.SemaphoreType.DMA((NSEG // UNROLL + 1,)),
        ],
        compiler_params=pltpu.CompilerParams(vmem_limit_bytes=110 * 1024 * 1024),
    )(
        A_x.reshape(NSEG, SEG, DM), A_mem0.reshape(MEM, DM),
        *(w.reshape(DM // 2, 2, H, DH) for w in (A_Wq, A_Wk, A_Wv)),
        A_Wo.reshape(H * DH, DM), B_w_r, B_w_gate, B_w_up, B_w_down,
    )
    return out.reshape(1, NSEG * SEG, DM)
```

```python
import functools
import math

import jax
import jax.numpy as jnp
from jax import lax
import jax.experimental.pallas as pl
import jax.experimental.pallas.tpu as pltpu

BF = jnp.bfloat16
F32 = jnp.float32
U32 = jnp.uint32
I32 = jnp.int32

H, DH, DM, MEM, SEG, NSEG, DFF = 32, 128, 512, 8, 32, 64, 1792
L = MEM + SEG
XR = 8
XS = SEG - XR
GH = 8
NCH = 3 * H // GH
NCB = DM // DH
UNROLL = 8
FILL = 1
D1, D2, D3, OTAIL = 4, 4, 1, 3
TOK = 1
NEARLY = 8
FG = 4
FS = 4
INITFIRST = 0
PAIRB = 1
NA = 6
QM = 0
STR = 32
OUTLOOP = 1
QBF = 0
PBF = 1
S0, S1, S2, SDUE = 0, 1, 2, 2
NV = 1
DV = 2
PD = 4
ORDER = 10
KBF = 0
MERGE = 0
XREV = 0
SUMPIN = 0
VBF = 0
NPIN = 0
OSTART = 0
ORDERS = ("kvqspx", "qkvsxp", "kqsvpx", "qkvspx", "kvsqpx", "kpvsqx", "skvpqx", "xkvqsp", "kxvsqp", "vkqpsx", "pkvqsx", "kvxqps")
SIDE = 7
SCOPES = 0
EPS = 1e-5
SCALE = 0.08837890625
C2 = SCALE * math.log2(math.e)
NEG = -1e9 / SCALE


def _dot(a, b):
    return lax.dot_general(a, b, (((1,), (0,)), ((), ())), preferred_element_type=F32)


def _dot_t(a, b):
    return lax.dot_general(a, b, (((1,), (1,)), ((), ())), preferred_element_type=F32)


def _rb(x):
    return x.astype(BF).astype(F32)


def _layernorm(x):
    n = x.shape[-1]
    mean = jnp.sum(x, axis=-1, keepdims=True) * (1.0 / n)
    xc = x - mean
    var = jnp.sum(xc * xc, axis=-1, keepdims=True) * (1.0 / n)
    den = _rb(jnp.sqrt(_rb(_rb(var) + EPS)))
    return _rb(_rb(x - _rb(mean)) * (1.0 / den))


def _layernorm_f32(x):
    n = x.shape[-1]
    xc = x - jnp.sum(x, axis=-1, keepdims=True) * (1.0 / n)
    var = jnp.sum(xc * xc, axis=-1, keepdims=True) * (1.0 / n)
    return xc * lax.rsqrt(var + EPS)


def _recip(l):
    r = pl.reciprocal(l, approx=True)
    return r * (2.0 - l * r)


def _tree(f, xs):
    while len(xs) > 1:
        xs = [f(xs[a], xs[a + 1]) if a + 1 < len(xs) else xs[a] for a in range(0, len(xs), 2)]
    return xs[0]


class _NoScope:
    def __enter__(self):
        return self

    def __exit__(self, *a):
        return False


def _scope(name):
    return jax.named_scope(name) if SCOPES else _NoScope()


def _kernel(x_hbm, m0_hbm, wq_hbm, wk_hbm, wv_hbm, wo_hbm, wr_hbm, wg_hbm, wu_hbm, wd_hbm,
            out_hbm,
            wp, wo, ex, st, stage, hh, xs, obuf, wg, wu, wd, xe, ybuf, top, xn, mem, x0s, m0s, wrs,
            sem_w, sem_x, sem_out):
    w_hbm = tuple(w.bitcast(U32) for w in (wq_hbm, wk_hbm, wv_hbm))
    nfill = 2 * FG * XR
    npro = NSEG * XR - nfill

    def w_start(c, hps=range(GH // 2), sem=None):
        for hp in hps:
            for t in range(2):
                pltpu.make_async_copy(w_hbm[c // 4].at[:, t, (c % 4) * (GH // 2) + hp, :],
                                      stage.at[c, hp, t], sem_w.at[c] if sem is None else sem).start()

    def w_wait(c, hp0=0, n=GH // 2, sem=None):
        part = stage.at[c, pl.ds(hp0, n)]
        pltpu.make_async_copy(part, part, sem_w.at[c] if sem is None else sem).wait()

    def wo_copy(j):
        rows = pl.ds(j * (H * DH // 8), H * DH // 8)
        return pltpu.make_async_copy(wo_hbm.bitcast(U32).at[rows], wo.at[rows], sem_x.at[15 + j])


    half = NSEG // 2

    hx = npro // XR // 2

    def x_copy(j):
        return pltpu.make_async_copy(x_hbm.at[pl.ds(j * hx, hx), pl.ds(XS, XR), :],
                                     xs.at[pl.ds(j * hx, hx), pl.ds(XS, XR), :], sem_x.at[8 + j])

    if nfill:
        xc_copy = pltpu.make_async_copy(x_hbm.at[pl.ds(2 * hx, NSEG - 2 * hx), pl.ds(XS, XR), :],
                                        xs.at[pl.ds(2 * hx, NSEG - 2 * hx), pl.ds(XS, XR), :], sem_x.at[7])

    def xr_copy(j):
        return pltpu.make_async_copy(x_hbm.at[pl.ds(j * half, half), pl.ds(0, XS), :],
                                     xs.at[pl.ds(j * half, half), pl.ds(0, XS), :], sem_x.at[12 + j])

    x0_copy = pltpu.make_async_copy(x_hbm.at[0, pl.ds(0, XS), :], x0s, sem_x.at[1])
    m0_copy = pltpu.make_async_copy(m0_hbm, m0s, sem_x.at[2])
    wr_copy = pltpu.make_async_copy(wr_hbm, wrs, sem_x.at[3])
    wg_copy = pltpu.make_async_copy(wg_hbm.bitcast(U32), wg, sem_x.at[4])
    wu_copy = pltpu.make_async_copy(wu_hbm.bitcast(U32), wu, sem_x.at[5])
    wd_copy = pltpu.make_async_copy(wd_hbm.bitcast(U32), wd, sem_x.at[6])

    def repack(c, hp):
        a = stage[c, hp, 0]
        b = stage[c, hp, 1]
        wp[c * GH + 2 * hp] = (a & jnp.uint32(0xFFFF)) | (b << 16)
        wp[c * GH + 2 * hp + 1] = (a >> 16) | (b & jnp.uint32(0xFFFF0000))

    def w_tile(j):
        return pltpu.bitcast(wp[j], BF)

    def project_extra(j, s0, n):
        r0 = s0 * XR if isinstance(s0, int) else pl.multiple_of(s0 * XR, XR)
        ex[pl.ds(s0, n), j] = _dot(xe[pl.ds(r0, n * XR), :], w_tile(j)).reshape(n, XR, DH)

    def ln_extra(s0, n):
        for g in range(s0, s0 + n):
            v = xs[g, XS:SEG, :].astype(F32)
            xe[g * XR:(g + 1) * XR, :] = _layernorm_f32(v)

    def start_late(j, carry):
        wo_copy(2 + j).start()
        return carry

    def start_x(j, carry):
        x_copy(j).start()
        return carry

    lax.fori_loop(0, 2, start_x, 0)
    w_start(0, [0], sem_x.at[0])
    with _scope("wait_xa"):
        x_copy(0).wait()
    w_start(0, [1, 2], sem_x.at[14])
    with _scope("ln_xa"):
        ln_extra(0, hx)
    with _scope("wait_xb"):
        x_copy(1).wait()
    w_start(0, [3])
    for cp in (x0_copy, m0_copy, wr_copy) + ((xc_copy,) if nfill else ()):
        cp.start()
    with _scope("ln_xb"):
        ln_extra(hx, hx)

    def project_pairs(pairs, n=NSEG - 2 * FG):
        repack(*pairs[0])
        for i, (c, hp) in enumerate(pairs):
            project_extra(c * GH + 2 * hp, 0, n)
            if i + 1 < len(pairs):
                repack(*pairs[i + 1])
            project_extra(c * GH + 2 * hp + 1, 0, n)

    def pro_one(c, carry):
        with _scope("pw"):
            w_wait(c)
        with _scope("part"):
            project_pairs([(c, hp) for hp in range(GH // 2)])
        return carry

    def pro_two(i, carry):
        with _scope("pw"):
            w_wait(2 * i)
            w_wait(2 * i + 1)
        with _scope("part"):
            project_pairs([(2 * i + e, hp) for e in range(2) for hp in range(GH // 2)], NSEG - 3 * FG)
        return carry

    def init_state():
        mem[...] = m0s[...].astype(F32)
        xn[...] = _layernorm_f32(x0s[...].astype(F32))
        if nfill:
            ln_extra(2 * hx, NSEG - 2 * hx)
        ybuf[...] = jnp.zeros((SEG, DM), F32)
        rows = lax.broadcasted_iota(I32, (SEG, 1), 0).astype(F32)
        top[0] = jnp.full((SEG, 1), -jnp.inf, F32)
        top[1] = rows
        top[2] = jnp.full((SEG, 1), -jnp.inf, F32)
        top[3] = rows + SEG

    with _scope("pro"):
        with _scope("pw"):
            w_wait(0, 0, 1, sem_x.at[0])
        for c in range(1, NEARLY):
            w_start(c)
        with _scope("p0a"):
            project_pairs([(0, 0)])
        with _scope("pw"):
            w_wait(0, 1, 2, sem_x.at[14])
        with _scope("p0b"):
            project_pairs([(0, 1), (0, 2)])
        with _scope("pw"):
            w_wait(0, 3, 1)
            for cp in (x0_copy, m0_copy, wr_copy) + ((xc_copy,) if nfill else ()):
                cp.wait()
        for j in range(2):
            xr_copy(j).start()
            wo_copy(j).start()
        with _scope("p0c"):
            if INITFIRST:
                init_state()
            project_pairs([(0, 3)])
            if not INITFIRST:
                init_state()
        lax.fori_loop(1, NA, pro_one, 0)
        for c in range(NEARLY, NCH):
            w_start(c)
        lax.fori_loop(0, 2, start_late, 0)
        if PAIRB:
            lax.fori_loop(NA // 2, NCH // 2, pro_two, 0)
        else:
            lax.fori_loop(NA, NCH, pro_one, 0)
    for cp in (wg_copy, wu_copy, wd_copy):
        cp.start()
    for j in range(2):
        xr_copy(j).wait()
    for j in range(4):
        wo_copy(j).wait()

    def finish_rows(s, y, r0, n, live):
        h = _rb(xs[s, r0:r0 + n, :].astype(F32) + _rb(y))
        hn = _layernorm(h)
        hh[s, r0:r0 + n, :] = h
        hh[s, SEG + r0:SEG + r0 + n, :] = hn
        obuf[s, r0:r0 + n, :] = (h + hn).astype(BF)
        r = _rb(jnp.sum(hn * wrs[...].astype(F32), axis=-1, keepdims=True))
        if live is not None:
            r = jnp.where(live, r, -jnp.inf)
        idx = (lax.broadcasted_iota(I32, (n, 1), 0) + (s * SEG + r0)).astype(F32)
        b1, i1, b2, i2 = (top[j, r0:r0 + n, :] for j in range(4))
        gt1 = r > b1
        gt2 = r > b2
        new = (jnp.where(gt1, r, b1), jnp.where(gt1, idx, i1),
               jnp.where(gt1, b1, jnp.where(gt2, r, b2)), jnp.where(gt1, i1, jnp.where(gt2, idx, i2)))
        for j in range(4):
            top[j, r0:r0 + n, :] = new[j]
        return new

    def step(it, k):
        s = it * UNROLL + k
        row = lax.broadcasted_iota(I32, (L, L), 0)
        col = lax.broadcasted_iota(I32, (L, L), 1)
        mask = (row < MEM) | (row >= col)
        hs = jnp.concatenate([mem[...], xn[...]], axis=0).astype(BF)
        s0 = pl.multiple_of(it * UNROLL, UNROLL)
        prev = s0 + (k - 1) if k else jnp.maximum(s - 1, 0)
        succ = s0 + (k + 1) if k + 1 < UNROLL else jnp.minimum(s + 1, NSEG - 1)
        yprev = ybuf[...]
        never = s < 0
        zero = jnp.minimum(s, 0)
        e0 = pl.multiple_of(it * (UNROLL * XR), UNROLL * XR) + k * XR

        def side_work(j):
            if j < 2:
                finish_rows(prev, yprev[16 * j:16 * j + 16], 16 * j, 16, None if k else s > 0)
                if not TOK:
                    return None
                z8 = pl.multiple_of(zero, 8)
                z16 = pl.multiple_of(zero, 16)
                t = hh[prev, pl.ds(z8, 8), 0:DH] + top[0, pl.ds(z8, 8), :]
                return t + obuf[prev, pl.ds(z16, 16), 0:DH].astype(F32)[0:8]
            xn[...] = _layernorm_f32(xs[succ, 0:XS, :].astype(F32))
            if not TOK:
                return None
            return xn[pl.ds(pl.multiple_of(zero, 8), 8), 0:DH]

        side_at = {S0: 0, S1: 1, S2: 2}
        due = {}

        sub = lax.broadcasted_iota(I32, (8, 1), 0)
        groups = [0] + list(range(1 + NV, L // 8))

        def project(t, m):
            if MERGE:
                if m == 1:
                    ms = (1, 2, 0) if MERGE == 1 else (0, 1, 2)
                    y = _dot(hs, jnp.concatenate([w_tile(a * H + t) for a in ms], axis=1))
                    for i, a in enumerate(ms):
                        st[t, a] = y[:, i * DH:(i + 1) * DH]
                return
            st[t, m] = _dot(hs, w_tile(m * H + t))

        def rows(t, m, gs):
            return [ex[s, m * H + t] if g == L // 8 - 1 else st[t, m, 8 * g:8 * g + 8, :] for g in gs]

        def probs(t):
            q = rows(t, 0, groups)
            if due.get(t) is not None:
                q[-1] = jnp.where(never, due[t], q[-1])
            kk = jnp.concatenate(rows(t, 1, range(L // 8)), axis=0)
            if KBF:
                kk = kk.astype(BF)
            mk = jnp.concatenate([mask[8 * g:8 * g + 8] for g in groups], axis=0)
            qq = jnp.concatenate(q, axis=0)
            sc = jnp.where(mk, _dot_t(qq.astype(BF) if QBF else qq, kk), NEG)
            p = jnp.exp2((sc - jnp.max(sc, axis=-1, keepdims=True)) * C2)
            return p, jnp.sum(p, axis=-1, keepdims=True)

        def first_rows(t):
            q = rows(t, 0, [1])[0] * C2
            kk = rows(t, 1, [0, 1])
            vv = rows(t, 2, [0, 1])

            def row(a, j):
                return jnp.broadcast_to(a[j // 8][j % 8:j % 8 + 1], (8, DH))

            order = list(range(MEM + 8))
            if XREV:
                order = order[::-1]
            sc = {}
            for j in order:
                sj = jnp.sum(q * row(kk, j), axis=-1, keepdims=True)
                sc[j] = jnp.where(sub >= j - MEM, sj, NEG * C2) if j > MEM else sj
            sc = [sc[j] for j in range(MEM + 8)]
            mx = _tree(jnp.maximum, sc)
            p = [jnp.exp2(sj - mx) for sj in sc]
            o = _tree(jnp.add, [p[j] * row(vv, j) for j in range(MEM + 8)])
            return o * _recip(_tree(jnp.add, p))

        def mix(t):
            p, l = pr[t]
            v = rows(t, 2, range(L // 8))
            if NV and t - PD >= 0:
                v[0] = jnp.where(never, first[t - PD], v[0])
            if NPIN and t - NPIN >= 0:
                v[2] = jnp.where(never, _tree(jnp.add, [mixed[t - NPIN][8 * g:8 * g + 8] for g in groups]), v[2])
            if SUMPIN and t - SUMPIN >= 0:
                ls = pr[t - SUMPIN][1]
                v[3] = jnp.where(never, _tree(jnp.add, [ls[8 * g:8 * g + 8] for g in range(len(groups))]), v[3])
            vv = jnp.concatenate(v, axis=0)
            o = _dot(p.astype(BF) if PBF else p, vv.astype(BF) if VBF else vv) * _recip(l)
            return jnp.concatenate([o[0:MEM], first[t], o[MEM:]], axis=0) if NV else o

        def project_out(o, t, acc):
            y = _dot(o, pltpu.bitcast(wo[t * (DH // 2):(t + 1) * (DH // 2), :], BF))
            return y if acc is None else acc + y

        pr, first, mixed = {}, {}, {}
        acc, nxt = None, 0
        for t in range(H + D1 + D2):
            u = t - D1 - D2
            for ch in ORDERS[ORDER]:
                if ch in "qkv":
                    if t < H:
                        project(t, "qkv".index(ch))
                elif ch == "s":
                    if t in side_at and (SIDE >> side_at[t]) & 1:
                        due[t + SDUE] = side_work(side_at[t])
                    if 0 <= t - D1 < H:
                        pr[t - D1] = probs(t - D1)
                elif ch == "x":
                    if NV and 0 <= t - DV < H:
                        first[t - DV] = first_rows(t - DV)
                elif 0 <= u < H:
                    if NV and u not in first:
                        first[u] = first_rows(u)
                    mixed[u] = mix(u)
            if t >= H or nxt < OSTART:
                for _ in range(OTAIL if t >= H else 1):
                    if nxt <= u - D3:
                        acc = project_out(mixed[nxt], nxt, acc)
                        nxt += 1
        while nxt < H:
            acc = project_out(mixed[nxt], nxt, acc)
            nxt += 1
        mem[...] = acc[0:MEM]
        ybuf[...] = acc[MEM:]

    def fill(it, k):
        for e in range(FS):
            n = (it * UNROLL + k) * FS + e
            g = (n >= 3 * H // 2).astype(I32) + (n >= 9 * H // 2).astype(I32)
            j = jnp.minimum(n + 3 * H // 2 - 3 * H * g, 3 * H - 1)
            project_extra(j, NSEG - 3 * FG + FG * g, FG)

    def out_copy(first, count, j):
        return pltpu.make_async_copy(obuf.at[pl.ds(first, count)], out_hbm.at[pl.ds(first, count)],
                                     sem_out.at[j])

    def block(it, carry):
        with _scope("blk"):
            for k in range(UNROLL):
                if FILL:
                    fill(it, k)
                step(it, k)

        if OUTLOOP:
            @pl.when(it == 0)
            def _():
                out_copy(0, UNROLL - 1, 0).start()

            @pl.when(it > 0)
            def _():
                out_copy(it * UNROLL - 1, UNROLL, it).start()

        return carry

    nblk = NSEG // UNROLL
    lax.fori_loop(0, nblk, block, 0)

    if not OUTLOOP:
        out_copy(0, NSEG - 1, 0).start()
    c1, j1, c2, j2 = finish_rows(NSEG - 1, ybuf[...], 0, SEG, None)

    big = float(2 ** 24)
    r1 = jnp.max(c1, axis=0, keepdims=True)
    k1 = jnp.min(jnp.where(c1 == r1, j1, big), axis=0, keepdims=True)
    won = j1 == k1
    c3 = jnp.where(won, c2, c1)
    j3 = jnp.where(won, j2, j1)
    r2 = jnp.max(c3, axis=0, keepdims=True)
    k2 = jnp.min(jnp.where(c3 == r2, j3, big), axis=0, keepdims=True)
    n1 = jnp.clip(k1.astype(I32)[0, 0], 0, NSEG * SEG - 1)
    n2 = jnp.clip(k2.astype(I32)[0, 0], 0, NSEG * SEG - 1)
    s1, s2 = n1 // SEG, n2 // SEG
    sub = lax.broadcasted_iota(I32, (8, 1), 0)
    xsel = jnp.where(sub == 0, hh[s1, pl.ds(SEG + n1 % SEG, 1), :],
                     jnp.where(sub == 1, hh[s2, pl.ds(SEG + n2 % SEG, 1), :], 0.0))
    out_copy(NSEG - 1, 1, nblk).start()
    wg_copy.wait()
    wu_copy.wait()
    wd_copy.wait()
    g = _rb(_dot(xsel, pltpu.bitcast(wg[...], BF)))
    g = _rb(g * jax.nn.sigmoid(g))
    u = _rb(_dot(xsel, pltpu.bitcast(wu[...], BF)))
    y = _rb(_dot(_rb(g * u), pltpu.bitcast(wd[...], BF)))
    gate = _rb(jax.nn.sigmoid(jnp.where(sub == 0, r1, r2)))
    y = _rb(y * gate)

    if OUTLOOP:
        out_copy(0, UNROLL - 1, 0).wait()
        for j in range(1, nblk):
            out_copy(j * UNROLL - 1, UNROLL, j).wait()
    else:
        out_copy(0, NSEG - 1, 0).wait()
    out_copy(NSEG - 1, 1, nblk).wait()

    def patch(s):
        idx = lax.broadcasted_iota(I32, (SEG, 1), 0) + s * SEG
        upd = jnp.where(idx == n1, y[0:1], jnp.where(idx == n2, y[1:2], 0.0))
        obuf[s] = (hh[s, 0:SEG, :] + _rb(hh[s, SEG:2 * SEG, :] + upd)).astype(BF)

    patch(s1)
    patch(s2)
    out_copy(s1, 1, 0).start()

    @pl.when(s2 != s1)
    def _():
        out_copy(s2, 1, 1).start()
        out_copy(s2, 1, 1).wait()

    out_copy(s1, 1, 0).wait()


@functools.partial(jax.jit, static_argnames=("A_seg_len",))
def pallas_sequential_preLN__memory_aug_recurrent_mem_tr__moe_arch_mod__prompt_kernel(
    A_x, A_mem0, A_Wq, A_Wk, A_Wv, A_Wo, A_seg_len, B_x, B_w_r, B_w_gate, B_w_up, B_w_down,
):
    del B_x
    assert A_seg_len == SEG and A_x.shape == (1, NSEG * SEG, DM) and A_mem0.shape == (1, MEM, DM)
    assert A_Wq.shape == (DM, H, DH) and A_Wo.shape == (H, DH, DM) and B_w_gate.shape == (DM, DFF)
    vmem = pltpu.VMEM
    out = pl.pallas_call(
        _kernel,
        out_shape=jax.ShapeDtypeStruct((NSEG, SEG, DM), BF),
        in_specs=[pl.BlockSpec(memory_space=pl.ANY)] * 10,
        out_specs=pl.BlockSpec(memory_space=pl.ANY),
        scratch_shapes=[
            vmem((3 * H, DM // 2, DH), U32),
            vmem((H * DH // 2, DM), U32),
            vmem((NSEG, 3 * H, XR, DH), F32),
            vmem((H, 3, STR, DH), F32),
            vmem((NCH, GH // 2, 2, DM // 2, DH), U32),
            vmem((NSEG, 2 * SEG, DM), F32),
            vmem((NSEG, SEG, DM), BF),
            vmem((NSEG, SEG, DM), BF),
            vmem((DM // 2, DFF), U32),
            vmem((DM // 2, DFF), U32),
            vmem((DFF // 2, DM), U32),
            vmem((NSEG * XR, DM), F32),
            vmem((SEG, DM), F32),
            vmem((4, SEG, 1), F32),
            vmem((XS, DM), F32),
            vmem((MEM, DM), F32),
            vmem((XS, DM), BF),
            vmem((MEM, DM), BF),
            vmem((DM,), BF),
            pltpu.SemaphoreType.DMA((NCH,)),
            pltpu.SemaphoreType.DMA((19,)),
            pltpu.SemaphoreType.DMA((NSEG // UNROLL + 1,)),
        ],
        compiler_params=pltpu.CompilerParams(vmem_limit_bytes=110 * 1024 * 1024),
    )(
        A_x.reshape(NSEG, SEG, DM), A_mem0.reshape(MEM, DM),
        *(w.reshape(DM // 2, 2, H, DH) for w in (A_Wq, A_Wk, A_Wv)),
        A_Wo.reshape(H * DH, DM), B_w_r, B_w_gate, B_w_up, B_w_down,
    )
    return out.reshape(1, NSEG * SEG, DM)
```

```python
import functools
import math

import jax
import jax.numpy as jnp
from jax import lax
import jax.experimental.pallas as pl
import jax.experimental.pallas.tpu as pltpu

BF = jnp.bfloat16
F32 = jnp.float32
U32 = jnp.uint32
I32 = jnp.int32

H, DH, DM, MEM, SEG, NSEG, DFF = 32, 128, 512, 8, 32, 64, 1792
L = MEM + SEG
XR = 8
XS = SEG - XR
GH = 8
NCH = 3 * H // GH
NCB = DM // DH
UNROLL = 8
FILL = 1
D1, D2, D3, OTAIL = 4, 4, 2, 4
TOK = 1
NEARLY = 8
FG = 4
FS = 4
INITFIRST = 0
PAIRB = 1
NA = 6
QM = 0
STR = 32
OUTLOOP = 1
QBF = 0
PBF = 1
S0, S1, S2, SDUE = 0, 1, 2, 2
PO0, PO1, PO2 = -1, -1, -1
LNFREE = 0
LAG = 1
PINW = 0
NOBC = 1
PLAN = 0
PLANS = (((1, 2, 3, 6), 9, 3), ((1, 2, 1, 4), 8, 3), ((1, 2, 3), 6, 3), ((1, 2, 3, 2), 8, 3), ((1, 2, 3, 6), 12, 4),
         ((1, 2, 3, 6), 6, 2))
NP0 = 32
NP1 = 40
FFNAT = -1
ONEP = 0
APIN = 0
HZ = 0
PR = 8
PYLOOP = 0
INLOOP = 1
EPIIN = 0
WRP = 2048
RB = 0
TAB = 1
CH0, CH1, CH2 = 0, 0, 0
AEV = 1
NOSC = 1
NV = 1
DV = 2
PD = 2
ORDER = 10
KBF = 0
MERGE = 0
XREV = 0
SUMPIN = 0
VBF = 0
NPIN = 0
OSTART = 0
ORDERS = ("kvqspx", "qkvsxp", "kqsvpx", "qkvspx", "kvsqpx", "kpvsqx", "skvpqx", "xkvqsp", "kxvsqp", "vkqpsx", "pkvqsx", "kvxqps")
SIDE = 7
SCOPES = 0
EPS = 1e-5
SCALE = 0.08837890625
C2 = SCALE * math.log2(math.e)
NEG = -1e9 / SCALE
LOWEST = -2 ** 31
FLIP = 0x7FFF0000


def _dot(a, b):
    return lax.dot_general(a, b, (((1,), (0,)), ((), ())), preferred_element_type=F32)


def _dot_t(a, b):
    return lax.dot_general(a, b, (((1,), (1,)), ((), ())), preferred_element_type=F32)


def _rb(x):
    return x.astype(BF).astype(F32)


def _layernorm(x):
    n = x.shape[-1]
    mean = jnp.sum(x, axis=-1, keepdims=True) * (1.0 / n)
    xc = x - mean
    var = jnp.sum(xc * xc, axis=-1, keepdims=True) * (1.0 / n)
    den = _rb(jnp.sqrt(_rb(_rb(var) + EPS)))
    return _rb(_rb(x - _rb(mean)) * (1.0 / den))


def _layernorm_f32(x):
    n = x.shape[-1]
    xc = x - jnp.sum(x, axis=-1, keepdims=True) * (1.0 / n)
    var = jnp.sum(xc * xc, axis=-1, keepdims=True) * (1.0 / n)
    return xc * lax.rsqrt(var + EPS)


def _recip(l):
    r = pl.reciprocal(l, approx=True)
    return r * (2.0 - l * r)


def _tree(f, xs):
    while len(xs) > 1:
        xs = [f(xs[a], xs[a + 1]) if a + 1 < len(xs) else xs[a] for a in range(0, len(xs), 2)]
    return xs[0]


def _chains(f, xs, n):
    if not n:
        return _tree(f, xs)
    return _tree(f, [functools.reduce(f, xs[i::n]) for i in range(n)])


class _NoScope:
    def __enter__(self):
        return self

    def __exit__(self, *a):
        return False


def _scope(name):
    return jax.named_scope(name) if SCOPES else _NoScope()


def _kernel(x_hbm, m0_hbm, wq_hbm, wk_hbm, wv_hbm, wo_hbm, wr_hbm, wg_hbm, wu_hbm, wd_hbm,
            out_hbm,
            wp, wo, ex, st, stage, hh, xs, obuf, wg, wu, wd, xe, ybuf, top, xn, hsb, mem, x0s, pbuf, m0s, wrs,
            tab, sem_w, sem_x, sem_out):
    w_hbm = tuple(w.bitcast(U32) for w in (wq_hbm, wk_hbm, wv_hbm))
    nfill = 2 * FG * XR
    npro = NSEG * XR - nfill

    peel, body, nlong = PLANS[PLAN]
    npair = 3 * H // 2
    p0 = sum(peel)
    nit = (npair - p0) // body
    assert p0 + nit * body == npair
    bounds = [sum(peel[:g]) for g in range(len(peel))] + [p0 + i * body for i in range(nit + 1)]

    short = body - nlong
    nu = 2 * nit * short
    assert nu + 6 * H <= (NSEG - FG + 1) * FS
    fill_plan = [(2 * (p0 + i * body + q) + e, NSEG - 3 * FG)
                 for i in range(nit) for q in range(nlong, body) for e in range(2)]
    fill_plan += [(j, NSEG - g * FG) for g in (2, 1) for j in range(3 * H)]
    fill_plan += fill_plan[-1:] * (NSEG * FS - len(fill_plan))

    def w_start(ps):
        for p in ps:
            g = max(i for i, b in enumerate(bounds) if b <= p)
            for t in range(2):
                pltpu.make_async_copy(w_hbm[p // (H // 2)].at[:, t, p % (H // 2), :],
                                      stage.at[p, t], sem_w.at[g]).start()

    def w_wait(g, first, n):
        part = stage.at[pl.ds(first, n)]
        pltpu.make_async_copy(part, part, sem_w.at[g]).wait()

    wo_copy = pltpu.make_async_copy(wo_hbm.bitcast(U32), wo, sem_x.at[0])

    half = NSEG // 2

    hx = npro // XR // 2

    def x_copy(j):
        return pltpu.make_async_copy(x_hbm.at[pl.ds(j * hx, hx), pl.ds(XS, XR), :],
                                     xs.at[pl.ds(j * hx, hx), pl.ds(XS, XR), :], sem_x.at[8 + j])

    if nfill:
        xc_copy = pltpu.make_async_copy(x_hbm.at[pl.ds(2 * hx, NSEG - 2 * hx), pl.ds(XS, XR), :],
                                        xs.at[pl.ds(2 * hx, NSEG - 2 * hx), pl.ds(XS, XR), :], sem_x.at[7])

    xr_copy = pltpu.make_async_copy(x_hbm.at[:, pl.ds(0, XS), :], xs.at[:, pl.ds(0, XS), :], sem_x.at[10])
    x0_copy = pltpu.make_async_copy(x_hbm.at[0, pl.ds(0, XS), :], x0s, sem_x.at[1])
    m0_copy = pltpu.make_async_copy(m0_hbm, m0s, sem_x.at[2])
    wr_copy = pltpu.make_async_copy(wr_hbm, wrs.at[pl.ds(0, DM)], sem_x.at[3])
    wg_copy = pltpu.make_async_copy(wg_hbm.bitcast(U32), wg, sem_x.at[4])
    wu_copy = pltpu.make_async_copy(wu_hbm.bitcast(U32), wu, sem_x.at[5])
    wd_copy = pltpu.make_async_copy(wd_hbm.bitcast(U32), wd, sem_x.at[6])

    def repack(p):
        a = stage[p, 0]
        b = stage[p, 1]
        wp[2 * p] = (a & jnp.uint32(0xFFFF)) | (b << 16)
        wp[2 * p + 1] = (a >> 16) | (b & jnp.uint32(0xFFFF0000))

    def w_tile(j):
        return pltpu.bitcast(wp[j], BF)

    def project_extra(j, s0, n):
        r0 = s0 * XR if isinstance(s0, int) else pl.multiple_of(s0 * XR, XR)
        ex[pl.ds(s0, n), j] = _dot(xe[pl.ds(r0, n * XR), :], w_tile(j)).reshape(n, XR, DH)

    def ln_extra(s0, n):
        for g in range(s0, s0 + n):
            v = xs[g, XS:SEG, :].astype(F32)
            xe[g * XR:(g + 1) * XR, :] = _layernorm_f32(v)

    def start_x(j, carry):
        x_copy(j).start()
        return carry

    lax.fori_loop(0, 2, start_x, 0)
    w_start(range(bounds[0], bounds[1]))
    small = (x0_copy, m0_copy, wr_copy, xc_copy)

    def project_pairs(first, count, long, starts=None):
        repack(first)
        if count == 1 and starts is not None:
            starts()
        for i in range(count):
            n = NSEG - (2 if i < long else 3) * FG
            project_extra(2 * (first + i), 0, n)
            if i + 1 < count:
                repack(first + i + 1)
                if i + 2 == count and starts is not None:
                    starts()
            project_extra(2 * (first + i) + 1, 0, n)

    def init_state():
        mem[...] = m0s[...].astype(F32)
        xn[...] = _layernorm_f32(x0s[...].astype(F32))
        if nfill:
            ln_extra(2 * hx, NSEG - 2 * hx)
        ybuf[...] = jnp.zeros((LAG, SEG, DM), F32)
        top[...] = jnp.full((2, SEG, 1), LOWEST, I32)
        if TAB:
            for n, (j, g) in enumerate(fill_plan):
                tab[2 * n] = j
                tab[2 * n + 1] = g

    def _when(c):
        return pl.when(c) if not isinstance(c, bool) else (lambda f: f() if c else None)

    def pro_loop(i, carry):
        @_when(i == 1)
        def _():
            wo_copy.start()

        if FFNAT >= 0:
            @pl.when(i == FFNAT)
            def _():
                for cp in (wg_copy, wu_copy, wd_copy):
                    cp.start()

        def starts():
            @_when(i == 0)
            def _():
                w_start(range(NP1, npair))
                xr_copy.start()

        with _scope("pw"):
            w_wait(len(peel) + i, p0 + i * body, body)
        with _scope("part"):
            project_pairs(p0 + i * body, body, nlong, starts)
        return carry

    def prologue():
        with _scope("wait_xa"):
            x_copy(0).wait()
        w_start(range(bounds[1], bounds[2]))
        with _scope("ln_xa"):
            ln_extra(0, hx)
        with _scope("wait_xb"):
            x_copy(1).wait()
        w_start(range(bounds[2], bounds[3]))
        for cp in small:
            cp.start()
        with _scope("ln_xb"):
            ln_extra(hx, hx)
        with _scope("pro"):
            for g, n in enumerate(peel):
                last = g + 1 == len(peel)
                ps = range(bounds[3], NP0) if g == 0 else range(NP0, NP1) if last else ()
                with _scope("pw"):
                    w_wait(g, bounds[g], n)
                    if last:
                        for cp in small:
                            cp.wait()
                with _scope("p0"):
                    project_pairs(bounds[g], n, n, functools.partial(w_start, ps))
                    if last:
                        init_state()
            lax.fori_loop(0, nit - PYLOOP, pro_loop, 0)
            for i in range(nit - PYLOOP, nit):
                pro_loop(i, 0)
        with _scope("t_start"):
            for cp in (wg_copy, wu_copy, wd_copy) if FFNAT < 0 else ():
                cp.start()
        with _scope("t_wait"):
            xr_copy.wait()
            wo_copy.wait()

    if not INLOOP:
        prologue()

    def finish_rows(s, y, r0, n, live, keep=True):
        h = _rb(xs[s, r0:r0 + n, :].astype(F32) + _rb(y))
        hn = _layernorm(h)
        hh[s, r0:r0 + n, :] = h
        hh[s, SEG + r0:SEG + r0 + n, :] = hn
        obuf[s, r0:r0 + n, :] = (h + hn).astype(BF)
        r = _rb(jnp.sum(hn * wrs[pl.ds(0, DM)].astype(F32), axis=-1, keepdims=True))
        b = lax.bitcast_convert_type(r, I32)
        back = (NSEG * SEG - 1 - r0 - s * SEG) - lax.broadcasted_iota(I32, (n, 1), 0)
        key = (b ^ ((b >> 31) & FLIP)) | back
        if live is not None:
            key = jnp.where(live, key, LOWEST)
        b1, b2 = top[0, r0:r0 + n, :], top[1, r0:r0 + n, :]
        new = jnp.maximum(key, b1), jnp.maximum(jnp.minimum(key, b1), b2)
        if keep:
            top[0, r0:r0 + n, :] = new[0]
            top[1, r0:r0 + n, :] = new[1]
        return new

    def step(it, k):
        s = it * UNROLL + k
        row = lax.broadcasted_iota(I32, (L, L), 0)
        col = lax.broadcasted_iota(I32, (L, L), 1)
        mask = (row < MEM) | (row >= col)
        hs = jnp.concatenate([mem[...], xn[...]], axis=0).astype(BF)
        hrows = (MEM + XS) // 2
        zz = pl.multiple_of(jnp.minimum(s, 0), 8)
        if HZ:
            hsb[pl.ds(zz, hrows), :] = pltpu.bitcast(hs, U32)

        def lhs(i):
            if not HZ:
                return hs
            if i and i % HZ == 0:
                hsb[pl.ds(zz + hrows, 8), 0:DH] = jnp.zeros((8, DH), U32)
            return pltpu.bitcast(hsb[0:hrows, :], BF)

        s0 = pl.multiple_of(it * UNROLL, UNROLL)
        prev = s0 + (k - LAG) if k >= LAG else jnp.maximum(s - LAG, 0)
        succ = s0 + (k + 1) if k + 1 < UNROLL else jnp.minimum(s + 1, NSEG - 1)
        yprev = ybuf[k % LAG]
        never = s < 0
        zero = jnp.minimum(s, 0)
        e0 = pl.multiple_of(it * (UNROLL * XR), UNROLL * XR) + k * XR

        def side_work(j):
            if j < 2:
                if ONEP and j == 1:
                    return []
                for i in range(2) if ONEP == 1 else [j]:
                    if ONEP == 2:
                        finish_rows(prev, yprev, 0, SEG, None if k >= LAG else s >= LAG)
                    else:
                        finish_rows(prev, yprev[16 * i:16 * i + 16], 16 * i, 16, None if k >= LAG else s >= LAG)
                if not TOK:
                    return None
                z8 = pl.multiple_of(zero, 8)
                z16 = pl.multiple_of(zero, 16)
                toks = [hh[prev, pl.ds(z8, 8), 0:DH], top[0, pl.ds(z8, 8), :].astype(F32),
                        obuf[prev, pl.ds(z16, 16), 0:DH].astype(F32)[0:8]]
                return [toks[0] + toks[1] + toks[2]] if PINW in (0, 3) else toks
            xn[...] = _layernorm_f32(xs[succ, 0:XS, :].astype(F32))
            if not TOK:
                return None
            return [xn[pl.ds(pl.multiple_of(zero, 8), 8), 0:DH]]

        side_at = {S0: 0, S1: 1, S2: 2}
        due = {}
        odue = {}
        po = (PO0, PO1, PO2)

        sub = lax.broadcasted_iota(I32, (8, 1), 0)
        groups = [0] + list(range(1 + NV, L // 8))

        def project(t, m):
            if MERGE:
                if m == 1:
                    ms = (1, 2, 0) if MERGE == 1 else (0, 1, 2)
                    y = _dot(hs, jnp.concatenate([w_tile(a * H + t) for a in ms], axis=1))
                    for i, a in enumerate(ms):
                        st[t, a] = y[:, i * DH:(i + 1) * DH]
                return
            st[t, m] = _dot(lhs(3 * t + ORDERS[ORDER].replace("s", "").replace("p", "").replace("x", "").index("qkv"[m])),
                            w_tile(m * H + t))

        def rows(t, m, gs):
            return [ex[s, m * H + t] if g == L // 8 - 1 else st[t, m, 8 * g:8 * g + 8, :] for g in gs]

        def probs(t):
            q = rows(t, 0, groups)
            kr = rows(t, 1, range(L // 8))
            for i, tok in enumerate(due.get(t, ())):
                if PINW < 2:
                    q[-1 - i] = jnp.where(never, tok, q[-1 - i])
                else:
                    kr[-1 - i] = jnp.where(never, tok, kr[-1 - i])
            kk = jnp.concatenate(kr, axis=0)
            if KBF:
                kk = kk.astype(BF)
            mk = jnp.concatenate([mask[8 * g:8 * g + 8] for g in groups], axis=0)
            qq = jnp.concatenate(q, axis=0)
            sc = jnp.where(mk, _dot_t(qq.astype(BF) if QBF else qq, kk), NEG)
            p = jnp.exp2((sc - jnp.max(sc, axis=-1, keepdims=True)) * C2)
            return p, jnp.sum(p, axis=-1, keepdims=True)

        def first_rows(t):
            q = rows(t, 0, [1])[0] * C2
            kk = rows(t, 1, [0, 1])
            vv = rows(t, 2, [0, 1])

            def row(a, j):
                if RB & (1 if a is kk else 2):
                    return jnp.broadcast_to(st[t, 1 if a is kk else 2, j:j + 1, :], (8, DH))
                return jnp.broadcast_to(a[j // 8][j % 8:j % 8 + 1], (8, DH))

            order = list(range(MEM + 8))
            if XREV:
                order = order[::-1]
            sc = {}
            for j in order:
                sj = jnp.sum(q * row(kk, j), axis=-1, keepdims=True)
                sc[j] = jnp.where(sub >= j - MEM, sj, NEG * C2) if j > MEM else sj
            sc = [sc[j] for j in range(MEM + 8)]
            mx = _chains(jnp.maximum, sc, CH0)
            p = [jnp.exp2(sj - mx) for sj in sc]
            o = _chains(jnp.add, [p[j] * row(vv, j) for j in range(MEM + 8)], CH1)
            return o * _recip(_chains(jnp.add, p, CH2))

        def mix(t):
            p, l = pr[t]
            v = rows(t, 2, range(L // 8))
            if NV and t - PD >= 0:
                v[0] = jnp.where(never, first[t - PD], v[0])
            if NPIN and t - NPIN >= 0:
                v[2] = jnp.where(never, _tree(jnp.add, [mixed[t - NPIN][8 * g:8 * g + 8] for g in groups]), v[2])
            if SUMPIN and t - SUMPIN >= 0:
                ls = pr[t - SUMPIN][1]
                v[3] = jnp.where(never, _tree(jnp.add, [ls[8 * g:8 * g + 8] for g in range(len(groups))]), v[3])
            vv = jnp.concatenate(v, axis=0)
            o = _dot(p.astype(BF) if PBF else p, vv.astype(BF) if VBF else vv) * _recip(l)
            return jnp.concatenate([o[0:MEM], first[t], o[MEM:]], axis=0) if NV else o

        def project_out(o, t, acc):
            for tok in odue.get(t, ()):
                o = jnp.concatenate([jnp.where(never, tok, o[0:8]), o[8:]], axis=0)
            if APIN and t - APIN >= 1 and t % AEV == 0:
                a = accs[t - APIN]
                o = jnp.where(never, _tree(jnp.add, [a[:, c * DH:(c + 1) * DH] for c in range(NCB)]), o)
            y = _dot(o, pltpu.bitcast(wo[t * (DH // 2):(t + 1) * (DH // 2), :], BF))
            accs[t] = y if acc is None else acc + y
            return accs[t]

        pr, first, mixed, accs = {}, {}, {}, {}
        acc, nxt = None, 0
        for t in range(H + D1 + D2):
            u = t - D1 - D2
            for ch in ORDERS[ORDER]:
                if ch in "qkv":
                    if t < H:
                        project(t, "qkv".index(ch))
                elif ch == "s":
                    if t in side_at and (SIDE >> side_at[t]) & 1:
                        j = side_at[t]
                        tok = side_work(j)
                        if j == 2 and LNFREE and k + 1 < UNROLL:
                            pass
                        elif po[j] >= 0:
                            odue.setdefault(po[j], []).extend(tok)
                        else:
                            due[t + SDUE] = tok
                    if 0 <= t - D1 < H:
                        pr[t - D1] = probs(t - D1)
                elif ch == "x":
                    if NV and 0 <= t - DV < H:
                        first[t - DV] = first_rows(t - DV)
                elif 0 <= u < H:
                    if NV and u not in first:
                        first[u] = first_rows(u)
                    mixed[u] = mix(u)
            if t >= H or nxt < OSTART:
                for _ in range(OTAIL if t >= H else 1):
                    if nxt <= u - D3:
                        acc = project_out(mixed[nxt], nxt, acc)
                        nxt += 1
        while nxt < H:
            acc = project_out(mixed[nxt], nxt, acc)
            nxt += 1
        mem[...] = acc[0:MEM]
        ybuf[k % LAG] = acc[MEM:]

    def fill(it, k):
        for e in range(FS):
            n = (it * UNROLL + k) * FS + e
            if TAB:
                project_extra(tab[2 * n], tab[2 * n + 1], FG)
            else:
                g = (n >= nu).astype(I32) + (n >= nu + 3 * H).astype(I32)
                skip = 2 * (p0 + nlong) + sum((n >= 2 * short * i).astype(I32) * (2 * nlong) for i in range(1, nit))
                j = jnp.where(n < nu, n + skip, jnp.minimum(n - nu - 3 * H * (g - 1), 3 * H - 1))
                project_extra(j, NSEG - 3 * FG + FG * g, FG)

    def out_copy(first, count):
        return pltpu.make_async_copy(obuf.at[pl.ds(first, count)], out_hbm.at[pl.ds(first, count)],
                                     sem_out.at[0])

    def block(it, carry):
        if INLOOP:
            pl.when(it == 0)(prologue)
        with _scope("blk"):
            for k in range(UNROLL):
                if FILL:
                    fill(it, k)
                step(it, k)

        if OUTLOOP:
            @pl.when(it == 0)
            def _():
                out_copy(0, UNROLL - LAG).start()

            @pl.when(it > 0)
            def _():
                out_copy(it * UNROLL - LAG, UNROLL).start()

        if EPIIN:
            pl.when(it == nblk - 1)(epilogue)
        return carry

    nblk = NSEG // UNROLL

    sub = lax.broadcasted_iota(I32, (8, 1), 0)
    last = NSEG * SEG - 1

    def select(b1, b2):
        k1 = jnp.max(b1, axis=0, keepdims=True)
        k2 = jnp.max(jnp.where(b1 == k1, b2, b1), axis=0, keepdims=True)
        return k1[0, 0], k2[0, 0]

    def place(key):
        n = last - (key & last)
        r = n & (SEG - 1)
        return n >> 5, r, pl.multiple_of(r & -PR, PR)

    def ffn(k1, k2):
        (s1, r1, _), (s2, r2, _) = place(k1), place(k2)
        xsel = jnp.where(sub == 0, hh[s1, pl.ds(SEG + r1, 1), :],
                         jnp.where(sub == 1, hh[s2, pl.ds(SEG + r2, 1), :], 0.0))
        g = _rb(_dot(xsel, pltpu.bitcast(wg[...], BF)))
        g = _rb(g * jax.nn.sigmoid(g))
        u = _rb(_dot(xsel, pltpu.bitcast(wu[...], BF)))
        return _rb(_dot(_rb(g * u), pltpu.bitcast(wd[...], BF)))

    def patch(y, k1, k2):
        hi = jnp.where(lax.broadcasted_iota(I32, (8, DH), 0) == 0, k1, k2) & -65536
        gate = _rb(jax.nn.sigmoid(lax.bitcast_convert_type(hi ^ ((hi >> 31) & FLIP), F32)))
        y = _rb(y * jnp.concatenate([gate] * NCB, axis=1))
        for j, key in enumerate((k1, k2)):
            s, _, g = place(key)
            back = (last - s * SEG - g) - lax.broadcasted_iota(I32, (PR, 1), 0)
            upd = jnp.where(back == (k1 & last), y[0:1], jnp.where(back == (k2 & last), y[1:2], 0.0))
            pbuf[j] = (hh[s, pl.ds(g, PR), :] + _rb(hh[s, pl.ds(SEG + g, PR), :] + upd)).astype(BF)

    def epilogue():
        with _scope("e_w"):
            wg_copy.wait()
            wu_copy.wait()
            wd_copy.wait()
        m1, m2 = select(top[0], top[1])
        y = ffn(m1, m2)
        for g in range(NSEG - LAG, NSEG):
            c1, c2 = finish_rows(g, ybuf[g % LAG], 0, SEG, None, g + 1 < NSEG)
        out_copy(NSEG - LAG, LAG).start()
        k1, k2 = select(c1, c2)
        patch(y, k1, k2)

        @pl.when((k1 != m1) | (k2 != m2))
        def _():
            patch(ffn(k1, k2), k1, k2)

        out_copy(0, NSEG).wait()
        (s1, _, g1), (s2, _, g2) = place(k1), place(k2)
        cp1 = pltpu.make_async_copy(pbuf.at[0], out_hbm.at[s1, pl.ds(g1, PR), :], sem_out.at[0])
        cp2 = pltpu.make_async_copy(pbuf.at[1], out_hbm.at[s2, pl.ds(g2, PR), :], sem_out.at[1])
        cp1.start()

        @pl.when((s2 != s1) | (g2 != g1))
        def _():
            cp2.start()
            cp2.wait()

        cp1.wait()

    lax.fori_loop(0, nblk, block, 0)
    if not EPIIN:
        epilogue()


@functools.partial(jax.jit, static_argnames=("A_seg_len",))
def pallas_sequential_preLN__memory_aug_recurrent_mem_tr__moe_arch_mod__prompt_kernel(
    A_x, A_mem0, A_Wq, A_Wk, A_Wv, A_Wo, A_seg_len, B_x, B_w_r, B_w_gate, B_w_up, B_w_down,
):
    del B_x
    assert A_seg_len == SEG and A_x.shape == (1, NSEG * SEG, DM) and A_mem0.shape == (1, MEM, DM)
    assert A_Wq.shape == (DM, H, DH) and A_Wo.shape == (H, DH, DM) and B_w_gate.shape == (DM, DFF)
    vmem = pltpu.VMEM
    out = pl.pallas_call(
        _kernel,
        out_shape=jax.ShapeDtypeStruct((NSEG, SEG, DM), BF),
        in_specs=[pl.BlockSpec(memory_space=pl.ANY)] * 10,
        out_specs=pl.BlockSpec(memory_space=pl.ANY),
        scratch_shapes=[
            vmem((3 * H, DM // 2, DH), U32),
            vmem((H * DH // 2, DM), U32),
            vmem((NSEG, 3 * H, XR, DH), F32),
            vmem((H, 3, STR, DH), F32),
            vmem((3 * H // 2, 2, DM // 2, DH), U32),
            vmem((NSEG, 2 * SEG, DM), F32),
            vmem((NSEG, SEG, DM), BF),
            vmem((NSEG, SEG, DM), BF),
            vmem((DM // 2, DFF), U32),
            vmem((DM // 2, DFF), U32),
            vmem((DFF // 2, DM), U32),
            vmem((NSEG * XR, DM), F32),
            vmem((LAG, SEG, DM), F32),
            vmem((2, SEG, 1), I32),
            vmem((XS, DM), F32),
            vmem(((MEM + XS) // 2 + 8, DM), U32),
            vmem((MEM, DM), F32),
            vmem((XS, DM), BF),
            vmem((2, PR, DM), BF),
            vmem((MEM, DM), BF),
            vmem((WRP,), BF),
            pltpu.SMEM((2 * NSEG * FS,), I32),
            pltpu.SemaphoreType.DMA((NCH,)),
            pltpu.SemaphoreType.DMA((11,)),
            pltpu.SemaphoreType.DMA((2,)),
        ],
        compiler_params=pltpu.CompilerParams(
            vmem_limit_bytes=110 * 1024 * 1024,
            disable_bounds_checks=bool(NOBC), disable_semaphore_checks=bool(NOSC)),
    )(
        A_x.reshape(NSEG, SEG, DM), A_mem0.reshape(MEM, DM),
        *(w.reshape(DM // 2, 2, H, DH) for w in (A_Wq, A_Wk, A_Wv)),
        A_Wo.reshape(H * DH, DM), B_w_r, B_w_gate, B_w_up, B_w_down,
    )
    return out.reshape(1, NSEG * SEG, DM)
```

```python
import functools
import math

import jax
import jax.numpy as jnp
from jax import lax
import jax.experimental.pallas as pl
import jax.experimental.pallas.tpu as pltpu

BF = jnp.bfloat16
F32 = jnp.float32
U32 = jnp.uint32
I32 = jnp.int32

H, DH, DM, MEM, SEG, NSEG, DFF = 32, 128, 512, 8, 32, 64, 1792
L = MEM + SEG
XR = 8
XS = SEG - XR
GH = 8
NCH = 3 * H // GH
NCB = DM // DH
UNROLL = 8
FILL = 1
D1, D2, D3, OTAIL = 4, 4, 2, 4
TOK = 1
NEARLY = 8
FG = 4
FS = 4
INITFIRST = 0
PAIRB = 1
NA = 6
QM = 0
STR = 32
OUTLOOP = 1
QBF = 0
PBF = 1
S0, S1, S2, SDUE = 0, 1, 2, 2
PO0, PO1, PO2 = -1, -1, -1
LNFREE = 0
LAG = 1
PINW = 0
NOBC = 1
PLAN = 0
PLANS = (((1, 2, 3, 6), 9, 3), ((1, 2, 1, 4), 8, 3), ((1, 2, 3), 6, 3), ((1, 2, 3, 2), 8, 3), ((1, 2, 3, 6), 12, 4),
         ((1, 2, 3, 6), 6, 2), ((1, 2, 3, 6, 10), 13, 0), ((1, 2, 3, 6, 8), 14, 1), ((1, 2, 3, 6, 9), 9, 1))
NP0 = 32
NP1 = 40
FFNAT = -1
ONEP = 0
APIN = 0
HZ = 0
PR = 8
PYLOOP = 0
NSH = 2
OV = {('FAT', 0): 1, ('FIN', 0): 4, ('MERGE', 0): 2, ('PD', 0): 1, ('RB', 0): 3, ('SDUE', 0): 1, ('CH2', 1): 2, ('LNFREE', 1): 1, ('PO2', 1): 28, ('QBF', 1): 1, ('CH1', 2): 1, ('XREV', 2): 1, ('CH1', 3): 2, ('PINW', 3): 1, ('LNFREE', 4): 1, ('PO2', 4): 28, ('LNFREE', 5): 1, ('PINW', 5): 1, ('PO2', 5): 28}
FIN = 0
FAT = 6
INLOOP = 1
EPIIN = 0
WRP = 2048
RB = 1
TAB = 1
CH0, CH1, CH2 = 0, 0, 0
AEV = 1
NOSC = 1
NV = 1
DV = 5
PD = 2
ORDER = 10
KBF = 0
MERGE = 0
XREV = 0
SUMPIN = 0
VBF = 0
NPIN = 0
OSTART = 0
ORDERS = ("kvqspx", "qkvsxp", "kqsvpx", "qkvspx", "kvsqpx", "kpvsqx", "skvpqx", "xkvqsp", "kxvsqp", "vkqpsx", "pkvqsx", "kvxqps")
SIDE = 7
SCOPES = 0
EPS = 1e-5
SCALE = 0.08837890625
C2 = SCALE * math.log2(math.e)
NEG = -1e9 / SCALE
LOWEST = -2 ** 31
FLIP = 0x7FFF0000


def _dot(a, b):
    return lax.dot_general(a, b, (((1,), (0,)), ((), ())), preferred_element_type=F32)


def _dot_t(a, b):
    return lax.dot_general(a, b, (((1,), (1,)), ((), ())), preferred_element_type=F32)


def _rb(x):
    return x.astype(BF).astype(F32)


def _layernorm(x):
    n = x.shape[-1]
    mean = jnp.sum(x, axis=-1, keepdims=True) * (1.0 / n)
    xc = x - mean
    var = jnp.sum(xc * xc, axis=-1, keepdims=True) * (1.0 / n)
    den = _rb(jnp.sqrt(_rb(_rb(var) + EPS)))
    return _rb(_rb(x - _rb(mean)) * (1.0 / den))


def _layernorm_f32(x):
    n = x.shape[-1]
    xc = x - jnp.sum(x, axis=-1, keepdims=True) * (1.0 / n)
    var = jnp.sum(xc * xc, axis=-1, keepdims=True) * (1.0 / n)
    return xc * lax.rsqrt(var + EPS)


def _recip(l):
    r = pl.reciprocal(l, approx=True)
    return r * (2.0 - l * r)


def _tree(f, xs):
    while len(xs) > 1:
        xs = [f(xs[a], xs[a + 1]) if a + 1 < len(xs) else xs[a] for a in range(0, len(xs), 2)]
    return xs[0]


def _chains(f, xs, n):
    if not n:
        return _tree(f, xs)
    return _tree(f, [functools.reduce(f, xs[i::n]) for i in range(n)])


class _NoScope:
    def __enter__(self):
        return self

    def __exit__(self, *a):
        return False


def _scope(name):
    return jax.named_scope(name) if SCOPES else _NoScope()


def _kernel(x_hbm, m0_hbm, wq_hbm, wk_hbm, wv_hbm, wo_hbm, wr_hbm, wg_hbm, wu_hbm, wd_hbm,
            out_hbm,
            wp, wo, ex, st, stage, hh, xs, obuf, wg, wu, wd, xe, ybuf, top, xn, hsb, mem, x0s, pbuf, m0s, wrs,
            tab, sem_w, sem_x, sem_out):
    w_hbm = tuple(w.bitcast(U32) for w in (wq_hbm, wk_hbm, wv_hbm))
    nfill = 2 * FG * XR
    npro = NSEG * XR - nfill

    peel, body, nlong = PLANS[PLAN]
    npair = 3 * H // 2
    p0 = sum(peel)
    nit = (npair - p0) // body
    assert p0 + nit * body == npair
    bounds = [sum(peel[:g]) for g in range(len(peel))] + [p0 + i * body for i in range(nit + 1)]

    left = list(range(p0 - NSH, p0)) + [p0 + i * body + q for i in range(nit) for q in range(nlong, body)]
    assert 2 * len(left) + 6 * H <= (NSEG - FG + 1) * FS
    fill_plan = [(2 * p + e, NSEG - 3 * FG) for p in left for e in range(2)]
    fill_plan += [(j, NSEG - g * FG) for g in (2, 1) for j in range(3 * H)]
    fill_plan += fill_plan[-1:] * (NSEG * FS - len(fill_plan))

    def w_start(ps):
        for p in ps:
            g = max(i for i, b in enumerate(bounds) if b <= p)
            for t in range(2):
                pltpu.make_async_copy(w_hbm[p // (H // 2)].at[:, t, p % (H // 2), :],
                                      stage.at[p, t], sem_w.at[g]).start()

    def w_wait(g, first, n):
        part = stage.at[pl.ds(first, n)]
        pltpu.make_async_copy(part, part, sem_w.at[g]).wait()

    wo_copy = pltpu.make_async_copy(wo_hbm.bitcast(U32), wo, sem_x.at[0])

    half = NSEG // 2

    hx = npro // XR // 2

    def x_copy(j):
        return pltpu.make_async_copy(x_hbm.at[pl.ds(j * hx, hx), pl.ds(XS, XR), :],
                                     xs.at[pl.ds(j * hx, hx), pl.ds(XS, XR), :], sem_x.at[8 + j])

    if nfill:
        xc_copy = pltpu.make_async_copy(x_hbm.at[pl.ds(2 * hx, NSEG - 2 * hx), pl.ds(XS, XR), :],
                                        xs.at[pl.ds(2 * hx, NSEG - 2 * hx), pl.ds(XS, XR), :], sem_x.at[7])

    xr_copy = pltpu.make_async_copy(x_hbm.at[:, pl.ds(0, XS), :], xs.at[:, pl.ds(0, XS), :], sem_x.at[10])
    x0_copy = pltpu.make_async_copy(x_hbm.at[0, pl.ds(0, XS), :], x0s, sem_x.at[1])
    m0_copy = pltpu.make_async_copy(m0_hbm, m0s, sem_x.at[2])
    wr_copy = pltpu.make_async_copy(wr_hbm, wrs.at[pl.ds(0, DM)], sem_x.at[3])
    wg_copy = pltpu.make_async_copy(wg_hbm.bitcast(U32), wg, sem_x.at[4])
    wu_copy = pltpu.make_async_copy(wu_hbm.bitcast(U32), wu, sem_x.at[5])
    wd_copy = pltpu.make_async_copy(wd_hbm.bitcast(U32), wd, sem_x.at[6])

    def repack(p):
        a = stage[p, 0]
        b = stage[p, 1]
        wp[2 * p] = (a & jnp.uint32(0xFFFF)) | (b << 16)
        wp[2 * p + 1] = (a >> 16) | (b & jnp.uint32(0xFFFF0000))

    def w_tile(j):
        return pltpu.bitcast(wp[j], BF)

    def project_extra(j, s0, n):
        r0 = s0 * XR if isinstance(s0, int) else pl.multiple_of(s0 * XR, XR)
        ex[pl.ds(s0, n), j] = _dot(xe[pl.ds(r0, n * XR), :], w_tile(j)).reshape(n, XR, DH)

    def ln_extra(s0, n):
        for g in range(s0, s0 + n):
            v = xs[g, XS:SEG, :].astype(F32)
            xe[g * XR:(g + 1) * XR, :] = _layernorm_f32(v)

    def start_x(j, carry):
        x_copy(j).start()
        return carry

    lax.fori_loop(0, 2, start_x, 0)
    w_start(range(bounds[0], bounds[1]))
    small = (x0_copy, m0_copy, wr_copy, xc_copy)

    def project_pairs(first, count, long, starts=None):
        repack(first)
        if count == 1 and starts is not None:
            starts()
        for i in range(count):
            n = NSEG - (2 if i < long else 3) * FG
            project_extra(2 * (first + i), 0, n)
            if i + 1 < count:
                repack(first + i + 1)
                if i + 2 == count and starts is not None:
                    starts()
            project_extra(2 * (first + i) + 1, 0, n)

    def init_state():
        mem[...] = m0s[...].astype(F32)
        xn[...] = _layernorm_f32(x0s[...].astype(F32))
        if nfill:
            ln_extra(2 * hx, NSEG - 2 * hx)
        ybuf[...] = jnp.zeros((LAG, SEG, DM), F32)
        top[...] = jnp.full((2, SEG, 1), LOWEST, I32)
        if TAB:
            for n, (j, g) in enumerate(fill_plan):
                tab[2 * n] = j
                tab[2 * n + 1] = g

    def _when(c):
        return pl.when(c) if not isinstance(c, bool) else (lambda f: f() if c else None)

    def stage_starts(k):
        @_when(k == 0)
        def _():
            w_start(range(bounds[3], NP0))

        @_when(k == 3)
        def _():
            w_start(range(NP0, NP1))

        @_when(k == 4)
        def _():
            w_start(range(NP1, npair))
            xr_copy.start()

    def pro_loop(i, carry):
        @_when(i == 5 - len(peel))
        def _():
            wo_copy.start()

        def starts():
            if len(peel) == 4:
                _when(i == 0)(functools.partial(stage_starts, 4))

        with _scope("pw"):
            w_wait(len(peel) + i, p0 + i * body, body)
        with _scope("part"):
            project_pairs(p0 + i * body, body, nlong, starts)
        return carry

    def prologue():
        with _scope("wait_xa"):
            x_copy(0).wait()
        w_start(range(bounds[1], bounds[2]))
        with _scope("ln_xa"):
            ln_extra(0, hx)
        with _scope("wait_xb"):
            x_copy(1).wait()
        w_start(range(bounds[2], bounds[3]))
        for cp in small:
            cp.start()
        with _scope("ln_xb"):
            ln_extra(hx, hx)
        with _scope("pro"):
            for g, n in enumerate(peel):
                last = g + 1 == len(peel)
                with _scope("pw"):
                    w_wait(g, bounds[g], n)
                    if last:
                        for cp in small:
                            cp.wait()
                with _scope("p0"):
                    project_pairs(bounds[g], n, n - NSH if last else n, functools.partial(stage_starts, g))
                    if last:
                        init_state()
            lax.fori_loop(0, nit - PYLOOP, pro_loop, 0)
            for i in range(nit - PYLOOP, nit):
                pro_loop(i, 0)
        with _scope("t_start"):
            for cp in (wg_copy, wu_copy, wd_copy):
                cp.start()
        with _scope("t_wait"):
            xr_copy.wait()
            wo_copy.wait()

    if not INLOOP:
        prologue()

    def finish_rows(s, y, r0, n, live, keep=True):
        h = _rb(xs[s, r0:r0 + n, :].astype(F32) + _rb(y))
        hn = _layernorm(h)
        hh[s, r0:r0 + n, :] = h
        hh[s, SEG + r0:SEG + r0 + n, :] = hn
        obuf[s, r0:r0 + n, :] = (h + hn).astype(BF)
        r = _rb(jnp.sum(hn * wrs[pl.ds(0, DM)].astype(F32), axis=-1, keepdims=True))
        b = lax.bitcast_convert_type(r, I32)
        back = (NSEG * SEG - 1 - r0 - s * SEG) - lax.broadcasted_iota(I32, (n, 1), 0)
        key = (b ^ ((b >> 31) & FLIP)) | back
        if live is not None:
            key = jnp.where(live, key, LOWEST)
        b1, b2 = top[0, r0:r0 + n, :], top[1, r0:r0 + n, :]
        new = jnp.maximum(key, b1), jnp.maximum(jnp.minimum(key, b1), b2)
        if keep:
            top[0, r0:r0 + n, :] = new[0]
            top[1, r0:r0 + n, :] = new[1]
        return new

    base = dict(D1=D1, D2=D2, DV=DV, PD=PD, OTAIL=OTAIL, D3=D3, ORDER=ORDER, QBF=QBF, PBF=PBF, VBF=VBF, MERGE=MERGE, XREV=XREV, SUMPIN=SUMPIN, NPIN=NPIN, S0=S0, S1=S1, S2=S2, SDUE=SDUE, PINW=PINW, ONEP=ONEP, APIN=APIN, AEV=AEV, CH0=CH0, CH1=CH1, CH2=CH2, RB=RB, LNFREE=LNFREE, PO2=PO2, FIN=FIN, FAT=FAT)

    def step(it, k):
        (D1, D2, DV, PD, OTAIL, D3, ORDER, QBF, PBF, VBF, MERGE, XREV, SUMPIN, NPIN, S0, S1, S2, SDUE, PINW, ONEP, APIN, AEV, CH0, CH1, CH2, RB, LNFREE, PO2, FIN, FAT) = [OV.get((n, k), v) for n, v in base.items()]
        s = it * UNROLL + k
        row = lax.broadcasted_iota(I32, (L, L), 0)
        col = lax.broadcasted_iota(I32, (L, L), 1)
        mask = (row < MEM) | (row >= col)
        hs = jnp.concatenate([mem[...], xn[...]], axis=0).astype(BF)
        hrows = (MEM + XS) // 2
        zz = pl.multiple_of(jnp.minimum(s, 0), 8)
        if HZ:
            hsb[pl.ds(zz, hrows), :] = pltpu.bitcast(hs, U32)

        def lhs(i):
            if not HZ:
                return hs
            if i and i % HZ == 0:
                hsb[pl.ds(zz + hrows, 8), 0:DH] = jnp.zeros((8, DH), U32)
            return pltpu.bitcast(hsb[0:hrows, :], BF)

        s0 = pl.multiple_of(it * UNROLL, UNROLL)
        prev = s0 + (k - LAG) if k >= LAG else jnp.maximum(s - LAG, 0)
        succ = s0 + (k + 1) if k + 1 < UNROLL else jnp.minimum(s + 1, NSEG - 1)
        yprev = ybuf[k % LAG]
        never = s < 0
        zero = jnp.minimum(s, 0)
        e0 = pl.multiple_of(it * (UNROLL * XR), UNROLL * XR) + k * XR

        def side_work(j):
            if j < 2:
                if ONEP and j == 1:
                    return []
                for i in range(2) if ONEP == 1 else [j]:
                    if ONEP == 2:
                        finish_rows(prev, yprev, 0, SEG, None if k >= LAG else s >= LAG)
                    else:
                        finish_rows(prev, yprev[16 * i:16 * i + 16], 16 * i, 16, None if k >= LAG else s >= LAG)
                if not TOK:
                    return None
                z8 = pl.multiple_of(zero, 8)
                z16 = pl.multiple_of(zero, 16)
                toks = [hh[prev, pl.ds(z8, 8), 0:DH], top[0, pl.ds(z8, 8), :].astype(F32),
                        obuf[prev, pl.ds(z16, 16), 0:DH].astype(F32)[0:8]]
                return [toks[0] + toks[1] + toks[2]] if PINW in (0, 3) else toks
            xn[...] = _layernorm_f32(xs[succ, 0:XS, :].astype(F32))
            if not TOK:
                return None
            return [xn[pl.ds(pl.multiple_of(zero, 8), 8), 0:DH]]

        side_at = {S0: 0, S1: 1, S2: 2}
        due = {}
        odue = {}
        po = (PO0, PO1, PO2)

        sub = lax.broadcasted_iota(I32, (8, 1), 0)
        groups = [0] + list(range(1 + NV, L // 8))

        def project(t, m):
            if MERGE:
                if m == 1:
                    ms = (1, 2, 0) if MERGE == 1 else (0, 1, 2)
                    y = _dot(hs, jnp.concatenate([w_tile(a * H + t) for a in ms], axis=1))
                    for i, a in enumerate(ms):
                        st[t, a] = y[:, i * DH:(i + 1) * DH]
                return
            st[t, m] = _dot(lhs(3 * t + ORDERS[ORDER].replace("s", "").replace("p", "").replace("x", "").index("qkv"[m])),
                            w_tile(m * H + t))

        def rows(t, m, gs):
            return [ex[s, m * H + t] if g == L // 8 - 1 else st[t, m, 8 * g:8 * g + 8, :] for g in gs]

        def probs(t):
            q = rows(t, 0, groups)
            kr = rows(t, 1, range(L // 8))
            for i, tok in enumerate(due.get(t, ())):
                if PINW < 2:
                    q[-1 - i] = jnp.where(never, tok, q[-1 - i])
                else:
                    kr[-1 - i] = jnp.where(never, tok, kr[-1 - i])
            kk = jnp.concatenate(kr, axis=0)
            if KBF:
                kk = kk.astype(BF)
            mk = jnp.concatenate([mask[8 * g:8 * g + 8] for g in groups], axis=0)
            qq = jnp.concatenate(q, axis=0)
            sc = jnp.where(mk, _dot_t(qq.astype(BF) if QBF else qq, kk), NEG)
            p = jnp.exp2((sc - jnp.max(sc, axis=-1, keepdims=True)) * C2)
            return p, jnp.sum(p, axis=-1, keepdims=True)

        def first_rows(t):
            q = rows(t, 0, [1])[0] * C2
            kk = rows(t, 1, [0, 1])
            vv = rows(t, 2, [0, 1])

            def row(a, j):
                if RB & (1 if a is kk else 2):
                    return jnp.broadcast_to(st[t, 1 if a is kk else 2, j:j + 1, :], (8, DH))
                return jnp.broadcast_to(a[j // 8][j % 8:j % 8 + 1], (8, DH))

            order = list(range(MEM + 8))
            if XREV:
                order = order[::-1]
            sc = {}
            for j in order:
                sj = jnp.sum(q * row(kk, j), axis=-1, keepdims=True)
                sc[j] = jnp.where(sub >= j - MEM, sj, NEG * C2) if j > MEM else sj
            sc = [sc[j] for j in range(MEM + 8)]
            mx = _chains(jnp.maximum, sc, CH0)
            p = [jnp.exp2(sj - mx) for sj in sc]
            o = _chains(jnp.add, [p[j] * row(vv, j) for j in range(MEM + 8)], CH1)
            return o * _recip(_chains(jnp.add, p, CH2))

        def mix(t):
            p, l = pr[t]
            v = rows(t, 2, range(L // 8))
            if NV and t - PD >= 0:
                v[0] = jnp.where(never, first[t - PD], v[0])
            if NPIN and t - NPIN >= 0:
                v[2] = jnp.where(never, _tree(jnp.add, [mixed[t - NPIN][8 * g:8 * g + 8] for g in groups]), v[2])
            if SUMPIN and t - SUMPIN >= 0:
                ls = pr[t - SUMPIN][1]
                v[3] = jnp.where(never, _tree(jnp.add, [ls[8 * g:8 * g + 8] for g in range(len(groups))]), v[3])
            vv = jnp.concatenate(v, axis=0)
            o = _dot(p.astype(BF) if PBF else p, vv.astype(BF) if VBF else vv) * _recip(l)
            return jnp.concatenate([o[0:MEM], first[t], o[MEM:]], axis=0) if NV else o

        def project_out(o, t, acc):
            for tok in odue.get(t, ()):
                o = jnp.concatenate([jnp.where(never, tok, o[0:8]), o[8:]], axis=0)
            if APIN and t - APIN >= 1 and t % AEV == 0:
                a = accs[t - APIN]
                o = jnp.where(never, _tree(jnp.add, [a[:, c * DH:(c + 1) * DH] for c in range(NCB)]), o)
            y = _dot(o, pltpu.bitcast(wo[t * (DH // 2):(t + 1) * (DH // 2), :], BF))
            accs[t] = y if acc is None else acc + y
            return accs[t]

        pr, first, mixed, accs = {}, {}, {}, {}
        acc, nxt = None, 0
        for t in range(H + D1 + D2):
            u = t - D1 - D2
            if FIN and t == FAT:
                fill(it, k, range(FS - FIN, FS))
            for ch in ORDERS[ORDER]:
                if ch in "qkv":
                    if t < H:
                        project(t, "qkv".index(ch))
                elif ch == "s":
                    if t in side_at and (SIDE >> side_at[t]) & 1:
                        j = side_at[t]
                        tok = side_work(j)
                        if j == 2 and LNFREE and k + 1 < UNROLL:
                            pass
                        elif po[j] >= 0:
                            odue.setdefault(po[j], []).extend(tok)
                        else:
                            due[t + SDUE] = tok
                    if 0 <= t - D1 < H:
                        pr[t - D1] = probs(t - D1)
                elif ch == "x":
                    if NV and 0 <= t - DV < H:
                        first[t - DV] = first_rows(t - DV)
                elif 0 <= u < H:
                    if NV and u not in first:
                        first[u] = first_rows(u)
                    mixed[u] = mix(u)
            if t >= H or nxt < OSTART:
                for _ in range(OTAIL if t >= H else 1):
                    if nxt <= u - D3:
                        acc = project_out(mixed[nxt], nxt, acc)
                        nxt += 1
        while nxt < H:
            acc = project_out(mixed[nxt], nxt, acc)
            nxt += 1
        mem[...] = acc[0:MEM]
        ybuf[k % LAG] = acc[MEM:]

    def fill(it, k, es):
        for e in es:
            n = (it * UNROLL + k) * FS + e
            project_extra(tab[2 * n], tab[2 * n + 1], FG)

    def out_copy(first, count):
        return pltpu.make_async_copy(obuf.at[pl.ds(first, count)], out_hbm.at[pl.ds(first, count)],
                                     sem_out.at[0])

    def block(it, carry):
        if INLOOP:
            pl.when(it == 0)(prologue)
        with _scope("blk"):
            for k in range(UNROLL):
                if FILL:
                    fill(it, k, range(FS - OV.get(("FIN", k), FIN)))
                step(it, k)

        if OUTLOOP:
            @pl.when(it == 0)
            def _():
                out_copy(0, UNROLL - LAG).start()

            @pl.when(it > 0)
            def _():
                out_copy(it * UNROLL - LAG, UNROLL).start()

        if EPIIN:
            pl.when(it == nblk - 1)(epilogue)
        return carry

    nblk = NSEG // UNROLL

    sub = lax.broadcasted_iota(I32, (8, 1), 0)
    last = NSEG * SEG - 1

    def select(b1, b2):
        k1 = jnp.max(b1, axis=0, keepdims=True)
        k2 = jnp.max(jnp.where(b1 == k1, b2, b1), axis=0, keepdims=True)
        return k1[0, 0], k2[0, 0]

    def place(key):
        n = last - (key & last)
        r = n & (SEG - 1)
        return n >> 5, r, pl.multiple_of(r & -PR, PR)

    def ffn(k1, k2):
        (s1, r1, _), (s2, r2, _) = place(k1), place(k2)
        xsel = jnp.where(sub == 0, hh[s1, pl.ds(SEG + r1, 1), :],
                         jnp.where(sub == 1, hh[s2, pl.ds(SEG + r2, 1), :], 0.0))
        g = _rb(_dot(xsel, pltpu.bitcast(wg[...], BF)))
        g = _rb(g * jax.nn.sigmoid(g))
        u = _rb(_dot(xsel, pltpu.bitcast(wu[...], BF)))
        return _rb(_dot(_rb(g * u), pltpu.bitcast(wd[...], BF)))

    def patch(y, k1, k2):
        hi = jnp.where(lax.broadcasted_iota(I32, (8, DH), 0) == 0, k1, k2) & -65536
        gate = _rb(jax.nn.sigmoid(lax.bitcast_convert_type(hi ^ ((hi >> 31) & FLIP), F32)))
        y = _rb(y * jnp.concatenate([gate] * NCB, axis=1))
        for j, key in enumerate((k1, k2)):
            s, _, g = place(key)
            back = (last - s * SEG - g) - lax.broadcasted_iota(I32, (PR, 1), 0)
            upd = jnp.where(back == (k1 & last), y[0:1], jnp.where(back == (k2 & last), y[1:2], 0.0))
            pbuf[j] = (hh[s, pl.ds(g, PR), :] + _rb(hh[s, pl.ds(SEG + g, PR), :] + upd)).astype(BF)

    def epilogue():
        with _scope("e_w"):
            wg_copy.wait()
            wu_copy.wait()
            wd_copy.wait()
        m1, m2 = select(top[0], top[1])
        y = ffn(m1, m2)
        for g in range(NSEG - LAG, NSEG):
            c1, c2 = finish_rows(g, ybuf[g % LAG], 0, SEG, None, g + 1 < NSEG)
        out_copy(NSEG - LAG, LAG).start()
        k1, k2 = select(c1, c2)
        patch(y, k1, k2)

        @pl.when((k1 != m1) | (k2 != m2))
        def _():
            patch(ffn(k1, k2), k1, k2)

        out_copy(0, NSEG).wait()
        (s1, _, g1), (s2, _, g2) = place(k1), place(k2)
        cp1 = pltpu.make_async_copy(pbuf.at[0], out_hbm.at[s1, pl.ds(g1, PR), :], sem_out.at[0])
        cp2 = pltpu.make_async_copy(pbuf.at[1], out_hbm.at[s2, pl.ds(g2, PR), :], sem_out.at[1])
        cp1.start()

        @pl.when((s2 != s1) | (g2 != g1))
        def _():
            cp2.start()
            cp2.wait()

        cp1.wait()

    lax.fori_loop(0, nblk, block, 0)
    if not EPIIN:
        epilogue()


@functools.partial(jax.jit, static_argnames=("A_seg_len",))
def pallas_sequential_preLN__memory_aug_recurrent_mem_tr__moe_arch_mod__prompt_kernel(
    A_x, A_mem0, A_Wq, A_Wk, A_Wv, A_Wo, A_seg_len, B_x, B_w_r, B_w_gate, B_w_up, B_w_down,
):
    del B_x
    assert A_seg_len == SEG and A_x.shape == (1, NSEG * SEG, DM) and A_mem0.shape == (1, MEM, DM)
    assert A_Wq.shape == (DM, H, DH) and A_Wo.shape == (H, DH, DM) and B_w_gate.shape == (DM, DFF)
    vmem = pltpu.VMEM
    out = pl.pallas_call(
        _kernel,
        out_shape=jax.ShapeDtypeStruct((NSEG, SEG, DM), BF),
        in_specs=[pl.BlockSpec(memory_space=pl.ANY)] * 10,
        out_specs=pl.BlockSpec(memory_space=pl.ANY),
        scratch_shapes=[
            vmem((3 * H, DM // 2, DH), U32),
            vmem((H * DH // 2, DM), U32),
            vmem((NSEG, 3 * H, XR, DH), F32),
            vmem((H, 3, STR, DH), F32),
            vmem((3 * H // 2, 2, DM // 2, DH), U32),
            vmem((NSEG, 2 * SEG, DM), F32),
            vmem((NSEG, SEG, DM), BF),
            vmem((NSEG, SEG, DM), BF),
            vmem((DM // 2, DFF), U32),
            vmem((DM // 2, DFF), U32),
            vmem((DFF // 2, DM), U32),
            vmem((NSEG * XR, DM), F32),
            vmem((LAG, SEG, DM), F32),
            vmem((2, SEG, 1), I32),
            vmem((XS, DM), F32),
            vmem(((MEM + XS) // 2 + 8, DM), U32),
            vmem((MEM, DM), F32),
            vmem((XS, DM), BF),
            vmem((2, PR, DM), BF),
            vmem((MEM, DM), BF),
            vmem((WRP,), BF),
            pltpu.SMEM((2 * NSEG * FS,), I32),
            pltpu.SemaphoreType.DMA((NCH,)),
            pltpu.SemaphoreType.DMA((11,)),
            pltpu.SemaphoreType.DMA((2,)),
        ],
        compiler_params=pltpu.CompilerParams(
            vmem_limit_bytes=110 * 1024 * 1024,
            disable_bounds_checks=bool(NOBC), disable_semaphore_checks=bool(NOSC)),
    )(
        A_x.reshape(NSEG, SEG, DM), A_mem0.reshape(MEM, DM),
        *(w.reshape(DM // 2, 2, H, DH) for w in (A_Wq, A_Wk, A_Wv)),
        A_Wo.reshape(H * DH, DM), B_w_r, B_w_gate, B_w_up, B_w_down,
    )
    return out.reshape(1, NSEG * SEG, DM)
```

```python
import functools
import math

import jax
import jax.numpy as jnp
from jax import lax
import jax.experimental.pallas as pl
import jax.experimental.pallas.tpu as pltpu

BF = jnp.bfloat16
F32 = jnp.float32
U32 = jnp.uint32
I32 = jnp.int32

H, DH, DM, MEM, SEG, NSEG, DFF = 32, 128, 512, 8, 32, 64, 1792
L = MEM + SEG
XR = 8
XS = SEG - XR
GH = 8
NCH = 3 * H // GH
NCB = DM // DH
UNROLL = 8
FILL = 1
D1, D2, D3, OTAIL = 4, 4, 2, 4
TOK = 1
NEARLY = 8
FG = 4
FS = 4
INITFIRST = 0
PAIRB = 1
NA = 6
QM = 0
STR = 32
OUTLOOP = 1
QBF = 0
PBF = 1
S0, S1, S2, SDUE = 0, 1, 2, 2
PO0, PO1, PO2 = -1, -1, -1
LNFREE = 0
LAG = 1
PINW = 0
NOBC = 1
PLAN = 0
PLANS = (((1, 2, 3, 6), 9, 3), ((1, 2, 1, 4), 8, 3), ((1, 2, 3), 6, 3), ((1, 2, 3, 2), 8, 3), ((1, 2, 3, 6), 12, 4),
         ((1, 2, 3, 6), 6, 2), ((1, 2, 3, 6, 10), 13, 0), ((1, 2, 3, 6, 8), 14, 1), ((1, 2, 3, 6, 9), 9, 1))
NP0 = 32
NP1 = 40
FFNAT = -1
ONEP = 0
APIN = 0
HZ = 0
PR = 8
PYLOOP = 0
NSH = 2
PVI = 0
QI = 0
SPL = 16
OV = {('FAT', 0): 1, ('FIN', 0): 4, ('MERGE', 0): 2, ('PD', 0): 1, ('RB', 0): 2, ('S2', 0): 26, ('SDUE', 0): 3, ('CH2', 1): 2, ('LNFREE', 1): 1, ('PO2', 1): 28, ('CH1', 2): 1, ('PD', 2): 3, ('XREV', 2): 1, ('CH1', 3): 2, ('PINW', 3): 1, ('PO2', 3): 24, ('XREV', 3): 1, ('CH1', 4): 2, ('LNFREE', 4): 1, ('PO2', 4): 28, ('QI', 4): 1, ('LNFREE', 5): 1, ('PINW', 5): 1, ('PO2', 5): 28, ('ORDER', 6): 7, ('CH2', 7): 4, ('LNFREE', 7): 1, ('PD', 7): 1, ('PO2', 7): 28, ('PVI', 7): 2}
FIN = 0
FAT = 6
INLOOP = 1
EPIIN = 0
WRP = 2048
RB = 1
TAB = 1
CH0, CH1, CH2 = 0, 0, 0
AEV = 1
NOSC = 1
NV = 1
DV = 5
PD = 2
ORDER = 10
KBF = 0
MERGE = 0
XREV = 0
SUMPIN = 0
VBF = 0
NPIN = 0
OSTART = 0
ORDERS = ("kvqspx", "qkvsxp", "kqsvpx", "qkvspx", "kvsqpx", "kpvsqx", "skvpqx", "xkvqsp", "kxvsqp", "vkqpsx", "pkvqsx", "kvxqps")
SIDE = 7
SCOPES = 0
EPS = 1e-5
SCALE = 0.08837890625
C2 = SCALE * math.log2(math.e)
NEG = -1e9 / SCALE
LOWEST = -2 ** 31
FLIP = 0x7FFF0000


def _dot(a, b):
    return lax.dot_general(a, b, (((1,), (0,)), ((), ())), preferred_element_type=F32)


def _dot_t(a, b):
    return lax.dot_general(a, b, (((1,), (1,)), ((), ())), preferred_element_type=F32)


def _rb(x):
    return x.astype(BF).astype(F32)


def _layernorm(x):
    n = x.shape[-1]
    mean = jnp.sum(x, axis=-1, keepdims=True) * (1.0 / n)
    xc = x - mean
    var = jnp.sum(xc * xc, axis=-1, keepdims=True) * (1.0 / n)
    den = _rb(jnp.sqrt(_rb(_rb(var) + EPS)))
    return _rb(_rb(x - _rb(mean)) * (1.0 / den))


def _layernorm_f32(x):
    n = x.shape[-1]
    xc = x - jnp.sum(x, axis=-1, keepdims=True) * (1.0 / n)
    var = jnp.sum(xc * xc, axis=-1, keepdims=True) * (1.0 / n)
    return xc * lax.rsqrt(var + EPS)


def _recip(l):
    r = pl.reciprocal(l, approx=True)
    return r * (2.0 - l * r)


def _tree(f, xs):
    while len(xs) > 1:
        xs = [f(xs[a], xs[a + 1]) if a + 1 < len(xs) else xs[a] for a in range(0, len(xs), 2)]
    return xs[0]


def _chains(f, xs, n):
    if not n:
        return _tree(f, xs)
    return _tree(f, [functools.reduce(f, xs[i::n]) for i in range(n)])


class _NoScope:
    def __enter__(self):
        return self

    def __exit__(self, *a):
        return False


def _scope(name):
    return jax.named_scope(name) if SCOPES else _NoScope()


def _kernel(x_hbm, m0_hbm, wq_hbm, wk_hbm, wv_hbm, wo_hbm, wr_hbm, wg_hbm, wu_hbm, wd_hbm,
            out_hbm,
            wp, wo, ex, st, stage, hh, xs, obuf, wg, wu, wd, xe, ybuf, top, xn, hsb, mem, x0s, pbuf, m0s, wrs,
            tab, sem_w, sem_x, sem_out):
    w_hbm = tuple(w.bitcast(U32) for w in (wq_hbm, wk_hbm, wv_hbm))
    nfill = 2 * FG * XR
    npro = NSEG * XR - nfill

    peel, body, nlong = PLANS[PLAN]
    npair = 3 * H // 2
    p0 = sum(peel)
    nit = (npair - p0) // body
    assert p0 + nit * body == npair
    bounds = [sum(peel[:g]) for g in range(len(peel))] + [p0 + i * body for i in range(nit + 1)]

    left = list(range(p0 - NSH, p0)) + [p0 + i * body + q for i in range(nit) for q in range(nlong, body)]
    assert 2 * len(left) + 6 * H <= (NSEG - FG + 1) * FS
    fill_plan = [(2 * p + e, NSEG - 3 * FG) for p in left for e in range(2)]
    fill_plan += [(j, NSEG - g * FG) for g in (2, 1) for j in range(3 * H)]
    fill_plan += fill_plan[-1:] * (NSEG * FS - len(fill_plan))

    def w_start(ps):
        for p in ps:
            g = max(i for i, b in enumerate(bounds) if b <= p)
            for t in range(2):
                pltpu.make_async_copy(w_hbm[p // (H // 2)].at[:, t, p % (H // 2), :],
                                      stage.at[p, t], sem_w.at[g]).start()

    def w_wait(g, first, n):
        part = stage.at[pl.ds(first, n)]
        pltpu.make_async_copy(part, part, sem_w.at[g]).wait()

    wo_copy = pltpu.make_async_copy(wo_hbm.bitcast(U32), wo, sem_x.at[0])

    half = NSEG // 2

    hx = npro // XR // 2

    def x_copy(j):
        return pltpu.make_async_copy(x_hbm.at[pl.ds(j * hx, hx), pl.ds(XS, XR), :],
                                     xs.at[pl.ds(j * hx, hx), pl.ds(XS, XR), :], sem_x.at[8 + j])

    if nfill:
        xc_copy = pltpu.make_async_copy(x_hbm.at[pl.ds(2 * hx, NSEG - 2 * hx), pl.ds(XS, XR), :],
                                        xs.at[pl.ds(2 * hx, NSEG - 2 * hx), pl.ds(XS, XR), :], sem_x.at[7])

    xr_copy = pltpu.make_async_copy(x_hbm.at[:, pl.ds(0, XS), :], xs.at[:, pl.ds(0, XS), :], sem_x.at[10])
    x0_copy = pltpu.make_async_copy(x_hbm.at[0, pl.ds(0, XS), :], x0s, sem_x.at[1])
    m0_copy = pltpu.make_async_copy(m0_hbm, m0s, sem_x.at[2])
    wr_copy = pltpu.make_async_copy(wr_hbm, wrs.at[pl.ds(0, DM)], sem_x.at[3])
    wg_copy = pltpu.make_async_copy(wg_hbm.bitcast(U32), wg, sem_x.at[4])
    wu_copy = pltpu.make_async_copy(wu_hbm.bitcast(U32), wu, sem_x.at[5])
    wd_copy = pltpu.make_async_copy(wd_hbm.bitcast(U32), wd, sem_x.at[6])

    def repack(p):
        a = stage[p, 0]
        b = stage[p, 1]
        wp[2 * p] = (a & jnp.uint32(0xFFFF)) | (b << 16)
        wp[2 * p + 1] = (a >> 16) | (b & jnp.uint32(0xFFFF0000))

    def w_tile(j):
        return pltpu.bitcast(wp[j], BF)

    def project_extra(j, s0, n):
        r0 = s0 * XR if isinstance(s0, int) else pl.multiple_of(s0 * XR, XR)
        ex[pl.ds(s0, n), j] = _dot(xe[pl.ds(r0, n * XR), :], w_tile(j)).reshape(n, XR, DH)

    def ln_extra(s0, n):
        for g in range(s0, s0 + n):
            v = xs[g, XS:SEG, :].astype(F32)
            xe[g * XR:(g + 1) * XR, :] = _layernorm_f32(v)

    def start_x(j, carry):
        x_copy(j).start()
        return carry

    lax.fori_loop(0, 2, start_x, 0)
    w_start(range(bounds[0], bounds[1]))
    small = (x0_copy, m0_copy, wr_copy, xc_copy)

    def project_pairs(first, count, long, starts=None):
        repack(first)
        if count == 1 and starts is not None:
            starts()
        for i in range(count):
            n = NSEG - (2 if i < long else 3) * FG
            project_extra(2 * (first + i), 0, n)
            if i + 1 < count:
                repack(first + i + 1)
                if i + 2 == count and starts is not None:
                    starts()
            project_extra(2 * (first + i) + 1, 0, n)

    def init_state():
        mem[...] = m0s[...].astype(F32)
        xn[...] = _layernorm_f32(x0s[...].astype(F32))
        if nfill:
            ln_extra(2 * hx, NSEG - 2 * hx)
        ybuf[...] = jnp.zeros((LAG, SEG, DM), F32)
        top[...] = jnp.full((2, SEG, 1), LOWEST, I32)
        if TAB:
            for n, (j, g) in enumerate(fill_plan):
                tab[2 * n] = j
                tab[2 * n + 1] = g

    def _when(c):
        return pl.when(c) if not isinstance(c, bool) else (lambda f: f() if c else None)

    def stage_starts(k):
        @_when(k == 0)
        def _():
            w_start(range(bounds[3], NP0))

        @_when(k == 3)
        def _():
            w_start(range(NP0, NP1))

        @_when(k == 4)
        def _():
            w_start(range(NP1, npair))
            xr_copy.start()

    def pro_loop(i, carry):
        @_when(i == 5 - len(peel))
        def _():
            wo_copy.start()

        def starts():
            if len(peel) == 4:
                _when(i == 0)(functools.partial(stage_starts, 4))

        with _scope("pw"):
            w_wait(len(peel) + i, p0 + i * body, body)
        with _scope("part"):
            project_pairs(p0 + i * body, body, nlong, starts)
        return carry

    def prologue():
        with _scope("wait_xa"):
            x_copy(0).wait()
        w_start(range(bounds[1], bounds[2]))
        with _scope("ln_xa"):
            ln_extra(0, hx)
        with _scope("wait_xb"):
            x_copy(1).wait()
        w_start(range(bounds[2], bounds[3]))
        for cp in small:
            cp.start()
        with _scope("ln_xb"):
            ln_extra(hx, hx)
        with _scope("pro"):
            for g, n in enumerate(peel):
                last = g + 1 == len(peel)
                with _scope("pw"):
                    w_wait(g, bounds[g], n)
                    if last:
                        for cp in small:
                            cp.wait()
                with _scope("p0"):
                    project_pairs(bounds[g], n, n - NSH if last else n, functools.partial(stage_starts, g))
                    if last:
                        init_state()
            lax.fori_loop(0, nit - PYLOOP, pro_loop, 0)
            for i in range(nit - PYLOOP, nit):
                pro_loop(i, 0)
        with _scope("t_start"):
            for cp in (wg_copy, wu_copy, wd_copy):
                cp.start()
        with _scope("t_wait"):
            xr_copy.wait()
            wo_copy.wait()

    if not INLOOP:
        prologue()

    def finish_rows(s, y, r0, n, live, keep=True):
        h = _rb(xs[s, r0:r0 + n, :].astype(F32) + _rb(y))
        hn = _layernorm(h)
        hh[s, r0:r0 + n, :] = h
        hh[s, SEG + r0:SEG + r0 + n, :] = hn
        obuf[s, r0:r0 + n, :] = (h + hn).astype(BF)
        r = _rb(jnp.sum(hn * wrs[pl.ds(0, DM)].astype(F32), axis=-1, keepdims=True))
        b = lax.bitcast_convert_type(r, I32)
        back = (NSEG * SEG - 1 - r0 - s * SEG) - lax.broadcasted_iota(I32, (n, 1), 0)
        key = (b ^ ((b >> 31) & FLIP)) | back
        if live is not None:
            key = jnp.where(live, key, LOWEST)
        b1, b2 = top[0, r0:r0 + n, :], top[1, r0:r0 + n, :]
        new = jnp.maximum(key, b1), jnp.maximum(jnp.minimum(key, b1), b2)
        if keep:
            top[0, r0:r0 + n, :] = new[0]
            top[1, r0:r0 + n, :] = new[1]
        return new

    base = dict(D1=D1, D2=D2, DV=DV, PD=PD, OTAIL=OTAIL, D3=D3, ORDER=ORDER, QBF=QBF, PBF=PBF, VBF=VBF, MERGE=MERGE, XREV=XREV, SUMPIN=SUMPIN, NPIN=NPIN, S0=S0, S1=S1, S2=S2, SDUE=SDUE, PINW=PINW, ONEP=ONEP, APIN=APIN, AEV=AEV, CH0=CH0, CH1=CH1, CH2=CH2, RB=RB, LNFREE=LNFREE, PO2=PO2, FIN=FIN, FAT=FAT, PVI=PVI, QI=QI, SPL=SPL)

    def step(it, k):
        (D1, D2, DV, PD, OTAIL, D3, ORDER, QBF, PBF, VBF, MERGE, XREV, SUMPIN, NPIN, S0, S1, S2, SDUE, PINW, ONEP, APIN, AEV, CH0, CH1, CH2, RB, LNFREE, PO2, FIN, FAT, PVI, QI, SPL) = [OV.get((n, k), v) for n, v in base.items()]
        s = it * UNROLL + k
        row = lax.broadcasted_iota(I32, (L, L), 0)
        col = lax.broadcasted_iota(I32, (L, L), 1)
        mask = (row < MEM) | (row >= col)
        hs = jnp.concatenate([mem[...], xn[...]], axis=0).astype(BF)
        hrows = (MEM + XS) // 2
        zz = pl.multiple_of(jnp.minimum(s, 0), 8)
        if HZ:
            hsb[pl.ds(zz, hrows), :] = pltpu.bitcast(hs, U32)

        def lhs(i):
            if not HZ:
                return hs
            if i and i % HZ == 0:
                hsb[pl.ds(zz + hrows, 8), 0:DH] = jnp.zeros((8, DH), U32)
            return pltpu.bitcast(hsb[0:hrows, :], BF)

        s0 = pl.multiple_of(it * UNROLL, UNROLL)
        prev = s0 + (k - LAG) if k >= LAG else jnp.maximum(s - LAG, 0)
        succ = s0 + (k + 1) if k + 1 < UNROLL else jnp.minimum(s + 1, NSEG - 1)
        yprev = ybuf[k % LAG]
        never = s < 0
        zero = jnp.minimum(s, 0)
        e0 = pl.multiple_of(it * (UNROLL * XR), UNROLL * XR) + k * XR

        def side_work(j):
            if j < 2:
                if ONEP and j == 1:
                    return []
                for i in range(2) if ONEP == 1 else [j]:
                    if ONEP == 2:
                        finish_rows(prev, yprev, 0, SEG, None if k >= LAG else s >= LAG)
                    else:
                        finish_rows(prev, yprev[16 * i:16 * i + 16], 16 * i, 16, None if k >= LAG else s >= LAG)
                if not TOK:
                    return None
                z8 = pl.multiple_of(zero, 8)
                z16 = pl.multiple_of(zero, 16)
                toks = [hh[prev, pl.ds(z8, 8), 0:DH], top[0, pl.ds(z8, 8), :].astype(F32),
                        obuf[prev, pl.ds(z16, 16), 0:DH].astype(F32)[0:8]]
                return [toks[0] + toks[1] + toks[2]] if PINW in (0, 3) else toks
            xn[...] = _layernorm_f32(xs[succ, 0:XS, :].astype(F32))
            if not TOK:
                return None
            return [xn[pl.ds(pl.multiple_of(zero, 8), 8), 0:DH]]

        side_at = {S0: 0, S1: 1, S2: 2}
        due = {}
        odue = {}
        po = (PO0, PO1, PO2)

        sub = lax.broadcasted_iota(I32, (8, 1), 0)
        groups = [0] + list(range(1 + NV, L // 8))

        def project(t, m):
            if MERGE:
                if m == 1:
                    ms = (1, 2, 0) if MERGE == 1 else (0, 1, 2)
                    y = _dot(hs, jnp.concatenate([w_tile(a * H + t) for a in ms], axis=1))
                    for i, a in enumerate(ms):
                        st[t, a] = y[:, i * DH:(i + 1) * DH]
                return
            st[t, m] = _dot(lhs(3 * t + ORDERS[ORDER].replace("s", "").replace("p", "").replace("x", "").index("qkv"[m])),
                            w_tile(m * H + t))

        def rows(t, m, gs):
            return [ex[s, m * H + t] if g == L // 8 - 1 else st[t, m, 8 * g:8 * g + 8, :] for g in gs]

        def probs(t):
            q = rows(t, 0, groups)
            kr = rows(t, 1, range(L // 8))
            for i, tok in enumerate(due.get(t, ())):
                if PINW < 2:
                    q[(-1 - i - QI) % 4] = jnp.where(never, tok, q[(-1 - i - QI) % 4])
                else:
                    kr[-1 - i] = jnp.where(never, tok, kr[-1 - i])
            kk = jnp.concatenate(kr, axis=0)
            if KBF:
                kk = kk.astype(BF)
            mk = jnp.concatenate([mask[8 * g:8 * g + 8] for g in groups], axis=0)
            qq = jnp.concatenate(q, axis=0)
            sc = jnp.where(mk, _dot_t(qq.astype(BF) if QBF else qq, kk), NEG)
            p = jnp.exp2((sc - jnp.max(sc, axis=-1, keepdims=True)) * C2)
            return p, jnp.sum(p, axis=-1, keepdims=True)

        def first_rows(t):
            q = rows(t, 0, [1])[0] * C2
            kk = rows(t, 1, [0, 1])
            vv = rows(t, 2, [0, 1])

            def row(a, j):
                if RB & (1 if a is kk else 2):
                    return jnp.broadcast_to(st[t, 1 if a is kk else 2, j:j + 1, :], (8, DH))
                return jnp.broadcast_to(a[j // 8][j % 8:j % 8 + 1], (8, DH))

            order = list(range(MEM + 8))
            if XREV:
                order = order[::-1]
            sc = {}
            for j in order:
                sj = jnp.sum(q * row(kk, j), axis=-1, keepdims=True)
                sc[j] = jnp.where(sub >= j - MEM, sj, NEG * C2) if j > MEM else sj
            sc = [sc[j] for j in range(MEM + 8)]
            mx = _chains(jnp.maximum, sc, CH0)
            p = [jnp.exp2(sj - mx) for sj in sc]
            o = _chains(jnp.add, [p[j] * row(vv, j) for j in range(MEM + 8)], CH1)
            return o * _recip(_chains(jnp.add, p, CH2))

        def mix(t):
            p, l = pr[t]
            v = rows(t, 2, range(L // 8))
            if NV and t - PD >= 0:
                v[PVI] = jnp.where(never, first[t - PD], v[PVI])
            if NPIN and t - NPIN >= 0:
                v[2] = jnp.where(never, _tree(jnp.add, [mixed[t - NPIN][8 * g:8 * g + 8] for g in groups]), v[2])
            if SUMPIN and t - SUMPIN >= 0:
                ls = pr[t - SUMPIN][1]
                v[3] = jnp.where(never, _tree(jnp.add, [ls[8 * g:8 * g + 8] for g in range(len(groups))]), v[3])
            vv = jnp.concatenate(v, axis=0)
            o = _dot(p.astype(BF) if PBF else p, vv.astype(BF) if VBF else vv) * _recip(l)
            return jnp.concatenate([o[0:MEM], first[t], o[MEM:]], axis=0) if NV else o

        def project_out(o, t, acc):
            for tok in odue.get(t, ()):
                o = jnp.concatenate([jnp.where(never, tok, o[0:8]), o[8:]], axis=0)
            if APIN and t - APIN >= 1 and t % AEV == 0:
                a = accs[t - APIN]
                o = jnp.where(never, _tree(jnp.add, [a[:, c * DH:(c + 1) * DH] for c in range(NCB)]), o)
            y = _dot(o, pltpu.bitcast(wo[t * (DH // 2):(t + 1) * (DH // 2), :], BF))
            accs[t] = y if acc is None else acc + y
            return accs[t]

        pr, first, mixed, accs = {}, {}, {}, {}
        acc, nxt = None, 0
        for t in range(H + D1 + D2):
            u = t - D1 - D2
            if FIN and t == FAT:
                fill(it, k, range(FS - FIN, FS))
            for ch in ORDERS[ORDER]:
                if ch in "qkv":
                    if t < H:
                        project(t, "qkv".index(ch))
                elif ch == "s":
                    if t in side_at and (SIDE >> side_at[t]) & 1:
                        j = side_at[t]
                        tok = side_work(j)
                        if j == 2 and LNFREE and k + 1 < UNROLL:
                            pass
                        elif po[j] >= 0:
                            odue.setdefault(po[j], []).extend(tok)
                        else:
                            due[t + SDUE] = tok
                    if 0 <= t - D1 < H:
                        pr[t - D1] = probs(t - D1)
                elif ch == "x":
                    if NV and 0 <= t - DV < H:
                        first[t - DV] = first_rows(t - DV)
                elif 0 <= u < H:
                    if NV and u not in first:
                        first[u] = first_rows(u)
                    mixed[u] = mix(u)
            if t >= H or nxt < OSTART:
                for _ in range(OTAIL if t >= H else 1):
                    if nxt <= u - D3:
                        acc = project_out(mixed[nxt], nxt, acc)
                        nxt += 1
        while nxt < H:
            acc = project_out(mixed[nxt], nxt, acc)
            nxt += 1
        mem[...] = acc[0:MEM]
        ybuf[k % LAG] = acc[MEM:]

    def fill(it, k, es):
        for e in es:
            n = (it * UNROLL + k) * FS + e
            project_extra(tab[2 * n], tab[2 * n + 1], FG)

    def out_copy(first, count):
        return pltpu.make_async_copy(obuf.at[pl.ds(first, count)], out_hbm.at[pl.ds(first, count)],
                                     sem_out.at[0])

    def block(it, carry):
        if INLOOP:
            pl.when(it == 0)(prologue)
        with _scope("blk"):
            for k in range(UNROLL):
                if FILL:
                    fill(it, k, range(FS - OV.get(("FIN", k), FIN)))
                step(it, k)

        if OUTLOOP:
            @pl.when(it == 0)
            def _():
                out_copy(0, UNROLL - LAG).start()

            @pl.when(it > 0)
            def _():
                out_copy(it * UNROLL - LAG, UNROLL).start()

        if EPIIN:
            pl.when(it == nblk - 1)(epilogue)
        return carry

    nblk = NSEG // UNROLL

    sub = lax.broadcasted_iota(I32, (8, 1), 0)
    last = NSEG * SEG - 1

    def select(b1, b2):
        k1 = jnp.max(b1, axis=0, keepdims=True)
        k2 = jnp.max(jnp.where(b1 == k1, b2, b1), axis=0, keepdims=True)
        return k1[0, 0], k2[0, 0]

    def place(key):
        n = last - (key & last)
        r = n & (SEG - 1)
        return n >> 5, r, pl.multiple_of(r & -PR, PR)

    def ffn(k1, k2):
        (s1, r1, _), (s2, r2, _) = place(k1), place(k2)
        xsel = jnp.where(sub == 0, hh[s1, pl.ds(SEG + r1, 1), :],
                         jnp.where(sub == 1, hh[s2, pl.ds(SEG + r2, 1), :], 0.0))
        g = _rb(_dot(xsel, pltpu.bitcast(wg[...], BF)))
        g = _rb(g * jax.nn.sigmoid(g))
        u = _rb(_dot(xsel, pltpu.bitcast(wu[...], BF)))
        return _rb(_dot(_rb(g * u), pltpu.bitcast(wd[...], BF)))

    def patch(y, k1, k2):
        hi = jnp.where(lax.broadcasted_iota(I32, (8, DH), 0) == 0, k1, k2) & -65536
        gate = _rb(jax.nn.sigmoid(lax.bitcast_convert_type(hi ^ ((hi >> 31) & FLIP), F32)))
        y = _rb(y * jnp.concatenate([gate] * NCB, axis=1))
        for j, key in enumerate((k1, k2)):
            s, _, g = place(key)
            back = (last - s * SEG - g) - lax.broadcasted_iota(I32, (PR, 1), 0)
            upd = jnp.where(back == (k1 & last), y[0:1], jnp.where(back == (k2 & last), y[1:2], 0.0))
            pbuf[j] = (hh[s, pl.ds(g, PR), :] + _rb(hh[s, pl.ds(SEG + g, PR), :] + upd)).astype(BF)

    def epilogue():
        with _scope("e_w"):
            wg_copy.wait()
            wu_copy.wait()
            wd_copy.wait()
        m1, m2 = select(top[0], top[1])
        y = ffn(m1, m2)
        for g in range(NSEG - LAG, NSEG):
            c1, c2 = finish_rows(g, ybuf[g % LAG], 0, SEG, None, g + 1 < NSEG)
        out_copy(NSEG - LAG, LAG).start()
        k1, k2 = select(c1, c2)
        patch(y, k1, k2)

        @pl.when((k1 != m1) | (k2 != m2))
        def _():
            patch(ffn(k1, k2), k1, k2)

        out_copy(0, NSEG).wait()
        (s1, _, g1), (s2, _, g2) = place(k1), place(k2)
        cp1 = pltpu.make_async_copy(pbuf.at[0], out_hbm.at[s1, pl.ds(g1, PR), :], sem_out.at[0])
        cp2 = pltpu.make_async_copy(pbuf.at[1], out_hbm.at[s2, pl.ds(g2, PR), :], sem_out.at[1])
        cp1.start()

        @pl.when((s2 != s1) | (g2 != g1))
        def _():
            cp2.start()
            cp2.wait()

        cp1.wait()

    lax.fori_loop(0, nblk, block, 0)
    if not EPIIN:
        epilogue()


@functools.partial(jax.jit, static_argnames=("A_seg_len",))
def pallas_sequential_preLN__memory_aug_recurrent_mem_tr__moe_arch_mod__prompt_kernel(
    A_x, A_mem0, A_Wq, A_Wk, A_Wv, A_Wo, A_seg_len, B_x, B_w_r, B_w_gate, B_w_up, B_w_down,
):
    del B_x
    assert A_seg_len == SEG and A_x.shape == (1, NSEG * SEG, DM) and A_mem0.shape == (1, MEM, DM)
    assert A_Wq.shape == (DM, H, DH) and A_Wo.shape == (H, DH, DM) and B_w_gate.shape == (DM, DFF)
    vmem = pltpu.VMEM
    out = pl.pallas_call(
        _kernel,
        out_shape=jax.ShapeDtypeStruct((NSEG, SEG, DM), BF),
        in_specs=[pl.BlockSpec(memory_space=pl.ANY)] * 10,
        out_specs=pl.BlockSpec(memory_space=pl.ANY),
        scratch_shapes=[
            vmem((3 * H, DM // 2, DH), U32),
            vmem((H * DH // 2, DM), U32),
            vmem((NSEG, 3 * H, XR, DH), F32),
            vmem((H, 3, STR, DH), F32),
            vmem((3 * H // 2, 2, DM // 2, DH), U32),
            vmem((NSEG, 2 * SEG, DM), F32),
            vmem((NSEG, SEG, DM), BF),
            vmem((NSEG, SEG, DM), BF),
            vmem((DM // 2, DFF), U32),
            vmem((DM // 2, DFF), U32),
            vmem((DFF // 2, DM), U32),
            vmem((NSEG * XR, DM), F32),
            vmem((LAG, SEG, DM), F32),
            vmem((2, SEG, 1), I32),
            vmem((XS, DM), F32),
            vmem(((MEM + XS) // 2 + 8, DM), U32),
            vmem((MEM, DM), F32),
            vmem((XS, DM), BF),
            vmem((2, PR, DM), BF),
            vmem((MEM, DM), BF),
            vmem((WRP,), BF),
            pltpu.SMEM((2 * NSEG * FS,), I32),
            pltpu.SemaphoreType.DMA((NCH,)),
            pltpu.SemaphoreType.DMA((11,)),
            pltpu.SemaphoreType.DMA((2,)),
        ],
        compiler_params=pltpu.CompilerParams(
            vmem_limit_bytes=110 * 1024 * 1024,
            disable_bounds_checks=bool(NOBC), disable_semaphore_checks=bool(NOSC)),
    )(
        A_x.reshape(NSEG, SEG, DM), A_mem0.reshape(MEM, DM),
        *(w.reshape(DM // 2, 2, H, DH) for w in (A_Wq, A_Wk, A_Wv)),
        A_Wo.reshape(H * DH, DM), B_w_r, B_w_gate, B_w_up, B_w_down,
    )
    return out.reshape(1, NSEG * SEG, DM)
```

```python
import functools
import math

import jax
import jax.numpy as jnp
from jax import lax
import jax.experimental.pallas as pl
import jax.experimental.pallas.tpu as pltpu

BF = jnp.bfloat16
F32 = jnp.float32
U32 = jnp.uint32
I32 = jnp.int32

H, DH, DM, MEM, SEG, NSEG, DFF = 32, 128, 512, 8, 32, 64, 1792
L = MEM + SEG
XR = 8
XS = SEG - XR
NCB = DM // DH
UNROLL = 8
FG = 4
FS = 4
PEEL, BODY, NLONG, NSH = (1, 2, 3, 6), 9, 3, 2
NP0, NP1 = 32, 40
PR = 8

ORDERS = ("kvqspx", "qkvsxp", "kqsvpx", "qkvspx", "kvsqpx", "kpvsqx", "skvpqx", "xkvqsp", "kxvsqp", "vkqpsx",
          "pkvqsx", "kvxqps")
LAYOUT = dict(D1=4, D2=4, DV=5, PD=2, OTAIL=4, D3=2, ORDER=10, QBF=0, PBF=1, VBF=0, MERGE=0, XREV=0,
              NPIN=0, S0=0, S1=1, S2=2, SDUE=2, PINW=0, ONEP=0, APIN=0, AEV=1, CH0=0, CH1=0, CH2=0,
              RB=1, LNFREE=0, PO2=-1, FIN=0, FAT=6, PVI=0, QI=0)
STEP_LAYOUT = (
    dict(FAT=1, FIN=4, MERGE=2, PD=1, RB=2, S2=26, SDUE=3),
    dict(CH2=2, LNFREE=1, PO2=28),
    dict(CH1=1, PD=3, XREV=1),
    dict(CH1=2, PINW=1, PO2=24, XREV=1),
    dict(CH1=2, LNFREE=1, PO2=28, QI=1),
    dict(LNFREE=1, PINW=1, PO2=28),
    dict(ORDER=7),
    dict(CH2=4, LNFREE=1, PD=1, PO2=28, PVI=2),
)

EPS = 1e-5
SCALE = 0.08837890625
C2 = SCALE * math.log2(math.e)
NEG = -1e9 / SCALE
LOWEST = -2 ** 31
FLIP = 0x7FFF0000


def _dot(a, b):
    return lax.dot_general(a, b, (((1,), (0,)), ((), ())), preferred_element_type=F32)


def _dot_t(a, b):
    return lax.dot_general(a, b, (((1,), (1,)), ((), ())), preferred_element_type=F32)


def _rb(x):
    return x.astype(BF).astype(F32)


def _layernorm(x):
    n = x.shape[-1]
    mean = jnp.sum(x, axis=-1, keepdims=True) * (1.0 / n)
    xc = x - mean
    var = jnp.sum(xc * xc, axis=-1, keepdims=True) * (1.0 / n)
    den = _rb(jnp.sqrt(_rb(_rb(var) + EPS)))
    return _rb(_rb(x - _rb(mean)) * (1.0 / den))


def _layernorm_f32(x):
    n = x.shape[-1]
    xc = x - jnp.sum(x, axis=-1, keepdims=True) * (1.0 / n)
    var = jnp.sum(xc * xc, axis=-1, keepdims=True) * (1.0 / n)
    return xc * lax.rsqrt(var + EPS)


def _recip(l):
    r = pl.reciprocal(l, approx=True)
    return r * (2.0 - l * r)


def _tree(f, xs):
    while len(xs) > 1:
        xs = [f(xs[a], xs[a + 1]) if a + 1 < len(xs) else xs[a] for a in range(0, len(xs), 2)]
    return xs[0]


def _chains(f, xs, n):
    if not n:
        return _tree(f, xs)
    return _tree(f, [functools.reduce(f, xs[i::n]) for i in range(n)])


def _kernel(x_hbm, m0_hbm, wq_hbm, wk_hbm, wv_hbm, wo_hbm, wr_hbm, wg_hbm, wu_hbm, wd_hbm,
            out_hbm,
            wp, wo, ex, st, stage, hh, xs, obuf, wg, wu, wd, xe, ybuf, top, xn, mem, x0s, pbuf, m0s, wrs,
            tab, sem_w, sem_x, sem_out):
    w_hbm = tuple(w.bitcast(U32) for w in (wq_hbm, wk_hbm, wv_hbm))
    peel, body, nlong = PEEL, BODY, NLONG
    npair = 3 * H // 2
    p0 = sum(peel)
    nit = (npair - p0) // body
    assert p0 + nit * body == npair
    bounds = [sum(peel[:g]) for g in range(len(peel))] + [p0 + i * body for i in range(nit + 1)]

    left = list(range(p0 - NSH, p0)) + [p0 + i * body + q for i in range(nit) for q in range(nlong, body)]
    assert 2 * len(left) + 6 * H <= (NSEG - FG + 1) * FS
    fill_plan = [(2 * p + e, NSEG - 3 * FG) for p in left for e in range(2)]
    fill_plan += [(j, NSEG - g * FG) for g in (2, 1) for j in range(3 * H)]
    fill_plan += fill_plan[-1:] * (NSEG * FS - len(fill_plan))

    def w_start(ps):
        for p in ps:
            g = max(i for i, b in enumerate(bounds) if b <= p)
            for t in range(2):
                pltpu.make_async_copy(w_hbm[p // (H // 2)].at[:, t, p % (H // 2), :],
                                      stage.at[p, t], sem_w.at[g]).start()

    def w_wait(g, first, n):
        part = stage.at[pl.ds(first, n)]
        pltpu.make_async_copy(part, part, sem_w.at[g]).wait()

    wo_copy = pltpu.make_async_copy(wo_hbm.bitcast(U32), wo, sem_x.at[0])

    hx = (NSEG - 2 * FG) // 2

    def x_copy(j):
        return pltpu.make_async_copy(x_hbm.at[pl.ds(j * hx, hx), pl.ds(XS, XR), :],
                                     xs.at[pl.ds(j * hx, hx), pl.ds(XS, XR), :], sem_x.at[8 + j])

    xc_copy = pltpu.make_async_copy(x_hbm.at[pl.ds(2 * hx, NSEG - 2 * hx), pl.ds(XS, XR), :],
                                    xs.at[pl.ds(2 * hx, NSEG - 2 * hx), pl.ds(XS, XR), :], sem_x.at[7])
    xr_copy = pltpu.make_async_copy(x_hbm.at[:, pl.ds(0, XS), :], xs.at[:, pl.ds(0, XS), :], sem_x.at[10])
    x0_copy = pltpu.make_async_copy(x_hbm.at[0, pl.ds(0, XS), :], x0s, sem_x.at[1])
    m0_copy = pltpu.make_async_copy(m0_hbm, m0s, sem_x.at[2])
    wr_copy = pltpu.make_async_copy(wr_hbm, wrs.at[pl.ds(0, DM)], sem_x.at[3])
    wg_copy = pltpu.make_async_copy(wg_hbm.bitcast(U32), wg, sem_x.at[4])
    wu_copy = pltpu.make_async_copy(wu_hbm.bitcast(U32), wu, sem_x.at[5])
    wd_copy = pltpu.make_async_copy(wd_hbm.bitcast(U32), wd, sem_x.at[6])

    def repack(p):
        a = stage[p, 0]
        b = stage[p, 1]
        wp[2 * p] = (a & jnp.uint32(0xFFFF)) | (b << 16)
        wp[2 * p + 1] = (a >> 16) | (b & jnp.uint32(0xFFFF0000))

    def w_tile(j):
        return pltpu.bitcast(wp[j], BF)

    def project_extra(j, s0, n):
        r0 = s0 * XR if isinstance(s0, int) else pl.multiple_of(s0 * XR, XR)
        ex[pl.ds(s0, n), j] = _dot(xe[pl.ds(r0, n * XR), :], w_tile(j)).reshape(n, XR, DH)

    def ln_extra(s0, n):
        for g in range(s0, s0 + n):
            v = xs[g, XS:SEG, :].astype(F32)
            xe[g * XR:(g + 1) * XR, :] = _layernorm_f32(v)

    def start_x(j, carry):
        x_copy(j).start()
        return carry

    lax.fori_loop(0, 2, start_x, 0)
    w_start(range(bounds[0], bounds[1]))
    small = (x0_copy, m0_copy, wr_copy, xc_copy)

    def project_pairs(first, count, long, starts=None):
        repack(first)
        if count == 1 and starts is not None:
            starts()
        for i in range(count):
            n = NSEG - (2 if i < long else 3) * FG
            project_extra(2 * (first + i), 0, n)
            if i + 1 < count:
                repack(first + i + 1)
                if i + 2 == count and starts is not None:
                    starts()
            project_extra(2 * (first + i) + 1, 0, n)

    def init_state():
        mem[...] = m0s[...].astype(F32)
        xn[...] = _layernorm_f32(x0s[...].astype(F32))
        ln_extra(2 * hx, NSEG - 2 * hx)
        ybuf[...] = jnp.zeros((1, SEG, DM), F32)
        top[...] = jnp.full((2, SEG, 1), LOWEST, I32)
        for n, (j, g) in enumerate(fill_plan):
            tab[2 * n] = j
            tab[2 * n + 1] = g

    def stage_starts(k):
        if k == 0:
            w_start(range(bounds[3], NP0))
        if k == 3:
            w_start(range(NP0, NP1))
        if k == 4:
            w_start(range(NP1, npair))
            xr_copy.start()

    def pro_loop(i, carry):
        @pl.when(i == 1)
        def _():
            wo_copy.start()

        def starts():
            pl.when(i == 0)(functools.partial(stage_starts, 4))

        w_wait(len(peel) + i, p0 + i * body, body)
        project_pairs(p0 + i * body, body, nlong, starts)
        return carry

    def prologue():
        x_copy(0).wait()
        w_start(range(bounds[1], bounds[2]))
        ln_extra(0, hx)
        x_copy(1).wait()
        w_start(range(bounds[2], bounds[3]))
        for cp in small:
            cp.start()
        ln_extra(hx, hx)
        for g, n in enumerate(peel):
            last = g + 1 == len(peel)
            w_wait(g, bounds[g], n)
            if last:
                for cp in small:
                    cp.wait()
            project_pairs(bounds[g], n, n - NSH if last else n, functools.partial(stage_starts, g))
            if last:
                init_state()
        lax.fori_loop(0, nit, pro_loop, 0)
        for cp in (wg_copy, wu_copy, wd_copy):
            cp.start()
        xr_copy.wait()
        wo_copy.wait()

    def finish_rows(s, y, r0, n, live, keep=True):
        h = _rb(xs[s, r0:r0 + n, :].astype(F32) + _rb(y))
        hn = _layernorm(h)
        hh[s, r0:r0 + n, :] = h
        hh[s, SEG + r0:SEG + r0 + n, :] = hn
        obuf[s, r0:r0 + n, :] = (h + hn).astype(BF)
        r = _rb(jnp.sum(hn * wrs[pl.ds(0, DM)].astype(F32), axis=-1, keepdims=True))
        b = lax.bitcast_convert_type(r, I32)
        back = (NSEG * SEG - 1 - r0 - s * SEG) - lax.broadcasted_iota(I32, (n, 1), 0)
        key = (b ^ ((b >> 31) & FLIP)) | back
        if live is not None:
            key = jnp.where(live, key, LOWEST)
        b1, b2 = top[0, r0:r0 + n, :], top[1, r0:r0 + n, :]
        new = jnp.maximum(key, b1), jnp.maximum(jnp.minimum(key, b1), b2)
        if keep:
            top[0, r0:r0 + n, :] = new[0]
            top[1, r0:r0 + n, :] = new[1]
        return new

    def step(it, k):
        (D1, D2, DV, PD, OTAIL, D3, ORDER, QBF, PBF, VBF, MERGE, XREV, NPIN, S0, S1, S2, SDUE, PINW, ONEP,
         APIN, AEV, CH0, CH1, CH2, RB, LNFREE, PO2, FIN, FAT, PVI, QI) = {**LAYOUT,
         **STEP_LAYOUT[k]}.values()
        s = it * UNROLL + k
        row = lax.broadcasted_iota(I32, (L, L), 0)
        col = lax.broadcasted_iota(I32, (L, L), 1)
        mask = (row < MEM) | (row >= col)
        hs = jnp.concatenate([mem[...], xn[...]], axis=0).astype(BF)
        s0 = pl.multiple_of(it * UNROLL, UNROLL)
        prev = s0 + (k - 1) if k else jnp.maximum(s - 1, 0)
        succ = s0 + (k + 1) if k + 1 < UNROLL else jnp.minimum(s + 1, NSEG - 1)
        yprev = ybuf[0]
        never = s < 0
        zero = jnp.minimum(s, 0)

        def side_work(j):
            if j < 2:
                if ONEP and j == 1:
                    return []
                for i in range(2) if ONEP == 1 else [j]:
                    if ONEP == 2:
                        finish_rows(prev, yprev, 0, SEG, None if k else s >= 1)
                    else:
                        finish_rows(prev, yprev[16 * i:16 * i + 16], 16 * i, 16, None if k else s >= 1)
                z8 = pl.multiple_of(zero, 8)
                z16 = pl.multiple_of(zero, 16)
                toks = [hh[prev, pl.ds(z8, 8), 0:DH], top[0, pl.ds(z8, 8), :].astype(F32),
                        obuf[prev, pl.ds(z16, 16), 0:DH].astype(F32)[0:8]]
                return [toks[0] + toks[1] + toks[2]] if not PINW else toks
            xn[...] = _layernorm_f32(xs[succ, 0:XS, :].astype(F32))
            return [xn[pl.ds(pl.multiple_of(zero, 8), 8), 0:DH]]

        side_at = {S0: 0, S1: 1, S2: 2}
        due = {}
        odue = {}

        sub = lax.broadcasted_iota(I32, (8, 1), 0)
        groups = [0] + list(range(2, L // 8))

        def project(t, m):
            if MERGE:
                if m == 1:
                    ms = (1, 2, 0) if MERGE == 1 else (0, 1, 2)
                    y = _dot(hs, jnp.concatenate([w_tile(a * H + t) for a in ms], axis=1))
                    for i, a in enumerate(ms):
                        st[t, a] = y[:, i * DH:(i + 1) * DH]
                return
            st[t, m] = _dot(hs, w_tile(m * H + t))

        def rows(t, m, gs):
            return [ex[s, m * H + t] if g == L // 8 - 1 else st[t, m, 8 * g:8 * g + 8, :] for g in gs]

        def probs(t):
            q = rows(t, 0, groups)
            kk = jnp.concatenate(rows(t, 1, range(L // 8)), axis=0)
            for i, tok in enumerate(due.get(t, ())):
                q[(-1 - i - QI) % 4] = jnp.where(never, tok, q[(-1 - i - QI) % 4])
            mk = jnp.concatenate([mask[8 * g:8 * g + 8] for g in groups], axis=0)
            qq = jnp.concatenate(q, axis=0)
            sc = jnp.where(mk, _dot_t(qq.astype(BF) if QBF else qq, kk), NEG)
            p = jnp.exp2((sc - jnp.max(sc, axis=-1, keepdims=True)) * C2)
            return p, jnp.sum(p, axis=-1, keepdims=True)

        def first_rows(t):
            q = rows(t, 0, [1])[0] * C2
            kk = rows(t, 1, [0, 1])
            vv = rows(t, 2, [0, 1])

            def row(a, j):
                if RB & (1 if a is kk else 2):
                    return jnp.broadcast_to(st[t, 1 if a is kk else 2, j:j + 1, :], (8, DH))
                return jnp.broadcast_to(a[j // 8][j % 8:j % 8 + 1], (8, DH))

            order = list(range(MEM + 8))
            if XREV:
                order = order[::-1]
            sc = {}
            for j in order:
                sj = jnp.sum(q * row(kk, j), axis=-1, keepdims=True)
                sc[j] = jnp.where(sub >= j - MEM, sj, NEG * C2) if j > MEM else sj
            sc = [sc[j] for j in range(MEM + 8)]
            mx = _chains(jnp.maximum, sc, CH0)
            p = [jnp.exp2(sj - mx) for sj in sc]
            o = _chains(jnp.add, [p[j] * row(vv, j) for j in range(MEM + 8)], CH1)
            return o * _recip(_chains(jnp.add, p, CH2))

        def mix(t):
            p, l = pr[t]
            v = rows(t, 2, range(L // 8))
            if t - PD >= 0:
                v[PVI] = jnp.where(never, first[t - PD], v[PVI])
            if NPIN and t - NPIN >= 0:
                v[2] = jnp.where(never, _tree(jnp.add, [mixed[t - NPIN][8 * g:8 * g + 8] for g in groups]), v[2])
            vv = jnp.concatenate(v, axis=0)
            o = _dot(p.astype(BF) if PBF else p, vv.astype(BF) if VBF else vv) * _recip(l)
            return jnp.concatenate([o[0:MEM], first[t], o[MEM:]], axis=0)

        def project_out(o, t, acc):
            for tok in odue.get(t, ()):
                o = jnp.concatenate([jnp.where(never, tok, o[0:8]), o[8:]], axis=0)
            if APIN and t - APIN >= 1 and t % AEV == 0:
                a = accs[t - APIN]
                o = jnp.where(never, _tree(jnp.add, [a[:, c * DH:(c + 1) * DH] for c in range(NCB)]), o)
            y = _dot(o, pltpu.bitcast(wo[t * (DH // 2):(t + 1) * (DH // 2), :], BF))
            accs[t] = y if acc is None else acc + y
            return accs[t]

        pr, first, mixed, accs = {}, {}, {}, {}
        acc, nxt = None, 0
        for t in range(H + D1 + D2):
            u = t - D1 - D2
            if FIN and t == FAT:
                fill(it, k, range(FS - FIN, FS))
            for ch in ORDERS[ORDER]:
                if ch in "qkv":
                    if t < H:
                        project(t, "qkv".index(ch))
                elif ch == "s":
                    if t in side_at:
                        j = side_at[t]
                        tok = side_work(j)
                        if j == 2 and LNFREE and k + 1 < UNROLL:
                            pass
                        elif j == 2 and PO2 >= 0:
                            odue[PO2] = tok
                        else:
                            due[t + SDUE] = tok
                    if 0 <= t - D1 < H:
                        pr[t - D1] = probs(t - D1)
                elif ch == "x":
                    if 0 <= t - DV < H:
                        first[t - DV] = first_rows(t - DV)
                elif 0 <= u < H:
                    if u not in first:
                        first[u] = first_rows(u)
                    mixed[u] = mix(u)
            if t >= H:
                for _ in range(OTAIL):
                    if nxt <= u - D3:
                        acc = project_out(mixed[nxt], nxt, acc)
                        nxt += 1
        while nxt < H:
            acc = project_out(mixed[nxt], nxt, acc)
            nxt += 1
        mem[...] = acc[0:MEM]
        ybuf[0] = acc[MEM:]

    def fill(it, k, es):
        for e in es:
            n = (it * UNROLL + k) * FS + e
            project_extra(tab[2 * n], tab[2 * n + 1], FG)

    def out_copy(first, count):
        return pltpu.make_async_copy(obuf.at[pl.ds(first, count)], out_hbm.at[pl.ds(first, count)],
                                     sem_out.at[0])

    def block(it, carry):
        pl.when(it == 0)(prologue)
        for k in range(UNROLL):
            fill(it, k, range(FS - {**LAYOUT, **STEP_LAYOUT[k]}["FIN"]))
            step(it, k)

        @pl.when(it == 0)
        def _():
            out_copy(0, UNROLL - 1).start()

        @pl.when(it > 0)
        def _():
            out_copy(it * UNROLL - 1, UNROLL).start()

        return carry

    nblk = NSEG // UNROLL

    sub = lax.broadcasted_iota(I32, (8, 1), 0)
    last = NSEG * SEG - 1

    def select(b1, b2):
        k1 = jnp.max(b1, axis=0, keepdims=True)
        k2 = jnp.max(jnp.where(b1 == k1, b2, b1), axis=0, keepdims=True)
        return k1[0, 0], k2[0, 0]

    def place(key):
        n = last - (key & last)
        r = n & (SEG - 1)
        return n >> 5, r, pl.multiple_of(r & -PR, PR)

    def ffn(k1, k2):
        (s1, r1, _), (s2, r2, _) = place(k1), place(k2)
        xsel = jnp.where(sub == 0, hh[s1, pl.ds(SEG + r1, 1), :],
                         jnp.where(sub == 1, hh[s2, pl.ds(SEG + r2, 1), :], 0.0))
        g = _rb(_dot(xsel, pltpu.bitcast(wg[...], BF)))
        g = _rb(g * jax.nn.sigmoid(g))
        u = _rb(_dot(xsel, pltpu.bitcast(wu[...], BF)))
        return _rb(_dot(_rb(g * u), pltpu.bitcast(wd[...], BF)))

    def patch(y, k1, k2):
        hi = jnp.where(lax.broadcasted_iota(I32, (8, DH), 0) == 0, k1, k2) & -65536
        gate = _rb(jax.nn.sigmoid(lax.bitcast_convert_type(hi ^ ((hi >> 31) & FLIP), F32)))
        y = _rb(y * jnp.concatenate([gate] * NCB, axis=1))
        for j, key in enumerate((k1, k2)):
            s, _, g = place(key)
            back = (last - s * SEG - g) - lax.broadcasted_iota(I32, (PR, 1), 0)
            upd = jnp.where(back == (k1 & last), y[0:1], jnp.where(back == (k2 & last), y[1:2], 0.0))
            pbuf[j] = (hh[s, pl.ds(g, PR), :] + _rb(hh[s, pl.ds(SEG + g, PR), :] + upd)).astype(BF)

    def epilogue():
        wg_copy.wait()
        wu_copy.wait()
        wd_copy.wait()
        m1, m2 = select(top[0], top[1])
        y = ffn(m1, m2)
        c1, c2 = finish_rows(NSEG - 1, ybuf[0], 0, SEG, None, False)
        out_copy(NSEG - 1, 1).start()
        k1, k2 = select(c1, c2)
        patch(y, k1, k2)

        @pl.when((k1 != m1) | (k2 != m2))
        def _():
            patch(ffn(k1, k2), k1, k2)

        out_copy(0, NSEG).wait()
        (s1, _, g1), (s2, _, g2) = place(k1), place(k2)
        cp1 = pltpu.make_async_copy(pbuf.at[0], out_hbm.at[s1, pl.ds(g1, PR), :], sem_out.at[0])
        cp2 = pltpu.make_async_copy(pbuf.at[1], out_hbm.at[s2, pl.ds(g2, PR), :], sem_out.at[1])
        cp1.start()

        @pl.when((s2 != s1) | (g2 != g1))
        def _():
            cp2.start()
            cp2.wait()

        cp1.wait()

    lax.fori_loop(0, nblk, block, 0)
    epilogue()


@functools.partial(jax.jit, static_argnames=("A_seg_len",))
def pallas_sequential_preLN__memory_aug_recurrent_mem_tr__moe_arch_mod__prompt_kernel(
    A_x, A_mem0, A_Wq, A_Wk, A_Wv, A_Wo, A_seg_len, B_x, B_w_r, B_w_gate, B_w_up, B_w_down,
):
    del B_x
    assert A_seg_len == SEG and A_x.shape == (1, NSEG * SEG, DM) and A_mem0.shape == (1, MEM, DM)
    assert A_Wq.shape == (DM, H, DH) and A_Wo.shape == (H, DH, DM) and B_w_gate.shape == (DM, DFF)
    vmem = pltpu.VMEM
    out = pl.pallas_call(
        _kernel,
        out_shape=jax.ShapeDtypeStruct((NSEG, SEG, DM), BF),
        in_specs=[pl.BlockSpec(memory_space=pl.ANY)] * 10,
        out_specs=pl.BlockSpec(memory_space=pl.ANY),
        scratch_shapes=[
            vmem((3 * H, DM // 2, DH), U32),
            vmem((H * DH // 2, DM), U32),
            vmem((NSEG, 3 * H, XR, DH), F32),
            vmem((H, 3, MEM + XS, DH), F32),
            vmem((3 * H // 2, 2, DM // 2, DH), U32),
            vmem((NSEG, 2 * SEG, DM), F32),
            vmem((NSEG, SEG, DM), BF),
            vmem((NSEG, SEG, DM), BF),
            vmem((DM // 2, DFF), U32),
            vmem((DM // 2, DFF), U32),
            vmem((DFF // 2, DM), U32),
            vmem((NSEG * XR, DM), F32),
            vmem((1, SEG, DM), F32),
            vmem((2, SEG, 1), I32),
            vmem((XS, DM), F32),
            vmem((MEM, DM), F32),
            vmem((XS, DM), BF),
            vmem((2, PR, DM), BF),
            vmem((MEM, DM), BF),
            vmem((4 * DM,), BF),
            pltpu.SMEM((2 * NSEG * FS,), I32),
            pltpu.SemaphoreType.DMA((12,)),
            pltpu.SemaphoreType.DMA((11,)),
            pltpu.SemaphoreType.DMA((2,)),
        ],
        compiler_params=pltpu.CompilerParams(
            vmem_limit_bytes=110 * 1024 * 1024,
            disable_bounds_checks=True, disable_semaphore_checks=True),
    )(
        A_x.reshape(NSEG, SEG, DM), A_mem0.reshape(MEM, DM),
        *(w.reshape(DM // 2, 2, H, DH) for w in (A_Wq, A_Wk, A_Wv)),
        A_Wo.reshape(H * DH, DM), B_w_r, B_w_gate, B_w_up, B_w_down,
    )
    return out.reshape(1, NSEG * SEG, DM)
```

```python
import functools
import math

import jax
import jax.numpy as jnp
from jax import lax
import jax.experimental.pallas as pl
import jax.experimental.pallas.tpu as pltpu

BF = jnp.bfloat16
F32 = jnp.float32
U32 = jnp.uint32
I32 = jnp.int32

H, DH, DM, MEM, SEG, NSEG, DFF = 32, 128, 512, 8, 32, 64, 1792
L = MEM + SEG
XR = 8
XS = SEG - XR
NCB = DM // DH
UNROLL = 8
FG = 4
FS = 4
PEEL, BODY, NLONG, NSH = (1, 2, 3, 6), 9, 3, 2
NP0, NP1 = 32, 40
PR = 8

ORDERS = ("kvqspx", "qkvsxp", "kqsvpx", "qkvspx", "kvsqpx", "kpvsqx", "skvpqx", "xkvqsp", "kxvsqp", "vkqpsx",
          "pkvqsx", "kvxqps")
LAYOUT = dict(D1=4, D2=4, DV=5, PD=2, OTAIL=4, D3=2, ORDER=10, QBF=0, PBF=1, VBF=0, MERGE=0, XREV=0,
              NPIN=0, S0=0, S1=1, S2=2, SDUE=2, PINW=0, ONEP=0, APIN=0, AEV=1, CH0=0, CH1=0, CH2=0,
              RB=1, LNFREE=0, PO2=-1, FIN=0, FAT=6, PVI=0, QI=0)
STEP_LAYOUT = (
    dict(FAT=1, FIN=4, MERGE=2, PD=1, RB=2, S2=26, SDUE=3),
    dict(CH2=2, LNFREE=1, PO2=28),
    dict(CH1=1, PD=3, XREV=1),
    dict(CH1=2, PINW=1, PO2=24, XREV=1),
    dict(CH0=2, CH1=2, LNFREE=1, PO2=28, QI=1),
    dict(CH1=1, LNFREE=1, PD=1, PINW=1, PO2=28),
    dict(AEV=8, APIN=5, ORDER=7, PO2=28, XREV=1),
    dict(CH2=4, LNFREE=1, PO2=28, PVI=2, RB=0),
)

EPS = 1e-5
SCALE = 0.08837890625
C2 = SCALE * math.log2(math.e)
NEG = -1e9 / SCALE
LOWEST = -2 ** 31
FLIP = 0x7FFF0000


def _dot(a, b):
    return lax.dot_general(a, b, (((1,), (0,)), ((), ())), preferred_element_type=F32)


def _dot_t(a, b):
    return lax.dot_general(a, b, (((1,), (1,)), ((), ())), preferred_element_type=F32)


def _rb(x):
    return x.astype(BF).astype(F32)


def _layernorm(x):
    n = x.shape[-1]
    mean = jnp.sum(x, axis=-1, keepdims=True) * (1.0 / n)
    xc = x - mean
    var = jnp.sum(xc * xc, axis=-1, keepdims=True) * (1.0 / n)
    den = _rb(jnp.sqrt(_rb(_rb(var) + EPS)))
    return _rb(_rb(x - _rb(mean)) * (1.0 / den))


def _layernorm_f32(x):
    n = x.shape[-1]
    xc = x - jnp.sum(x, axis=-1, keepdims=True) * (1.0 / n)
    var = jnp.sum(xc * xc, axis=-1, keepdims=True) * (1.0 / n)
    return xc * lax.rsqrt(var + EPS)


def _recip(l):
    r = pl.reciprocal(l, approx=True)
    return r * (2.0 - l * r)


def _tree(f, xs):
    while len(xs) > 1:
        xs = [f(xs[a], xs[a + 1]) if a + 1 < len(xs) else xs[a] for a in range(0, len(xs), 2)]
    return xs[0]


def _chains(f, xs, n):
    if not n:
        return _tree(f, xs)
    return _tree(f, [functools.reduce(f, xs[i::n]) for i in range(n)])


def _kernel(x_hbm, m0_hbm, wq_hbm, wk_hbm, wv_hbm, wo_hbm, wr_hbm, wg_hbm, wu_hbm, wd_hbm,
            out_hbm,
            wp, wo, ex, st, stage, hh, xs, obuf, wg, wu, wd, xe, ybuf, top, xn, mem, x0s, pbuf, m0s, wrs,
            tab, sem_w, sem_x, sem_out):
    w_hbm = tuple(w.bitcast(U32) for w in (wq_hbm, wk_hbm, wv_hbm))
    peel, body, nlong = PEEL, BODY, NLONG
    npair = 3 * H // 2
    p0 = sum(peel)
    nit = (npair - p0) // body
    assert p0 + nit * body == npair
    bounds = [sum(peel[:g]) for g in range(len(peel))] + [p0 + i * body for i in range(nit + 1)]

    left = list(range(p0 - NSH, p0)) + [p0 + i * body + q for i in range(nit) for q in range(nlong, body)]
    assert 2 * len(left) + 6 * H <= (NSEG - FG + 1) * FS
    fill_plan = [(2 * p + e, NSEG - 3 * FG) for p in left for e in range(2)]
    fill_plan += [(j, NSEG - g * FG) for g in (2, 1) for j in range(3 * H)]
    fill_plan += fill_plan[-1:] * (NSEG * FS - len(fill_plan))

    def w_start(ps):
        for p in ps:
            g = max(i for i, b in enumerate(bounds) if b <= p)
            for t in range(2):
                pltpu.make_async_copy(w_hbm[p // (H // 2)].at[:, t, p % (H // 2), :],
                                      stage.at[p, t], sem_w.at[g]).start()

    def w_wait(g, first, n):
        part = stage.at[pl.ds(first, n)]
        pltpu.make_async_copy(part, part, sem_w.at[g]).wait()

    wo_copy = pltpu.make_async_copy(wo_hbm.bitcast(U32), wo, sem_x.at[0])

    hx = (NSEG - 2 * FG) // 2

    def x_copy(j):
        return pltpu.make_async_copy(x_hbm.at[pl.ds(j * hx, hx), pl.ds(XS, XR), :],
                                     xs.at[pl.ds(j * hx, hx), pl.ds(XS, XR), :], sem_x.at[8 + j])

    xc_copy = pltpu.make_async_copy(x_hbm.at[pl.ds(2 * hx, NSEG - 2 * hx), pl.ds(XS, XR), :],
                                    xs.at[pl.ds(2 * hx, NSEG - 2 * hx), pl.ds(XS, XR), :], sem_x.at[7])
    xr_copy = pltpu.make_async_copy(x_hbm.at[:, pl.ds(0, XS), :], xs.at[:, pl.ds(0, XS), :], sem_x.at[10])
    x0_copy = pltpu.make_async_copy(x_hbm.at[0, pl.ds(0, XS), :], x0s, sem_x.at[1])
    m0_copy = pltpu.make_async_copy(m0_hbm, m0s, sem_x.at[2])
    wr_copy = pltpu.make_async_copy(wr_hbm, wrs.at[pl.ds(0, DM)], sem_x.at[3])
    wg_copy = pltpu.make_async_copy(wg_hbm.bitcast(U32), wg, sem_x.at[4])
    wu_copy = pltpu.make_async_copy(wu_hbm.bitcast(U32), wu, sem_x.at[5])
    wd_copy = pltpu.make_async_copy(wd_hbm.bitcast(U32), wd, sem_x.at[6])

    def repack(p):
        a = stage[p, 0]
        b = stage[p, 1]
        wp[2 * p] = (a & jnp.uint32(0xFFFF)) | (b << 16)
        wp[2 * p + 1] = (a >> 16) | (b & jnp.uint32(0xFFFF0000))

    def w_tile(j):
        return pltpu.bitcast(wp[j], BF)

    def project_extra(j, s0, n):
        r0 = s0 * XR if isinstance(s0, int) else pl.multiple_of(s0 * XR, XR)
        ex[pl.ds(s0, n), j] = _dot(xe[pl.ds(r0, n * XR), :], w_tile(j)).reshape(n, XR, DH)

    def ln_extra(s0, n):
        for g in range(s0, s0 + n):
            v = xs[g, XS:SEG, :].astype(F32)
            xe[g * XR:(g + 1) * XR, :] = _layernorm_f32(v)

    def start_x(j, carry):
        x_copy(j).start()
        return carry

    lax.fori_loop(0, 2, start_x, 0)
    w_start(range(bounds[0], bounds[1]))
    small = (x0_copy, m0_copy, wr_copy, xc_copy)

    def project_pairs(first, count, long, starts=None):
        repack(first)
        if count == 1 and starts is not None:
            starts()
        for i in range(count):
            n = NSEG - (2 if i < long else 3) * FG
            project_extra(2 * (first + i), 0, n)
            if i + 1 < count:
                repack(first + i + 1)
                if i + 2 == count and starts is not None:
                    starts()
            project_extra(2 * (first + i) + 1, 0, n)

    def init_state():
        mem[...] = m0s[...].astype(F32)
        xn[...] = _layernorm_f32(x0s[...].astype(F32))
        ln_extra(2 * hx, NSEG - 2 * hx)
        ybuf[...] = jnp.zeros((1, SEG, DM), F32)
        top[...] = jnp.full((2, SEG, 1), LOWEST, I32)
        for n, (j, g) in enumerate(fill_plan):
            tab[2 * n] = j
            tab[2 * n + 1] = g

    def stage_starts(k):
        if k == 0:
            w_start(range(bounds[3], NP0))
        if k == 3:
            w_start(range(NP0, NP1))
        if k == 4:
            w_start(range(NP1, npair))
            xr_copy.start()

    def pro_loop(i, carry):
        @pl.when(i == 1)
        def _():
            wo_copy.start()

        def starts():
            pl.when(i == 0)(functools.partial(stage_starts, 4))

        w_wait(len(peel) + i, p0 + i * body, body)
        project_pairs(p0 + i * body, body, nlong, starts)
        return carry

    def prologue():
        x_copy(0).wait()
        w_start(range(bounds[1], bounds[2]))
        ln_extra(0, hx)
        x_copy(1).wait()
        w_start(range(bounds[2], bounds[3]))
        for cp in small:
            cp.start()
        ln_extra(hx, hx)
        for g, n in enumerate(peel):
            last = g + 1 == len(peel)
            w_wait(g, bounds[g], n)
            if last:
                for cp in small:
                    cp.wait()
            project_pairs(bounds[g], n, n - NSH if last else n, functools.partial(stage_starts, g))
            if last:
                init_state()
        lax.fori_loop(0, nit, pro_loop, 0)
        for cp in (wg_copy, wu_copy, wd_copy):
            cp.start()
        xr_copy.wait()
        wo_copy.wait()

    def finish_rows(s, y, r0, n, live, keep=True):
        h = _rb(xs[s, r0:r0 + n, :].astype(F32) + _rb(y))
        hn = _layernorm(h)
        hh[s, r0:r0 + n, :] = h
        hh[s, SEG + r0:SEG + r0 + n, :] = hn
        obuf[s, r0:r0 + n, :] = (h + hn).astype(BF)
        r = _rb(jnp.sum(hn * wrs[pl.ds(0, DM)].astype(F32), axis=-1, keepdims=True))
        b = lax.bitcast_convert_type(r, I32)
        back = (NSEG * SEG - 1 - r0 - s * SEG) - lax.broadcasted_iota(I32, (n, 1), 0)
        key = (b ^ ((b >> 31) & FLIP)) | back
        if live is not None:
            key = jnp.where(live, key, LOWEST)
        b1, b2 = top[0, r0:r0 + n, :], top[1, r0:r0 + n, :]
        new = jnp.maximum(key, b1), jnp.maximum(jnp.minimum(key, b1), b2)
        if keep:
            top[0, r0:r0 + n, :] = new[0]
            top[1, r0:r0 + n, :] = new[1]
        return new

    def step(it, k):
        (D1, D2, DV, PD, OTAIL, D3, ORDER, QBF, PBF, VBF, MERGE, XREV, NPIN, S0, S1, S2, SDUE, PINW, ONEP,
         APIN, AEV, CH0, CH1, CH2, RB, LNFREE, PO2, FIN, FAT, PVI, QI) = {**LAYOUT,
         **STEP_LAYOUT[k]}.values()
        s = it * UNROLL + k
        row = lax.broadcasted_iota(I32, (L, L), 0)
        col = lax.broadcasted_iota(I32, (L, L), 1)
        mask = (row < MEM) | (row >= col)
        hs = jnp.concatenate([mem[...], xn[...]], axis=0).astype(BF)
        s0 = pl.multiple_of(it * UNROLL, UNROLL)
        prev = s0 + (k - 1) if k else jnp.maximum(s - 1, 0)
        succ = s0 + (k + 1) if k + 1 < UNROLL else jnp.minimum(s + 1, NSEG - 1)
        yprev = ybuf[0]
        never = s < 0
        zero = jnp.minimum(s, 0)

        def side_work(j):
            if j < 2:
                if ONEP and j == 1:
                    return []
                for i in range(2) if ONEP == 1 else [j]:
                    if ONEP == 2:
                        finish_rows(prev, yprev, 0, SEG, None if k else s >= 1)
                    else:
                        finish_rows(prev, yprev[16 * i:16 * i + 16], 16 * i, 16, None if k else s >= 1)
                z8 = pl.multiple_of(zero, 8)
                z16 = pl.multiple_of(zero, 16)
                toks = [hh[prev, pl.ds(z8, 8), 0:DH], top[0, pl.ds(z8, 8), :].astype(F32),
                        obuf[prev, pl.ds(z16, 16), 0:DH].astype(F32)[0:8]]
                return [toks[0] + toks[1] + toks[2]] if not PINW else toks
            xn[...] = _layernorm_f32(xs[succ, 0:XS, :].astype(F32))
            return [xn[pl.ds(pl.multiple_of(zero, 8), 8), 0:DH]]

        side_at = {S0: 0, S1: 1, S2: 2}
        due = {}
        odue = {}

        sub = lax.broadcasted_iota(I32, (8, 1), 0)
        groups = [0] + list(range(2, L // 8))

        def project(t, m):
            if MERGE:
                if m == 1:
                    ms = (1, 2, 0) if MERGE == 1 else (0, 1, 2)
                    y = _dot(hs, jnp.concatenate([w_tile(a * H + t) for a in ms], axis=1))
                    for i, a in enumerate(ms):
                        st[t, a] = y[:, i * DH:(i + 1) * DH]
                return
            st[t, m] = _dot(hs, w_tile(m * H + t))

        def rows(t, m, gs):
            return [ex[s, m * H + t] if g == L // 8 - 1 else st[t, m, 8 * g:8 * g + 8, :] for g in gs]

        def probs(t):
            q = rows(t, 0, groups)
            kk = jnp.concatenate(rows(t, 1, range(L // 8)), axis=0)
            for i, tok in enumerate(due.get(t, ())):
                q[(-1 - i - QI) % 4] = jnp.where(never, tok, q[(-1 - i - QI) % 4])
            mk = jnp.concatenate([mask[8 * g:8 * g + 8] for g in groups], axis=0)
            qq = jnp.concatenate(q, axis=0)
            sc = jnp.where(mk, _dot_t(qq.astype(BF) if QBF else qq, kk), NEG)
            p = jnp.exp2((sc - jnp.max(sc, axis=-1, keepdims=True)) * C2)
            return p, jnp.sum(p, axis=-1, keepdims=True)

        def first_rows(t):
            q = rows(t, 0, [1])[0] * C2
            kk = rows(t, 1, [0, 1])
            vv = rows(t, 2, [0, 1])

            def row(a, j):
                if RB & (1 if a is kk else 2):
                    return jnp.broadcast_to(st[t, 1 if a is kk else 2, j:j + 1, :], (8, DH))
                return jnp.broadcast_to(a[j // 8][j % 8:j % 8 + 1], (8, DH))

            order = list(range(MEM + 8))
            if XREV:
                order = order[::-1]
            sc = {}
            for j in order:
                sj = jnp.sum(q * row(kk, j), axis=-1, keepdims=True)
                sc[j] = jnp.where(sub >= j - MEM, sj, NEG * C2) if j > MEM else sj
            sc = [sc[j] for j in range(MEM + 8)]
            mx = _chains(jnp.maximum, sc, CH0)
            p = [jnp.exp2(sj - mx) for sj in sc]
            o = _chains(jnp.add, [p[j] * row(vv, j) for j in range(MEM + 8)], CH1)
            return o * _recip(_chains(jnp.add, p, CH2))

        def mix(t):
            p, l = pr[t]
            v = rows(t, 2, range(L // 8))
            if t - PD >= 0:
                v[PVI] = jnp.where(never, first[t - PD], v[PVI])
            if NPIN and t - NPIN >= 0:
                v[2] = jnp.where(never, _tree(jnp.add, [mixed[t - NPIN][8 * g:8 * g + 8] for g in groups]), v[2])
            vv = jnp.concatenate(v, axis=0)
            o = _dot(p.astype(BF) if PBF else p, vv.astype(BF) if VBF else vv) * _recip(l)
            return jnp.concatenate([o[0:MEM], first[t], o[MEM:]], axis=0)

        def project_out(o, t, acc):
            for tok in odue.get(t, ()):
                o = jnp.concatenate([jnp.where(never, tok, o[0:8]), o[8:]], axis=0)
            if APIN and t - APIN >= 1 and t % AEV == 0:
                a = accs[t - APIN]
                o = jnp.where(never, _tree(jnp.add, [a[:, c * DH:(c + 1) * DH] for c in range(NCB)]), o)
            y = _dot(o, pltpu.bitcast(wo[t * (DH // 2):(t + 1) * (DH // 2), :], BF))
            accs[t] = y if acc is None else acc + y
            return accs[t]

        pr, first, mixed, accs = {}, {}, {}, {}
        acc, nxt = None, 0
        for t in range(H + D1 + D2):
            u = t - D1 - D2
            if FIN and t == FAT:
                fill(it, k, range(FS - FIN, FS))
            for ch in ORDERS[ORDER]:
                if ch in "qkv":
                    if t < H:
                        project(t, "qkv".index(ch))
                elif ch == "s":
                    if t in side_at:
                        j = side_at[t]
                        tok = side_work(j)
                        if j == 2 and LNFREE and k + 1 < UNROLL:
                            pass
                        elif j == 2 and PO2 >= 0:
                            odue[PO2] = tok
                        else:
                            due[t + SDUE] = tok
                    if 0 <= t - D1 < H:
                        pr[t - D1] = probs(t - D1)
                elif ch == "x":
                    if 0 <= t - DV < H:
                        first[t - DV] = first_rows(t - DV)
                elif 0 <= u < H:
                    if u not in first:
                        first[u] = first_rows(u)
                    mixed[u] = mix(u)
            if t >= H:
                for _ in range(OTAIL):
                    if nxt <= u - D3:
                        acc = project_out(mixed[nxt], nxt, acc)
                        nxt += 1
        while nxt < H:
            acc = project_out(mixed[nxt], nxt, acc)
            nxt += 1
        mem[...] = acc[0:MEM]
        ybuf[0] = acc[MEM:]

    def fill(it, k, es):
        for e in es:
            n = (it * UNROLL + k) * FS + e
            project_extra(tab[2 * n], tab[2 * n + 1], FG)

    def out_copy(first, count):
        return pltpu.make_async_copy(obuf.at[pl.ds(first, count)], out_hbm.at[pl.ds(first, count)],
                                     sem_out.at[0])

    def block(it, carry):
        pl.when(it == 0)(prologue)
        for k in range(UNROLL):
            fill(it, k, range(FS - {**LAYOUT, **STEP_LAYOUT[k]}["FIN"]))
            step(it, k)

        @pl.when(it == 0)
        def _():
            out_copy(0, UNROLL - 1).start()

        @pl.when(it > 0)
        def _():
            out_copy(it * UNROLL - 1, UNROLL).start()

        return carry

    nblk = NSEG // UNROLL

    sub = lax.broadcasted_iota(I32, (8, 1), 0)
    last = NSEG * SEG - 1

    def select(b1, b2):
        k1 = jnp.max(b1, axis=0, keepdims=True)
        k2 = jnp.max(jnp.where(b1 == k1, b2, b1), axis=0, keepdims=True)
        return k1[0, 0], k2[0, 0]

    def place(key):
        n = last - (key & last)
        r = n & (SEG - 1)
        return n >> 5, r, pl.multiple_of(r & -PR, PR)

    def ffn(k1, k2):
        (s1, r1, _), (s2, r2, _) = place(k1), place(k2)
        xsel = jnp.where(sub == 0, hh[s1, pl.ds(SEG + r1, 1), :],
                         jnp.where(sub == 1, hh[s2, pl.ds(SEG + r2, 1), :], 0.0))
        g = _rb(_dot(xsel, pltpu.bitcast(wg[...], BF)))
        g = _rb(g * jax.nn.sigmoid(g))
        u = _rb(_dot(xsel, pltpu.bitcast(wu[...], BF)))
        return _rb(_dot(_rb(g * u), pltpu.bitcast(wd[...], BF)))

    def patch(y, k1, k2):
        hi = jnp.where(lax.broadcasted_iota(I32, (8, DH), 0) == 0, k1, k2) & -65536
        gate = _rb(jax.nn.sigmoid(lax.bitcast_convert_type(hi ^ ((hi >> 31) & FLIP), F32)))
        y = _rb(y * jnp.concatenate([gate] * NCB, axis=1))
        for j, key in enumerate((k1, k2)):
            s, _, g = place(key)
            back = (last - s * SEG - g) - lax.broadcasted_iota(I32, (PR, 1), 0)
            upd = jnp.where(back == (k1 & last), y[0:1], jnp.where(back == (k2 & last), y[1:2], 0.0))
            pbuf[j] = (hh[s, pl.ds(g, PR), :] + _rb(hh[s, pl.ds(SEG + g, PR), :] + upd)).astype(BF)

    def epilogue():
        wg_copy.wait()
        wu_copy.wait()
        wd_copy.wait()
        m1, m2 = select(top[0], top[1])
        y = ffn(m1, m2)
        c1, c2 = finish_rows(NSEG - 1, ybuf[0], 0, SEG, None, False)
        out_copy(NSEG - 1, 1).start()
        k1, k2 = select(c1, c2)
        patch(y, k1, k2)

        @pl.when((k1 != m1) | (k2 != m2))
        def _():
            patch(ffn(k1, k2), k1, k2)

        out_copy(0, NSEG).wait()
        (s1, _, g1), (s2, _, g2) = place(k1), place(k2)
        cp1 = pltpu.make_async_copy(pbuf.at[0], out_hbm.at[s1, pl.ds(g1, PR), :], sem_out.at[0])
        cp2 = pltpu.make_async_copy(pbuf.at[1], out_hbm.at[s2, pl.ds(g2, PR), :], sem_out.at[1])
        cp1.start()

        @pl.when((s2 != s1) | (g2 != g1))
        def _():
            cp2.start()
            cp2.wait()

        cp1.wait()

    lax.fori_loop(0, nblk, block, 0)
    epilogue()


@functools.partial(jax.jit, static_argnames=("A_seg_len",))
def pallas_sequential_preLN__memory_aug_recurrent_mem_tr__moe_arch_mod__prompt_kernel(
    A_x, A_mem0, A_Wq, A_Wk, A_Wv, A_Wo, A_seg_len, B_x, B_w_r, B_w_gate, B_w_up, B_w_down,
):
    del B_x
    assert A_seg_len == SEG and A_x.shape == (1, NSEG * SEG, DM) and A_mem0.shape == (1, MEM, DM)
    assert A_Wq.shape == (DM, H, DH) and A_Wo.shape == (H, DH, DM) and B_w_gate.shape == (DM, DFF)
    vmem = pltpu.VMEM
    out = pl.pallas_call(
        _kernel,
        out_shape=jax.ShapeDtypeStruct((NSEG, SEG, DM), BF),
        in_specs=[pl.BlockSpec(memory_space=pl.ANY)] * 10,
        out_specs=pl.BlockSpec(memory_space=pl.ANY),
        scratch_shapes=[
            vmem((3 * H, DM // 2, DH), U32),
            vmem((H * DH // 2, DM), U32),
            vmem((NSEG, 3 * H, XR, DH), F32),
            vmem((H, 3, MEM + XS, DH), F32),
            vmem((3 * H // 2, 2, DM // 2, DH), U32),
            vmem((NSEG, 2 * SEG, DM), F32),
            vmem((NSEG, SEG, DM), BF),
            vmem((NSEG, SEG, DM), BF),
            vmem((DM // 2, DFF), U32),
            vmem((DM // 2, DFF), U32),
            vmem((DFF // 2, DM), U32),
            vmem((NSEG * XR, DM), F32),
            vmem((1, SEG, DM), F32),
            vmem((2, SEG, 1), I32),
            vmem((XS, DM), F32),
            vmem((MEM, DM), F32),
            vmem((XS, DM), BF),
            vmem((2, PR, DM), BF),
            vmem((MEM, DM), BF),
            vmem((4 * DM,), BF),
            pltpu.SMEM((2 * NSEG * FS,), I32),
            pltpu.SemaphoreType.DMA((12,)),
            pltpu.SemaphoreType.DMA((11,)),
            pltpu.SemaphoreType.DMA((2,)),
        ],
        compiler_params=pltpu.CompilerParams(
            vmem_limit_bytes=110 * 1024 * 1024,
            disable_bounds_checks=True, disable_semaphore_checks=True),
    )(
        A_x.reshape(NSEG, SEG, DM), A_mem0.reshape(MEM, DM),
        *(w.reshape(DM // 2, 2, H, DH) for w in (A_Wq, A_Wk, A_Wv)),
        A_Wo.reshape(H * DH, DM), B_w_r, B_w_gate, B_w_up, B_w_down,
    )
    return out.reshape(1, NSEG * SEG, DM)
```

```python
import functools
import math

import jax
import jax.numpy as jnp
from jax import lax
import jax.experimental.pallas as pl
import jax.experimental.pallas.tpu as pltpu

BF = jnp.bfloat16
F32 = jnp.float32
U32 = jnp.uint32
I32 = jnp.int32

H, DH, DM, MEM, SEG, NSEG, DFF = 32, 128, 512, 8, 32, 64, 1792
L = MEM + SEG
XR = 8
XS = SEG - XR
NCB = DM // DH
UNROLL = 8
FG = 4
FS = 4
PEEL, BODY, NLONG, NSH = (1, 2, 3, 6), 9, 3, 2
NP0, NP1 = 32, 40
PR = 8

ORDERS = ("kvqspx", "qkvsxp", "kqsvpx", "qkvspx", "kvsqpx", "kpvsqx", "skvpqx", "xkvqsp", "kxvsqp", "vkqpsx",
          "pkvqsx", "kvxqps")
LAYOUT = dict(D1=4, D2=4, DV=5, PD=2, OTAIL=4, D3=2, ORDER=10, QBF=0, PBF=1, VBF=0, MERGE=0, XREV=0,
              NPIN=0, S0=0, S1=1, S2=2, SDUE=2, PINW=0, ONEP=0, APIN=0, AEV=1, CH0=0, CH1=0, CH2=0,
              RB=1, LNFREE=0, PO2=-1, FIN=0, FAT=6, PVI=0, QI=0, ACC=0)
STEP_LAYOUT = (
    dict(FAT=1, FIN=4, MERGE=2, PD=1, RB=2, S2=26, SDUE=3),
    dict(CH2=2, LNFREE=1, PO2=28),
    dict(CH1=1, PD=3, XREV=1),
    dict(CH1=2, PINW=1, PO2=28, XREV=1),
    dict(CH0=2, CH1=2, LNFREE=1, ORDER=8, PO2=24, QI=1, SDUE=3),
    dict(CH1=1, LNFREE=1, MERGE=3, PD=1, PINW=1, PO2=28),
    dict(AEV=8, APIN=5, ORDER=7, PO2=28, XREV=1),
    dict(CH2=4, LNFREE=1, PO2=28, PVI=2, RB=0),
)

EPS = 1e-5
SCALE = 0.08837890625
C2 = SCALE * math.log2(math.e)
NEG = -1e9 / SCALE
LOWEST = -2 ** 31
FLIP = 0x7FFF0000


def _dot(a, b):
    return lax.dot_general(a, b, (((1,), (0,)), ((), ())), preferred_element_type=F32)


def _dot_t(a, b):
    return lax.dot_general(a, b, (((1,), (1,)), ((), ())), preferred_element_type=F32)


def _rb(x):
    return x.astype(BF).astype(F32)


def _layernorm(x):
    n = x.shape[-1]
    mean = jnp.sum(x, axis=-1, keepdims=True) * (1.0 / n)
    xc = x - mean
    var = jnp.sum(xc * xc, axis=-1, keepdims=True) * (1.0 / n)
    den = _rb(jnp.sqrt(_rb(_rb(var) + EPS)))
    return _rb(_rb(x - _rb(mean)) * (1.0 / den))


def _layernorm_f32(x):
    n = x.shape[-1]
    xc = x - jnp.sum(x, axis=-1, keepdims=True) * (1.0 / n)
    var = jnp.sum(xc * xc, axis=-1, keepdims=True) * (1.0 / n)
    return xc * lax.rsqrt(var + EPS)


def _recip(l):
    r = pl.reciprocal(l, approx=True)
    return r * (2.0 - l * r)


def _tree(f, xs):
    while len(xs) > 1:
        xs = [f(xs[a], xs[a + 1]) if a + 1 < len(xs) else xs[a] for a in range(0, len(xs), 2)]
    return xs[0]


def _chains(f, xs, n):
    if not n:
        return _tree(f, xs)
    return _tree(f, [functools.reduce(f, xs[i::n]) for i in range(n)])


def _kernel(x_hbm, m0_hbm, wq_hbm, wk_hbm, wv_hbm, wo_hbm, wr_hbm, wg_hbm, wu_hbm, wd_hbm,
            out_hbm,
            wp, wo, ex, st, stage, hh, xs, obuf, wg, wu, wd, xe, ybuf, top, xn, mem, x0s, pbuf, m0s, wrs,
            tab, sem_w, sem_x, sem_out):
    w_hbm = tuple(w.bitcast(U32) for w in (wq_hbm, wk_hbm, wv_hbm))
    peel, body, nlong = PEEL, BODY, NLONG
    npair = 3 * H // 2
    p0 = sum(peel)
    nit = (npair - p0) // body
    assert p0 + nit * body == npair
    bounds = [sum(peel[:g]) for g in range(len(peel))] + [p0 + i * body for i in range(nit + 1)]

    left = list(range(p0 - NSH, p0)) + [p0 + i * body + q for i in range(nit) for q in range(nlong, body)]
    assert 2 * len(left) + 6 * H <= (NSEG - FG + 1) * FS
    fill_plan = [(2 * p + e, NSEG - 3 * FG) for p in left for e in range(2)]
    fill_plan += [(j, NSEG - g * FG) for g in (2, 1) for j in range(3 * H)]
    fill_plan += fill_plan[-1:] * (NSEG * FS - len(fill_plan))

    def w_start(ps):
        for p in ps:
            g = max(i for i, b in enumerate(bounds) if b <= p)
            for t in range(2):
                pltpu.make_async_copy(w_hbm[p // (H // 2)].at[:, t, p % (H // 2), :],
                                      stage.at[p, t], sem_w.at[g]).start()

    def w_wait(g, first, n):
        part = stage.at[pl.ds(first, n)]
        pltpu.make_async_copy(part, part, sem_w.at[g]).wait()

    wo_copy = pltpu.make_async_copy(wo_hbm.bitcast(U32), wo, sem_x.at[0])

    hx = (NSEG - 2 * FG) // 2

    def x_copy(j):
        return pltpu.make_async_copy(x_hbm.at[pl.ds(j * hx, hx), pl.ds(XS, XR), :],
                                     xs.at[pl.ds(j * hx, hx), pl.ds(XS, XR), :], sem_x.at[8 + j])

    xc_copy = pltpu.make_async_copy(x_hbm.at[pl.ds(2 * hx, NSEG - 2 * hx), pl.ds(XS, XR), :],
                                    xs.at[pl.ds(2 * hx, NSEG - 2 * hx), pl.ds(XS, XR), :], sem_x.at[7])
    xr_copy = pltpu.make_async_copy(x_hbm.at[:, pl.ds(0, XS), :], xs.at[:, pl.ds(0, XS), :], sem_x.at[10])
    x0_copy = pltpu.make_async_copy(x_hbm.at[0, pl.ds(0, XS), :], x0s, sem_x.at[1])
    m0_copy = pltpu.make_async_copy(m0_hbm, m0s, sem_x.at[2])
    wr_copy = pltpu.make_async_copy(wr_hbm, wrs.at[pl.ds(0, DM)], sem_x.at[3])
    wg_copy = pltpu.make_async_copy(wg_hbm.bitcast(U32), wg, sem_x.at[4])
    wu_copy = pltpu.make_async_copy(wu_hbm.bitcast(U32), wu, sem_x.at[5])
    wd_copy = pltpu.make_async_copy(wd_hbm.bitcast(U32), wd, sem_x.at[6])

    def repack(p):
        a = stage[p, 0]
        b = stage[p, 1]
        wp[2 * p] = (a & jnp.uint32(0xFFFF)) | (b << 16)
        wp[2 * p + 1] = (a >> 16) | (b & jnp.uint32(0xFFFF0000))

    def w_tile(j):
        return pltpu.bitcast(wp[j], BF)

    def project_extra(j, s0, n):
        r0 = s0 * XR if isinstance(s0, int) else pl.multiple_of(s0 * XR, XR)
        ex[pl.ds(s0, n), j] = _dot(xe[pl.ds(r0, n * XR), :], w_tile(j)).reshape(n, XR, DH)

    def ln_extra(s0, n):
        for g in range(s0, s0 + n):
            v = xs[g, XS:SEG, :].astype(F32)
            xe[g * XR:(g + 1) * XR, :] = _layernorm_f32(v)

    def start_x(j, carry):
        x_copy(j).start()
        return carry

    lax.fori_loop(0, 2, start_x, 0)
    w_start(range(bounds[0], bounds[1]))
    small = (x0_copy, m0_copy, wr_copy, xc_copy)

    def project_pairs(first, count, long, starts=None):
        repack(first)
        if count == 1 and starts is not None:
            starts()
        for i in range(count):
            n = NSEG - (2 if i < long else 3) * FG
            project_extra(2 * (first + i), 0, n)
            if i + 1 < count:
                repack(first + i + 1)
                if i + 2 == count and starts is not None:
                    starts()
            project_extra(2 * (first + i) + 1, 0, n)

    def init_state():
        mem[...] = m0s[...].astype(F32)
        xn[...] = _layernorm_f32(x0s[...].astype(F32))
        ln_extra(2 * hx, NSEG - 2 * hx)
        ybuf[...] = jnp.zeros((1, SEG, DM), F32)
        top[...] = jnp.full((2, SEG, 1), LOWEST, I32)
        for n, (j, g) in enumerate(fill_plan):
            tab[2 * n] = j
            tab[2 * n + 1] = g

    def stage_starts(k):
        if k == 0:
            w_start(range(bounds[3], NP0))
        if k == 3:
            w_start(range(NP0, NP1))
        if k == 4:
            w_start(range(NP1, npair))
            xr_copy.start()

    def pro_loop(i, carry):
        @pl.when(i == 1)
        def _():
            wo_copy.start()

        def starts():
            pl.when(i == 0)(functools.partial(stage_starts, 4))

        w_wait(len(peel) + i, p0 + i * body, body)
        project_pairs(p0 + i * body, body, nlong, starts)
        return carry

    def prologue():
        x_copy(0).wait()
        w_start(range(bounds[1], bounds[2]))
        ln_extra(0, hx)
        x_copy(1).wait()
        w_start(range(bounds[2], bounds[3]))
        for cp in small:
            cp.start()
        ln_extra(hx, hx)
        for g, n in enumerate(peel):
            last = g + 1 == len(peel)
            w_wait(g, bounds[g], n)
            if last:
                for cp in small:
                    cp.wait()
            project_pairs(bounds[g], n, n - NSH if last else n, functools.partial(stage_starts, g))
            if last:
                init_state()
        lax.fori_loop(0, nit, pro_loop, 0)
        for cp in (wg_copy, wu_copy, wd_copy):
            cp.start()
        xr_copy.wait()
        wo_copy.wait()

    def finish_rows(s, y, r0, n, live, keep=True):
        h = _rb(xs[s, r0:r0 + n, :].astype(F32) + _rb(y))
        hn = _layernorm(h)
        hh[s, r0:r0 + n, :] = h
        hh[s, SEG + r0:SEG + r0 + n, :] = hn
        obuf[s, r0:r0 + n, :] = (h + hn).astype(BF)
        r = _rb(jnp.sum(hn * wrs[pl.ds(0, DM)].astype(F32), axis=-1, keepdims=True))
        b = lax.bitcast_convert_type(r, I32)
        back = (NSEG * SEG - 1 - r0 - s * SEG) - lax.broadcasted_iota(I32, (n, 1), 0)
        key = (b ^ ((b >> 31) & FLIP)) | back
        if live is not None:
            key = jnp.where(live, key, LOWEST)
        b1, b2 = top[0, r0:r0 + n, :], top[1, r0:r0 + n, :]
        new = jnp.maximum(key, b1), jnp.maximum(jnp.minimum(key, b1), b2)
        if keep:
            top[0, r0:r0 + n, :] = new[0]
            top[1, r0:r0 + n, :] = new[1]
        return new

    def step(it, k):
        (D1, D2, DV, PD, OTAIL, D3, ORDER, QBF, PBF, VBF, MERGE, XREV, NPIN, S0, S1, S2, SDUE, PINW, ONEP,
         APIN, AEV, CH0, CH1, CH2, RB, LNFREE, PO2, FIN, FAT, PVI, QI, ACC) = {**LAYOUT,
         **STEP_LAYOUT[k]}.values()
        s = it * UNROLL + k
        row = lax.broadcasted_iota(I32, (L, L), 0)
        col = lax.broadcasted_iota(I32, (L, L), 1)
        mask = (row < MEM) | (row >= col)
        hs = jnp.concatenate([mem[...], xn[...]], axis=0).astype(BF)
        s0 = pl.multiple_of(it * UNROLL, UNROLL)
        prev = s0 + (k - 1) if k else jnp.maximum(s - 1, 0)
        succ = s0 + (k + 1) if k + 1 < UNROLL else jnp.minimum(s + 1, NSEG - 1)
        yprev = ybuf[0]
        never = s < 0
        zero = jnp.minimum(s, 0)

        def side_work(j):
            if j < 2:
                if ONEP and j == 1:
                    return []
                for i in range(2) if ONEP == 1 else [j]:
                    if ONEP == 2:
                        finish_rows(prev, yprev, 0, SEG, None if k else s >= 1)
                    else:
                        finish_rows(prev, yprev[16 * i:16 * i + 16], 16 * i, 16, None if k else s >= 1)
                z8 = pl.multiple_of(zero, 8)
                z16 = pl.multiple_of(zero, 16)
                toks = [hh[prev, pl.ds(z8, 8), 0:DH], top[0, pl.ds(z8, 8), :].astype(F32),
                        obuf[prev, pl.ds(z16, 16), 0:DH].astype(F32)[0:8]]
                return [toks[0] + toks[1] + toks[2]] if not PINW else toks
            xn[...] = _layernorm_f32(xs[succ, 0:XS, :].astype(F32))
            return [xn[pl.ds(pl.multiple_of(zero, 8), 8), 0:DH]]

        side_at = {S0: 0, S1: 1, S2: 2}
        due = {}
        odue = {}

        sub = lax.broadcasted_iota(I32, (8, 1), 0)
        groups = [0] + list(range(2, L // 8))

        def project(t, m):
            if MERGE >= 3:
                ms = ((1, 2), (0, 1), (2, 0))[MERGE - 3]
                if m == ms[0]:
                    y = _dot(hs, jnp.concatenate([w_tile(a * H + t) for a in ms], axis=1))
                    for i, a in enumerate(ms):
                        st[t, a] = y[:, i * DH:(i + 1) * DH]
                if m in ms:
                    return
            elif MERGE:
                if m == 1:
                    ms = (1, 2, 0) if MERGE == 1 else (0, 1, 2)
                    y = _dot(hs, jnp.concatenate([w_tile(a * H + t) for a in ms], axis=1))
                    for i, a in enumerate(ms):
                        st[t, a] = y[:, i * DH:(i + 1) * DH]
                return
            st[t, m] = _dot(hs, w_tile(m * H + t))

        def rows(t, m, gs):
            return [ex[s, m * H + t] if g == L // 8 - 1 else st[t, m, 8 * g:8 * g + 8, :] for g in gs]

        def probs(t):
            q = rows(t, 0, groups)
            kk = jnp.concatenate(rows(t, 1, range(L // 8)), axis=0)
            for i, tok in enumerate(due.get(t, ())):
                q[(-1 - i - QI) % 4] = jnp.where(never, tok, q[(-1 - i - QI) % 4])
            mk = jnp.concatenate([mask[8 * g:8 * g + 8] for g in groups], axis=0)
            qq = jnp.concatenate(q, axis=0)
            sc = jnp.where(mk, _dot_t(qq.astype(BF) if QBF else qq, kk), NEG)
            p = jnp.exp2((sc - jnp.max(sc, axis=-1, keepdims=True)) * C2)
            return p, jnp.sum(p, axis=-1, keepdims=True)

        def first_rows(t):
            q = rows(t, 0, [1])[0] * C2
            kk = rows(t, 1, [0, 1])
            vv = rows(t, 2, [0, 1])

            def row(a, j):
                if RB & (1 if a is kk else 2):
                    return jnp.broadcast_to(st[t, 1 if a is kk else 2, j:j + 1, :], (8, DH))
                return jnp.broadcast_to(a[j // 8][j % 8:j % 8 + 1], (8, DH))

            order = list(range(MEM + 8))
            if XREV:
                order = order[::-1]
            sc = {}
            for j in order:
                sj = jnp.sum(q * row(kk, j), axis=-1, keepdims=True)
                sc[j] = jnp.where(sub >= j - MEM, sj, NEG * C2) if j > MEM else sj
            sc = [sc[j] for j in range(MEM + 8)]
            mx = _chains(jnp.maximum, sc, CH0)
            p = [jnp.exp2(sj - mx) for sj in sc]
            o = _chains(jnp.add, [p[j] * row(vv, j) for j in range(MEM + 8)], CH1)
            return o * _recip(_chains(jnp.add, p, CH2))

        def mix(t):
            p, l = pr[t]
            v = rows(t, 2, range(L // 8))
            if t - PD >= 0:
                v[PVI] = jnp.where(never, first[t - PD], v[PVI])
            if NPIN and t - NPIN >= 0:
                v[2] = jnp.where(never, _tree(jnp.add, [mixed[t - NPIN][8 * g:8 * g + 8] for g in groups]), v[2])
            vv = jnp.concatenate(v, axis=0)
            o = _dot(p.astype(BF) if PBF else p, vv.astype(BF) if VBF else vv) * _recip(l)
            return jnp.concatenate([o[0:MEM], first[t], o[MEM:]], axis=0)

        def project_out(o, t, acc):
            for tok in odue.get(t, ()):
                o = jnp.concatenate([jnp.where(never, tok, o[0:8]), o[8:]], axis=0)
            if APIN and t - APIN >= 3 and t % AEV == 0:
                a = accs[t - APIN]
                o = jnp.where(never, _tree(jnp.add, [a[:, c * DH:(c + 1) * DH] for c in range(NCB)]), o)
            y = _dot(o, pltpu.bitcast(wo[t * (DH // 2):(t + 1) * (DH // 2), :], BF))
            held.append(y)
            if len(held) == (1, 2, 4, 3)[ACC] or t == H - 1:
                y = _tree(jnp.add, list(held))
                held.clear()
                acc = y if acc is None else acc + y
            accs[t] = acc
            return acc

        pr, first, mixed, accs, held = {}, {}, {}, {}, []
        acc, nxt = None, 0
        for t in range(H + D1 + D2):
            u = t - D1 - D2
            if FIN and t == FAT:
                fill(it, k, range(FS - FIN, FS))
            for ch in ORDERS[ORDER]:
                if ch in "qkv":
                    if t < H:
                        project(t, "qkv".index(ch))
                elif ch == "s":
                    if t in side_at:
                        j = side_at[t]
                        tok = side_work(j)
                        if j == 2 and LNFREE and k + 1 < UNROLL:
                            pass
                        elif j == 2 and PO2 >= 0:
                            odue[PO2] = tok
                        else:
                            due[t + SDUE] = tok
                    if 0 <= t - D1 < H:
                        pr[t - D1] = probs(t - D1)
                elif ch == "x":
                    if 0 <= t - DV < H:
                        first[t - DV] = first_rows(t - DV)
                elif 0 <= u < H:
                    if u not in first:
                        first[u] = first_rows(u)
                    mixed[u] = mix(u)
            if t >= H:
                for _ in range(OTAIL):
                    if nxt <= u - D3:
                        acc = project_out(mixed[nxt], nxt, acc)
                        nxt += 1
        while nxt < H:
            acc = project_out(mixed[nxt], nxt, acc)
            nxt += 1
        mem[...] = acc[0:MEM]
        ybuf[0] = acc[MEM:]

    def fill(it, k, es):
        for e in es:
            n = (it * UNROLL + k) * FS + e
            project_extra(tab[2 * n], tab[2 * n + 1], FG)

    def out_copy(first, count):
        return pltpu.make_async_copy(obuf.at[pl.ds(first, count)], out_hbm.at[pl.ds(first, count)],
                                     sem_out.at[0])

    def block(it, carry):
        pl.when(it == 0)(prologue)
        for k in range(UNROLL):
            fill(it, k, range(FS - {**LAYOUT, **STEP_LAYOUT[k]}["FIN"]))
            step(it, k)

        @pl.when(it == 0)
        def _():
            out_copy(0, UNROLL - 1).start()

        @pl.when(it > 0)
        def _():
            out_copy(it * UNROLL - 1, UNROLL).start()

        return carry

    nblk = NSEG // UNROLL

    sub = lax.broadcasted_iota(I32, (8, 1), 0)
    last = NSEG * SEG - 1

    def select(b1, b2):
        k1 = jnp.max(b1, axis=0, keepdims=True)
        k2 = jnp.max(jnp.where(b1 == k1, b2, b1), axis=0, keepdims=True)
        return k1[0, 0], k2[0, 0]

    def place(key):
        n = last - (key & last)
        r = n & (SEG - 1)
        return n >> 5, r, pl.multiple_of(r & -PR, PR)

    def ffn(k1, k2):
        (s1, r1, _), (s2, r2, _) = place(k1), place(k2)
        xsel = jnp.where(sub == 0, hh[s1, pl.ds(SEG + r1, 1), :],
                         jnp.where(sub == 1, hh[s2, pl.ds(SEG + r2, 1), :], 0.0))
        g = _rb(_dot(xsel, pltpu.bitcast(wg[...], BF)))
        g = _rb(g * jax.nn.sigmoid(g))
        u = _rb(_dot(xsel, pltpu.bitcast(wu[...], BF)))
        return _rb(_dot(_rb(g * u), pltpu.bitcast(wd[...], BF)))

    def patch(y, k1, k2):
        hi = jnp.where(lax.broadcasted_iota(I32, (8, DH), 0) == 0, k1, k2) & -65536
        gate = _rb(jax.nn.sigmoid(lax.bitcast_convert_type(hi ^ ((hi >> 31) & FLIP), F32)))
        y = _rb(y * jnp.concatenate([gate] * NCB, axis=1))
        for j, key in enumerate((k1, k2)):
            s, _, g = place(key)
            back = (last - s * SEG - g) - lax.broadcasted_iota(I32, (PR, 1), 0)
            upd = jnp.where(back == (k1 & last), y[0:1], jnp.where(back == (k2 & last), y[1:2], 0.0))
            pbuf[j] = (hh[s, pl.ds(g, PR), :] + _rb(hh[s, pl.ds(SEG + g, PR), :] + upd)).astype(BF)

    def epilogue():
        wg_copy.wait()
        wu_copy.wait()
        wd_copy.wait()
        m1, m2 = select(top[0], top[1])
        y = ffn(m1, m2)
        c1, c2 = finish_rows(NSEG - 1, ybuf[0], 0, SEG, None, False)
        out_copy(NSEG - 1, 1).start()
        k1, k2 = select(c1, c2)
        patch(y, k1, k2)

        @pl.when((k1 != m1) | (k2 != m2))
        def _():
            patch(ffn(k1, k2), k1, k2)

        out_copy(0, NSEG).wait()
        (s1, _, g1), (s2, _, g2) = place(k1), place(k2)
        cp1 = pltpu.make_async_copy(pbuf.at[0], out_hbm.at[s1, pl.ds(g1, PR), :], sem_out.at[0])
        cp2 = pltpu.make_async_copy(pbuf.at[1], out_hbm.at[s2, pl.ds(g2, PR), :], sem_out.at[1])
        cp1.start()

        @pl.when((s2 != s1) | (g2 != g1))
        def _():
            cp2.start()
            cp2.wait()

        cp1.wait()

    lax.fori_loop(0, nblk, block, 0)
    epilogue()


@functools.partial(jax.jit, static_argnames=("A_seg_len",))
def pallas_sequential_preLN__memory_aug_recurrent_mem_tr__moe_arch_mod__prompt_kernel(
    A_x, A_mem0, A_Wq, A_Wk, A_Wv, A_Wo, A_seg_len, B_x, B_w_r, B_w_gate, B_w_up, B_w_down,
):
    del B_x
    assert A_seg_len == SEG and A_x.shape == (1, NSEG * SEG, DM) and A_mem0.shape == (1, MEM, DM)
    assert A_Wq.shape == (DM, H, DH) and A_Wo.shape == (H, DH, DM) and B_w_gate.shape == (DM, DFF)
    vmem = pltpu.VMEM
    out = pl.pallas_call(
        _kernel,
        out_shape=jax.ShapeDtypeStruct((NSEG, SEG, DM), BF),
        in_specs=[pl.BlockSpec(memory_space=pl.ANY)] * 10,
        out_specs=pl.BlockSpec(memory_space=pl.ANY),
        scratch_shapes=[
            vmem((3 * H, DM // 2, DH), U32),
            vmem((H * DH // 2, DM), U32),
            vmem((NSEG, 3 * H, XR, DH), F32),
            vmem((H, 3, MEM + XS, DH), F32),
            vmem((3 * H // 2, 2, DM // 2, DH), U32),
            vmem((NSEG, 2 * SEG, DM), F32),
            vmem((NSEG, SEG, DM), BF),
            vmem((NSEG, SEG, DM), BF),
            vmem((DM // 2, DFF), U32),
            vmem((DM // 2, DFF), U32),
            vmem((DFF // 2, DM), U32),
            vmem((NSEG * XR, DM), F32),
            vmem((1, SEG, DM), F32),
            vmem((2, SEG, 1), I32),
            vmem((XS, DM), F32),
            vmem((MEM, DM), F32),
            vmem((XS, DM), BF),
            vmem((2, PR, DM), BF),
            vmem((MEM, DM), BF),
            vmem((4 * DM,), BF),
            pltpu.SMEM((2 * NSEG * FS,), I32),
            pltpu.SemaphoreType.DMA((len(PEEL) + (3 * H // 2 - sum(PEEL)) // BODY,)),
            pltpu.SemaphoreType.DMA((11,)),
            pltpu.SemaphoreType.DMA((2,)),
        ],
        compiler_params=pltpu.CompilerParams(
            vmem_limit_bytes=110 * 1024 * 1024,
            disable_bounds_checks=True, disable_semaphore_checks=True),
    )(
        A_x.reshape(NSEG, SEG, DM), A_mem0.reshape(MEM, DM),
        *(w.reshape(DM // 2, 2, H, DH) for w in (A_Wq, A_Wk, A_Wv)),
        A_Wo.reshape(H * DH, DM), B_w_r, B_w_gate, B_w_up, B_w_down,
    )
    return out.reshape(1, NSEG * SEG, DM)
```

```python
import functools
import math

import jax
import jax.numpy as jnp
from jax import lax
import jax.experimental.pallas as pl
import jax.experimental.pallas.tpu as pltpu

BF = jnp.bfloat16
F32 = jnp.float32
U32 = jnp.uint32
I32 = jnp.int32

H, DH, DM, MEM, SEG, NSEG, DFF = 32, 128, 512, 8, 32, 64, 1792
L = MEM + SEG
XR = 8
XS = SEG - XR
NCB = DM // DH
UNROLL = 8
FG = 4
FS = 4
PEEL, BODY, NLONG, NSH = (1, 2, 3, 6), 9, 3, 2
NP0, NP1 = 32, 40
PR = 8

ORDERS = ("kvqspx", "qkvsxp", "kqsvpx", "qkvspx", "kvsqpx", "kpvsqx", "skvpqx", "xkvqsp", "kxvsqp", "vkqpsx",
          "pkvqsx", "kvxqps")
LAYOUT = dict(D1=4, D2=4, DV=5, PD=2, OTAIL=4, D3=2, ORDER=10, QBF=0, PBF=1, VBF=0, MERGE=0, XREV=0,
              NPIN=0, S0=0, S1=1, S2=2, SDUE=2, PINW=0, ONEP=0, APIN=0, AEV=1, CH0=0, CH1=0, CH2=0,
              RB=1, LNFREE=0, PO2=-1, FIN=0, FAT=6, PVI=0, QI=0, ACC=0)
STEP_LAYOUT = (
    dict(CH1=4, FAT=1, FIN=4, MERGE=2, PD=1, PVI=4, RB=2, S2=26, SDUE=3),
    dict(CH2=2, LNFREE=1, PO2=28, QBF=1),
    dict(CH1=1, PD=3, XREV=1),
    dict(CH1=2, PINW=1, PO2=28, RB=2, XREV=1),
    dict(CH0=2, CH1=2, LNFREE=1, MERGE=3, ORDER=8, PO2=24, QI=1, SDUE=3),
    dict(CH1=1, LNFREE=1, MERGE=3, PD=1, PINW=1, PO2=28),
    dict(AEV=8, APIN=5, ORDER=7, PO2=28, XREV=1),
    dict(CH2=4, LNFREE=1, PO2=28, PVI=2, RB=0),
)

EPS = 1e-5
SCALE = 0.08837890625
C2 = SCALE * math.log2(math.e)
NEG = -1e9 / SCALE
LOWEST = -2 ** 31
FLIP = 0x7FFF0000


def _dot(a, b):
    return lax.dot_general(a, b, (((1,), (0,)), ((), ())), preferred_element_type=F32)


def _dot_t(a, b):
    return lax.dot_general(a, b, (((1,), (1,)), ((), ())), preferred_element_type=F32)


def _rb(x):
    return x.astype(BF).astype(F32)


def _layernorm(x):
    n = x.shape[-1]
    mean = jnp.sum(x, axis=-1, keepdims=True) * (1.0 / n)
    xc = x - mean
    var = jnp.sum(xc * xc, axis=-1, keepdims=True) * (1.0 / n)
    den = _rb(jnp.sqrt(_rb(_rb(var) + EPS)))
    return _rb(_rb(x - _rb(mean)) * (1.0 / den))


def _layernorm_f32(x):
    n = x.shape[-1]
    xc = x - jnp.sum(x, axis=-1, keepdims=True) * (1.0 / n)
    var = jnp.sum(xc * xc, axis=-1, keepdims=True) * (1.0 / n)
    return xc * lax.rsqrt(var + EPS)


def _recip(l):
    r = pl.reciprocal(l, approx=True)
    return r * (2.0 - l * r)


def _tree(f, xs):
    while len(xs) > 1:
        xs = [f(xs[a], xs[a + 1]) if a + 1 < len(xs) else xs[a] for a in range(0, len(xs), 2)]
    return xs[0]


def _chains(f, xs, n):
    if not n:
        return _tree(f, xs)
    return _tree(f, [functools.reduce(f, xs[i::n]) for i in range(n)])


def _kernel(x_hbm, m0_hbm, wq_hbm, wk_hbm, wv_hbm, wo_hbm, wr_hbm, wg_hbm, wu_hbm, wd_hbm,
            out_hbm,
            wp, wo, ex, st, stage, hh, xs, obuf, wg, wu, wd, xe, ybuf, top, xn, mem, x0s, pbuf, m0s, wrs,
            tab, sem_w, sem_x, sem_out):
    w_hbm = tuple(w.bitcast(U32) for w in (wq_hbm, wk_hbm, wv_hbm))
    peel, body, nlong = PEEL, BODY, NLONG
    npair = 3 * H // 2
    p0 = sum(peel)
    nit = (npair - p0) // body
    assert p0 + nit * body == npair
    bounds = [sum(peel[:g]) for g in range(len(peel))] + [p0 + i * body for i in range(nit + 1)]

    left = list(range(p0 - NSH, p0)) + [p0 + i * body + q for i in range(nit) for q in range(nlong, body)]
    assert 2 * len(left) + 6 * H <= (NSEG - FG + 1) * FS
    fill_plan = [(2 * p + e, NSEG - 3 * FG) for p in left for e in range(2)]
    ntall = NSEG // UNROLL
    fill_plan += [(j, NSEG - g * FG) for g in (2, 1) for j in range(3 * H - ntall)]
    todo = fill_plan + fill_plan[-1:] * NSEG
    fill_plan = []
    for n in range(NSEG * FS):
        e = n % (UNROLL * FS)
        fill_plan.append((3 * H - ntall + n // (UNROLL * FS), NSEG - 2 * FG) if e < 2 else todo.pop(0))
    assert len(todo) - NSEG <= -(FG - 1) * FS

    def w_start(ps):
        for p in ps:
            g = max(i for i, b in enumerate(bounds) if b <= p)
            for t in range(2):
                pltpu.make_async_copy(w_hbm[p // (H // 2)].at[:, t, p % (H // 2), :],
                                      stage.at[p, t], sem_w.at[g]).start()

    def w_wait(g, first, n):
        part = stage.at[pl.ds(first, n)]
        pltpu.make_async_copy(part, part, sem_w.at[g]).wait()

    wo_copy = pltpu.make_async_copy(wo_hbm.bitcast(U32), wo, sem_x.at[0])

    hx = (NSEG - 2 * FG) // 2

    def x_copy(j):
        return pltpu.make_async_copy(x_hbm.at[pl.ds(j * hx, hx), pl.ds(XS, XR), :],
                                     xs.at[pl.ds(j * hx, hx), pl.ds(XS, XR), :], sem_x.at[8 + j])

    xc_copy = pltpu.make_async_copy(x_hbm.at[pl.ds(2 * hx, NSEG - 2 * hx), pl.ds(XS, XR), :],
                                    xs.at[pl.ds(2 * hx, NSEG - 2 * hx), pl.ds(XS, XR), :], sem_x.at[7])
    xr_copy = pltpu.make_async_copy(x_hbm.at[:, pl.ds(0, XS), :], xs.at[:, pl.ds(0, XS), :], sem_x.at[10])
    x0_copy = pltpu.make_async_copy(x_hbm.at[0, pl.ds(0, XS), :], x0s, sem_x.at[1])
    m0_copy = pltpu.make_async_copy(m0_hbm, m0s, sem_x.at[2])
    wr_copy = pltpu.make_async_copy(wr_hbm, wrs.at[pl.ds(0, DM)], sem_x.at[3])
    wg_copy = pltpu.make_async_copy(wg_hbm.bitcast(U32), wg, sem_x.at[4])
    wu_copy = pltpu.make_async_copy(wu_hbm.bitcast(U32), wu, sem_x.at[5])
    wd_copy = pltpu.make_async_copy(wd_hbm.bitcast(U32), wd, sem_x.at[6])

    def repack(p):
        a = stage[p, 0]
        b = stage[p, 1]
        wp[2 * p] = (a & jnp.uint32(0xFFFF)) | (b << 16)
        wp[2 * p + 1] = (a >> 16) | (b & jnp.uint32(0xFFFF0000))

    def w_tile(j):
        return pltpu.bitcast(wp[j], BF)

    def project_extra(j, s0, n):
        r0 = s0 * XR if isinstance(s0, int) else pl.multiple_of(s0 * XR, XR)
        ex[pl.ds(s0, n), j] = _dot(xe[pl.ds(r0, n * XR), :], w_tile(j)).reshape(n, XR, DH)

    def ln_extra(s0, n):
        for g in range(s0, s0 + n):
            v = xs[g, XS:SEG, :].astype(F32)
            xe[g * XR:(g + 1) * XR, :] = _layernorm_f32(v)

    def start_x(j, carry):
        x_copy(j).start()
        return carry

    lax.fori_loop(0, 2, start_x, 0)
    w_start(range(bounds[0], bounds[1]))
    small = (x0_copy, m0_copy, wr_copy, xc_copy)

    def project_pairs(first, count, long, starts=None):
        repack(first)
        if count == 1 and starts is not None:
            starts()
        for i in range(count):
            n = NSEG - (2 if i < long else 3) * FG
            project_extra(2 * (first + i), 0, n)
            if i + 1 < count:
                repack(first + i + 1)
                if i + 2 == count and starts is not None:
                    starts()
            project_extra(2 * (first + i) + 1, 0, n)

    def init_state():
        mem[...] = m0s[...].astype(F32)
        xn[...] = _layernorm_f32(x0s[...].astype(F32))
        ln_extra(2 * hx, NSEG - 2 * hx)
        ybuf[...] = jnp.zeros((1, SEG, DM), F32)
        top[...] = jnp.full((2, SEG, 1), LOWEST, I32)
        for n, (j, g) in enumerate(fill_plan):
            tab[2 * n] = j
            tab[2 * n + 1] = g

    def stage_starts(k):
        if k == 0:
            w_start(range(bounds[3], NP0))
        if k == 3:
            w_start(range(NP0, NP1))
        if k == 4:
            w_start(range(NP1, npair))
            xr_copy.start()

    def pro_loop(i, carry):
        @pl.when(i == 1)
        def _():
            wo_copy.start()

        def starts():
            pl.when(i == 0)(functools.partial(stage_starts, 4))

        w_wait(len(peel) + i, p0 + i * body, body)
        project_pairs(p0 + i * body, body, nlong, starts)
        return carry

    def prologue():
        x_copy(0).wait()
        w_start(range(bounds[1], bounds[2]))
        ln_extra(0, hx)
        x_copy(1).wait()
        w_start(range(bounds[2], bounds[3]))
        for cp in small:
            cp.start()
        ln_extra(hx, hx)
        for g, n in enumerate(peel):
            last = g + 1 == len(peel)
            w_wait(g, bounds[g], n)
            if last:
                for cp in small:
                    cp.wait()
            project_pairs(bounds[g], n, n - NSH if last else n, functools.partial(stage_starts, g))
            if last:
                init_state()
        lax.fori_loop(0, nit, pro_loop, 0)
        for cp in (wg_copy, wu_copy, wd_copy):
            cp.start()
        xr_copy.wait()
        wo_copy.wait()

    def finish_rows(s, y, r0, n, live, keep=True):
        h = _rb(xs[s, r0:r0 + n, :].astype(F32) + _rb(y))
        hn = _layernorm(h)
        hh[s, r0:r0 + n, :] = h
        hh[s, SEG + r0:SEG + r0 + n, :] = hn
        obuf[s, r0:r0 + n, :] = (h + hn).astype(BF)
        r = _rb(jnp.sum(hn * wrs[pl.ds(0, DM)].astype(F32), axis=-1, keepdims=True))
        b = lax.bitcast_convert_type(r, I32)
        back = (NSEG * SEG - 1 - r0 - s * SEG) - lax.broadcasted_iota(I32, (n, 1), 0)
        key = (b ^ ((b >> 31) & FLIP)) | back
        if live is not None:
            key = jnp.where(live, key, LOWEST)
        b1, b2 = top[0, r0:r0 + n, :], top[1, r0:r0 + n, :]
        new = jnp.maximum(key, b1), jnp.maximum(jnp.minimum(key, b1), b2)
        if keep:
            top[0, r0:r0 + n, :] = new[0]
            top[1, r0:r0 + n, :] = new[1]
        return new

    def step(it, k):
        (D1, D2, DV, PD, OTAIL, D3, ORDER, QBF, PBF, VBF, MERGE, XREV, NPIN, S0, S1, S2, SDUE, PINW, ONEP,
         APIN, AEV, CH0, CH1, CH2, RB, LNFREE, PO2, FIN, FAT, PVI, QI, ACC) = {**LAYOUT,
         **STEP_LAYOUT[k]}.values()
        s = it * UNROLL + k
        row = lax.broadcasted_iota(I32, (L, L), 0)
        col = lax.broadcasted_iota(I32, (L, L), 1)
        mask = (row < MEM) | (row >= col)
        hs = jnp.concatenate([mem[...], xn[...]], axis=0).astype(BF)
        s0 = pl.multiple_of(it * UNROLL, UNROLL)
        prev = s0 + (k - 1) if k else jnp.maximum(s - 1, 0)
        succ = s0 + (k + 1) if k + 1 < UNROLL else jnp.minimum(s + 1, NSEG - 1)
        yprev = ybuf[0]
        never = s < 0
        zero = jnp.minimum(s, 0)

        def side_work(j):
            if j < 2:
                if ONEP and j == 1:
                    return []
                for i in range(2) if ONEP == 1 else [j]:
                    if ONEP == 2:
                        finish_rows(prev, yprev, 0, SEG, None if k else s >= 1)
                    else:
                        finish_rows(prev, yprev[16 * i:16 * i + 16], 16 * i, 16, None if k else s >= 1)
                z8 = pl.multiple_of(zero, 8)
                z16 = pl.multiple_of(zero, 16)
                toks = [hh[prev, pl.ds(z8, 8), 0:DH], top[0, pl.ds(z8, 8), :].astype(F32),
                        obuf[prev, pl.ds(z16, 16), 0:DH].astype(F32)[0:8]]
                return [toks[0] + toks[1] + toks[2]] if not PINW else toks
            xn[...] = _layernorm_f32(xs[succ, 0:XS, :].astype(F32))
            return [xn[pl.ds(pl.multiple_of(zero, 8), 8), 0:DH]]

        side_at = {S0: 0, S1: 1, S2: 2}
        due = {}
        odue = {}

        sub = lax.broadcasted_iota(I32, (8, 1), 0)
        groups = [0] + list(range(2, L // 8))

        def project(t, m):
            if MERGE >= 3:
                ms = ((1, 2), (0, 1), (2, 0))[MERGE - 3]
                if m == ms[0]:
                    y = _dot(hs, jnp.concatenate([w_tile(a * H + t) for a in ms], axis=1))
                    for i, a in enumerate(ms):
                        st[t, a] = y[:, i * DH:(i + 1) * DH]
                if m in ms:
                    return
            elif MERGE:
                if m == 1:
                    ms = (1, 2, 0) if MERGE == 1 else (0, 1, 2)
                    y = _dot(hs, jnp.concatenate([w_tile(a * H + t) for a in ms], axis=1))
                    for i, a in enumerate(ms):
                        st[t, a] = y[:, i * DH:(i + 1) * DH]
                return
            st[t, m] = _dot(hs, w_tile(m * H + t))

        def rows(t, m, gs):
            return [ex[s, m * H + t] if g == L // 8 - 1 else st[t, m, 8 * g:8 * g + 8, :] for g in gs]

        def probs(t):
            q = rows(t, 0, groups)
            kk = jnp.concatenate(rows(t, 1, range(L // 8)), axis=0)
            for i, tok in enumerate(due.get(t, ())):
                q[(-1 - i - QI) % 4] = jnp.where(never, tok, q[(-1 - i - QI) % 4])
            mk = jnp.concatenate([mask[8 * g:8 * g + 8] for g in groups], axis=0)
            qq = jnp.concatenate(q, axis=0)
            sc = jnp.where(mk, _dot_t(qq.astype(BF) if QBF else qq, kk), NEG)
            p = jnp.exp2((sc - jnp.max(sc, axis=-1, keepdims=True)) * C2)
            return p, jnp.sum(p, axis=-1, keepdims=True)

        def first_rows(t):
            q = rows(t, 0, [1])[0] * C2
            kk = rows(t, 1, [0, 1])
            vv = rows(t, 2, [0, 1])

            def row(a, j):
                if RB & (1 if a is kk else 2):
                    return jnp.broadcast_to(st[t, 1 if a is kk else 2, j:j + 1, :], (8, DH))
                return jnp.broadcast_to(a[j // 8][j % 8:j % 8 + 1], (8, DH))

            order = list(range(MEM + 8))
            if XREV:
                order = order[::-1]
            sc = {}
            for j in order:
                sj = jnp.sum(q * row(kk, j), axis=-1, keepdims=True)
                sc[j] = jnp.where(sub >= j - MEM, sj, NEG * C2) if j > MEM else sj
            sc = [sc[j] for j in range(MEM + 8)]
            mx = _chains(jnp.maximum, sc, CH0)
            p = [jnp.exp2(sj - mx) for sj in sc]
            o = _chains(jnp.add, [p[j] * row(vv, j) for j in range(MEM + 8)], CH1)
            return o * _recip(_chains(jnp.add, p, CH2))

        def mix(t):
            p, l = pr[t]
            v = rows(t, 2, range(L // 8))
            if t - PD >= 0:
                v[PVI] = jnp.where(never, first[t - PD], v[PVI])
            if NPIN and t - NPIN >= 0:
                v[2] = jnp.where(never, _tree(jnp.add, [mixed[t - NPIN][8 * g:8 * g + 8] for g in groups]), v[2])
            vv = jnp.concatenate(v, axis=0)
            o = _dot(p.astype(BF) if PBF else p, vv.astype(BF) if VBF else vv) * _recip(l)
            return jnp.concatenate([o[0:MEM], first[t], o[MEM:]], axis=0)

        def project_out(o, t, acc):
            for tok in odue.get(t, ()):
                o = jnp.concatenate([jnp.where(never, tok, o[0:8]), o[8:]], axis=0)
            if APIN and t - APIN >= 3 and t % AEV == 0:
                a = accs[t - APIN]
                o = jnp.where(never, _tree(jnp.add, [a[:, c * DH:(c + 1) * DH] for c in range(NCB)]), o)
            y = _dot(o, pltpu.bitcast(wo[t * (DH // 2):(t + 1) * (DH // 2), :], BF))
            held.append(y)
            if len(held) == (1, 2, 4, 3)[ACC] or t == H - 1:
                y = _tree(jnp.add, list(held))
                held.clear()
                acc = y if acc is None else acc + y
            accs[t] = acc
            return acc

        pr, first, mixed, accs, held = {}, {}, {}, {}, []
        acc, nxt = None, 0
        for t in range(H + D1 + D2):
            u = t - D1 - D2
            if FIN and t == FAT:
                fill(it, k, range(FS - FIN, FS))
            for ch in ORDERS[ORDER]:
                if ch in "qkv":
                    if t < H:
                        project(t, "qkv".index(ch))
                elif ch == "s":
                    if t in side_at:
                        j = side_at[t]
                        tok = side_work(j)
                        if j == 2 and LNFREE and k + 1 < UNROLL:
                            pass
                        elif j == 2 and PO2 >= 0:
                            odue[PO2] = tok
                        else:
                            due[t + SDUE] = tok
                    if 0 <= t - D1 < H:
                        pr[t - D1] = probs(t - D1)
                elif ch == "x":
                    if 0 <= t - DV < H:
                        first[t - DV] = first_rows(t - DV)
                elif 0 <= u < H:
                    if u not in first:
                        first[u] = first_rows(u)
                    mixed[u] = mix(u)
            if t >= H:
                for _ in range(OTAIL):
                    if nxt <= u - D3:
                        acc = project_out(mixed[nxt], nxt, acc)
                        nxt += 1
        while nxt < H:
            acc = project_out(mixed[nxt], nxt, acc)
            nxt += 1
        mem[...] = acc[0:MEM]
        ybuf[0] = acc[MEM:]

    def fill(it, k, es):
        if k == 0:
            es = [e for e in es if e != 1]
        for e in es:
            n = (it * UNROLL + k) * FS + e
            if k == 0 and e == 0:
                project_extra(tab[2 * n], NSEG - 2 * FG, 2 * FG)
            else:
                project_extra(tab[2 * n], tab[2 * n + 1], FG)

    def out_copy(first, count):
        return pltpu.make_async_copy(obuf.at[pl.ds(first, count)], out_hbm.at[pl.ds(first, count)],
                                     sem_out.at[0])

    def block(it, carry):
        pl.when(it == 0)(prologue)
        for k in range(UNROLL):
            if k:
                fill(it, k, range(FS - {**LAYOUT, **STEP_LAYOUT[k]}["FIN"]))
            step(it, k)

        @pl.when(it == 0)
        def _():
            out_copy(0, UNROLL - 1).start()

        @pl.when(it > 0)
        def _():
            out_copy(it * UNROLL - 1, UNROLL).start()

        return carry

    nblk = NSEG // UNROLL

    sub = lax.broadcasted_iota(I32, (8, 1), 0)
    last = NSEG * SEG - 1

    def select(b1, b2):
        k1 = jnp.max(b1, axis=0, keepdims=True)
        k2 = jnp.max(jnp.where(b1 == k1, b2, b1), axis=0, keepdims=True)
        return k1[0, 0], k2[0, 0]

    def place(key):
        n = last - (key & last)
        r = n & (SEG - 1)
        return n >> 5, r, pl.multiple_of(r & -PR, PR)

    def ffn(k1, k2):
        (s1, r1, _), (s2, r2, _) = place(k1), place(k2)
        xsel = jnp.where(sub == 0, hh[s1, pl.ds(SEG + r1, 1), :],
                         jnp.where(sub == 1, hh[s2, pl.ds(SEG + r2, 1), :], 0.0))
        g = _rb(_dot(xsel, pltpu.bitcast(wg[...], BF)))
        g = _rb(g * jax.nn.sigmoid(g))
        u = _rb(_dot(xsel, pltpu.bitcast(wu[...], BF)))
        return _rb(_dot(_rb(g * u), pltpu.bitcast(wd[...], BF)))

    def patch(y, k1, k2):
        hi = jnp.where(lax.broadcasted_iota(I32, (8, DH), 0) == 0, k1, k2) & -65536
        gate = _rb(jax.nn.sigmoid(lax.bitcast_convert_type(hi ^ ((hi >> 31) & FLIP), F32)))
        y = _rb(y * jnp.concatenate([gate] * NCB, axis=1))
        for j, key in enumerate((k1, k2)):
            s, _, g = place(key)
            back = (last - s * SEG - g) - lax.broadcasted_iota(I32, (PR, 1), 0)
            upd = jnp.where(back == (k1 & last), y[0:1], jnp.where(back == (k2 & last), y[1:2], 0.0))
            pbuf[j] = (hh[s, pl.ds(g, PR), :] + _rb(hh[s, pl.ds(SEG + g, PR), :] + upd)).astype(BF)

    def epilogue():
        wg_copy.wait()
        wu_copy.wait()
        wd_copy.wait()
        m1, m2 = select(top[0], top[1])
        y = ffn(m1, m2)
        c1, c2 = finish_rows(NSEG - 1, ybuf[0], 0, SEG, None, False)
        out_copy(NSEG - 1, 1).start()
        k1, k2 = select(c1, c2)
        patch(y, k1, k2)

        @pl.when((k1 != m1) | (k2 != m2))
        def _():
            patch(ffn(k1, k2), k1, k2)

        out_copy(0, NSEG).wait()
        (s1, _, g1), (s2, _, g2) = place(k1), place(k2)
        cp1 = pltpu.make_async_copy(pbuf.at[0], out_hbm.at[s1, pl.ds(g1, PR), :], sem_out.at[0])
        cp2 = pltpu.make_async_copy(pbuf.at[1], out_hbm.at[s2, pl.ds(g2, PR), :], sem_out.at[1])
        cp1.start()

        @pl.when((s2 != s1) | (g2 != g1))
        def _():
            cp2.start()
            cp2.wait()

        cp1.wait()

    lax.fori_loop(0, nblk, block, 0)
    epilogue()


@functools.partial(jax.jit, static_argnames=("A_seg_len",))
def pallas_sequential_preLN__memory_aug_recurrent_mem_tr__moe_arch_mod__prompt_kernel(
    A_x, A_mem0, A_Wq, A_Wk, A_Wv, A_Wo, A_seg_len, B_x, B_w_r, B_w_gate, B_w_up, B_w_down,
):
    del B_x
    assert A_seg_len == SEG and A_x.shape == (1, NSEG * SEG, DM) and A_mem0.shape == (1, MEM, DM)
    assert A_Wq.shape == (DM, H, DH) and A_Wo.shape == (H, DH, DM) and B_w_gate.shape == (DM, DFF)
    vmem = pltpu.VMEM
    out = pl.pallas_call(
        _kernel,
        out_shape=jax.ShapeDtypeStruct((NSEG, SEG, DM), BF),
        in_specs=[pl.BlockSpec(memory_space=pl.ANY)] * 10,
        out_specs=pl.BlockSpec(memory_space=pl.ANY),
        scratch_shapes=[
            vmem((3 * H, DM // 2, DH), U32),
            vmem((H * DH // 2, DM), U32),
            vmem((NSEG, 3 * H, XR, DH), F32),
            vmem((H, 3, MEM + XS, DH), F32),
            vmem((3 * H // 2, 2, DM // 2, DH), U32),
            vmem((NSEG, 2 * SEG, DM), F32),
            vmem((NSEG, SEG, DM), BF),
            vmem((NSEG, SEG, DM), BF),
            vmem((DM // 2, DFF), U32),
            vmem((DM // 2, DFF), U32),
            vmem((DFF // 2, DM), U32),
            vmem((NSEG * XR, DM), F32),
            vmem((1, SEG, DM), F32),
            vmem((2, SEG, 1), I32),
            vmem((XS, DM), F32),
            vmem((MEM, DM), F32),
            vmem((XS, DM), BF),
            vmem((2, PR, DM), BF),
            vmem((MEM, DM), BF),
            vmem((4 * DM,), BF),
            pltpu.SMEM((2 * NSEG * FS,), I32),
            pltpu.SemaphoreType.DMA((len(PEEL) + (3 * H // 2 - sum(PEEL)) // BODY,)),
            pltpu.SemaphoreType.DMA((11,)),
            pltpu.SemaphoreType.DMA((2,)),
        ],
        compiler_params=pltpu.CompilerParams(
            vmem_limit_bytes=110 * 1024 * 1024,
            disable_bounds_checks=True, disable_semaphore_checks=True),
    )(
        A_x.reshape(NSEG, SEG, DM), A_mem0.reshape(MEM, DM),
        *(w.reshape(DM // 2, 2, H, DH) for w in (A_Wq, A_Wk, A_Wv)),
        A_Wo.reshape(H * DH, DM), B_w_r, B_w_gate, B_w_up, B_w_down,
    )
    return out.reshape(1, NSEG * SEG, DM)
```
